```python
import jax
import jax.numpy as jnp

def _softmax(x, axis=-1):
    return jax.nn.softmax(x, axis=axis)
def _gelu(x):
    return jax.nn.gelu(x, approximate=True)
def _silu(x):
    return jax.nn.silu(x)
def _sigmoid(x):
    return jax.nn.sigmoid(x)
def _layernorm(x, axis=-1, eps=1e-5):
    m = jnp.mean(x, axis=axis, keepdims=True)
    v = jnp.var(x, axis=axis, keepdims=True)
    return (x - m) / jnp.sqrt(v + eps)
def _scatter_add(tgt, idx, src, axis=0):
    return tgt.at[idx].add(src)
def _segment_sum(src, seg, n):
    return jax.ops.segment_sum(src, seg, n)
class _Rng:
    def __init__(self, key):
        self._k = key
    def _next(self):
        self._k, sub = jax.random.split(self._k)
        return sub
    def normal(self, shape):
        return jax.random.normal(self._next(), shape, dtype=jnp.bfloat16)
    def randint(self, lo, hi, shape):
        return jax.random.randint(self._next(), shape, lo, hi, dtype=jnp.int32)
    def uniform(self, shape, lo=0.0, hi=1.0):
        return jax.random.uniform(self._next(), shape, jnp.bfloat16, lo, hi)
    def permutation(self, n):
        return jax.random.permutation(self._next(), n)


kernel_name = 'interleave_layers__compressed_kv_cla__moe_arch_mod__decode'

def setup_inputs():
    _rng = _Rng(jax.random.key(int.from_bytes(__import__("os").urandom(4), "little")))
    _w = (lambda a: (lambda t: t.astype(jnp.bfloat16) if jnp.issubdtype(t.dtype, jnp.floating) else t)(jnp.asarray(a)))
    def _A_setup():
        B, H, Sq, Sk, D, M = 1, 32, 1, 4096, 128, 640
        Dc = 4 * D
        return {
            "x": _w((lambda *s: _rng.normal(s) * 0.05)(B, Sq, M)),
            "c_kv": _w((lambda *s: _rng.normal(s) * 0.05)(B, Sk, Dc)),
            "w_q": _w((lambda *s: _rng.normal(s) * 0.05)(M, H, D) * (M ** -0.5)),
            "w_uk": _w((lambda *s: _rng.normal(s) * 0.05)(Dc, H, D) * (Dc ** -0.5)),
            "w_uv": _w((lambda *s: _rng.normal(s) * 0.05)(Dc, H, D) * (Dc ** -0.5)),
            "w_o": _w((lambda *s: _rng.normal(s) * 0.05)(H, D, M) * ((H * D) ** -0.5)),
        }
    _A_in = _A_setup()

    def _B_setup():
        B, S, D, F, C = 1, 1, 640, 1728, 1
        return {
            "x": _w((lambda *s: _rng.normal(s) * 0.05)(B, S, D)),
            "w_r": _w((lambda *s: _rng.normal(s) * 0.05)(D)),
            "w_gate": _w((lambda *s: _rng.normal(s) * 0.05)(D, F)),
            "w_up": _w((lambda *s: _rng.normal(s) * 0.05)(D, F)),
            "w_down": _w((lambda *s: _rng.normal(s) * 0.05)(F, D)),
        }
    _B_in = _B_setup()

    return {
        "A_x": _A_in["x"],
        "A_c_kv": _A_in["c_kv"],
        "A_w_q": _A_in["w_q"],
        "A_w_uk": _A_in["w_uk"],
        "A_w_uv": _A_in["w_uv"],
        "A_w_o": _A_in["w_o"],
        "B_x": _B_in["x"],
        "B_w_r": _B_in["w_r"],
        "B_w_gate": _B_in["w_gate"],
        "B_w_up": _B_in["w_up"],
        "B_w_down": _B_in["w_down"],
    }

def reference(A_x, A_c_kv, A_w_q, A_w_uk, A_w_uv, A_w_o, B_x, B_w_r, B_w_gate, B_w_up, B_w_down):
    def _A_ref(x, c_kv, w_q, w_uk, w_uv, w_o):
        B, Sq, M = x.shape[0], x.shape[1], x.shape[2]
        Sk = c_kv.shape[1]
        H, D = w_q.shape[1], w_q.shape[2]
        q = jnp.einsum("bqm,mhd->bhqd", x, w_q)
        k = jnp.einsum("bkc,chd->bhkd", c_kv, w_uk)
        v = jnp.einsum("bkc,chd->bhkd", c_kv, w_uv)
        scores = jnp.einsum("bhqd,bhkd->bhqk", q, k) * (D ** -0.5)
        off = Sk - Sq
        qi = jnp.arange(Sq)[:, None]
        kj = jnp.arange(Sk)[None, :]
        cmask = kj <= (qi + off)
        scores = jnp.where(cmask[None, None], scores, -1e9)
        p = _softmax(scores, axis=-1)
        ctx = jnp.einsum("bhqk,bhkd->bhqd", p, v)
        return jnp.einsum("bhqd,hdm->bqm", ctx, w_o)

    def _B_ref(x, w_r, w_gate, w_up, w_down):
        B, S, D = x.shape
        C = 1
        r = x @ w_r
        idx = jnp.argsort(-r, axis=-1)[:, :C]
        idx_e = jnp.repeat(idx.reshape(B, C, 1), D, axis=2)
        x_sel = jnp.take_along_axis(x, idx_e, axis=1)
        g = _silu(x_sel @ w_gate)
        u = x_sel @ w_up
        y = (g * u) @ w_down
        r_sel = _sigmoid(jnp.take_along_axis(r, idx, axis=1))
        y = y * r_sel.reshape(B, C, 1)
        b_off = (jnp.arange(B) * S).reshape(B, 1)
        flat_idx = (idx + b_off).reshape(B * C)
        zero = (x * 0.0).reshape(B * S, D)
        upd = _scatter_add(zero, flat_idx, y.reshape(B * C, D), axis=0)
        return x + upd.reshape(B, S, D)

    x = A_x
    x = x + _A_ref(_layernorm(x, axis=-1), A_c_kv, A_w_q, A_w_uk, A_w_uv, A_w_o)
    x = x + _B_ref(_layernorm(x, axis=-1), B_w_r, B_w_gate, B_w_up, B_w_down)
    x = x + _A_ref(_layernorm(x, axis=-1), A_c_kv, A_w_q, A_w_uk, A_w_uv, A_w_o)
    x = x + _B_ref(_layernorm(x, axis=-1), B_w_r, B_w_gate, B_w_up, B_w_down)
    return x
```

```python
import functools

import jax
import jax.numpy as jnp
import jax.experimental.pallas as pl
import jax.experimental.pallas.tpu as pltpu

F32 = jnp.float32
BF16 = jnp.bfloat16

H = 32
D = 128
M = 640
DC = 512
SK = 4096
FF = 1728
EPS = 1e-5
R = 8


def _dot(a, b):
    return jnp.dot(a, b, preferred_element_type=F32)


def _dot_nt(a, b):
    return jax.lax.dot_general(a, b, (((1,), (1,)), ((), ())),
                               preferred_element_type=F32)


def _layernorm(x):
    mu = jnp.mean(x, axis=-1, keepdims=True)
    xc = x - mu
    var = jnp.mean(xc * xc, axis=-1, keepdims=True)
    return xc / jnp.sqrt(var + EPS)


def _kernel(x_hbm, wr_hbm, wq_hbm, wuk_hbm, ckv_hbm, wuv_hbm, wo_hbm, wg_hbm,
            wu_hbm, wd_hbm,
            o_ref,
            x_v, wr_v, wq_l, wuk_l, ckv, wuv_l, wo, wg, wu, wd,
            wq_h, wuk_h, wuv_h, sems):
    srcs = (x_hbm, wr_hbm, wq_hbm, wuk_hbm, ckv_hbm, wuv_hbm, wo_hbm, wg_hbm,
            wu_hbm, wd_hbm)
    dsts = (x_v, wr_v, wq_l, wuk_l, ckv, wuv_l, wo, wg, wu, wd)
    copies = [pltpu.make_async_copy(s, d, sems.at[i])
              for i, (s, d) in enumerate(zip(srcs, dsts))]
    (c_x, c_wr, c_wq, c_wuk, c_ckv, c_wuv, c_wo, c_wg, c_wu, c_wd) = copies
    for c in copies:
        c.start()

    def relayout(src, dst, rows):
        chunk = 64
        for r0 in range(0, rows, chunk):
            dst[:, r0:r0 + chunk, :] = jnp.swapaxes(src[r0:r0 + chunk], 0, 1)

    sub = jax.lax.broadcasted_iota(jnp.int32, (R, 1), 0)

    def attention(x, first):
        xn = _layernorm(x)
        xn8 = jnp.broadcast_to(xn, (R, M)).astype(BF16)
        if first:
            c_wq.wait()
            relayout(wq_l, wq_h, M)
        q = [_dot(xn8, wq_h[h]).astype(BF16) for h in range(H)]
        if first:
            c_wuk.wait()
            relayout(wuk_l, wuk_h, DC)
        groups = []
        for g in range(H // R):
            acc = None
            for i in range(R):
                h = g * R + i
                qa = _dot_nt(q[h], wuk_h[h])
                acc = qa if acc is None else jnp.where(sub == i, qa, acc)
            groups.append(acc)
        qabs = jnp.concatenate(groups, axis=0) * (D ** -0.5)
        qabs = qabs.astype(BF16)
        if first:
            c_ckv.wait()
        s = _dot_nt(qabs, ckv[...])
        mx = jnp.max(s, axis=-1, keepdims=True)
        e = jnp.exp(s - mx)
        l = jnp.sum(e, axis=-1, keepdims=True)
        lat = _dot(e.astype(BF16), ckv[...]) / l
        lat = lat.astype(BF16)
        if first:
            c_wuv.wait()
            relayout(wuv_l, wuv_h, DC)
        ctx = []
        for h in range(H):
            g, i = divmod(h, R)
            c = _dot(lat[g * R:(g + 1) * R], wuv_h[h])
            ctx.append(jnp.where(sub == i, c, 0.0).astype(BF16))
        ctx = jnp.concatenate(ctx, axis=1)
        if first:
            c_wo.wait()
        o = _dot(ctx, wo[...])
        return x + jnp.sum(o, axis=0, keepdims=True)

    def ffn(x, first):
        xn = _layernorm(x)
        r = jnp.sum(xn * wr_v[...].astype(F32), axis=-1, keepdims=True)
        gate = jax.nn.sigmoid(r)
        xn8 = jnp.broadcast_to(xn, (R, M)).astype(BF16)
        if first:
            c_wg.wait()
        g = _dot_nt(xn8, wg[...])
        if first:
            c_wu.wait()
        u = _dot_nt(xn8, wu[...])
        act = (g * jax.nn.sigmoid(g) * u).astype(BF16)
        if first:
            c_wd.wait()
        y = _dot(act, wd[...])
        return x + xn + y[0:1] * gate

    c_x.wait()
    c_wr.wait()
    x = x_v[...].astype(F32)
    x = attention(x, True)
    x = ffn(x, True)
    x = attention(x, False)
    x = ffn(x, False)
    o_ref[...] = x.astype(o_ref.dtype)


@jax.jit
def pallas_interleave_layers__compressed_kv_cla__moe_arch_mod__decode_kernel(
    A_x: jax.Array,
    A_c_kv: jax.Array,
    A_w_q: jax.Array,
    A_w_uk: jax.Array,
    A_w_uv: jax.Array,
    A_w_o: jax.Array,
    B_x: jax.Array,
    B_w_r: jax.Array,
    B_w_gate: jax.Array,
    B_w_up: jax.Array,
    B_w_down: jax.Array,
):
    del B_x
    args = (
        A_x.reshape(1, M),
        B_w_r.reshape(1, M),
        A_w_q,
        A_w_uk,
        A_c_kv.reshape(SK, DC),
        A_w_uv,
        A_w_o.reshape(H * D, M),
        B_w_gate.T,
        B_w_up.T,
        B_w_down,
    )
    scratch = [pltpu.VMEM(a.shape, a.dtype) for a in args]
    scratch += [
        pltpu.VMEM((H, M, D), BF16),
        pltpu.VMEM((H, DC, D), BF16),
        pltpu.VMEM((H, DC, D), BF16),
        pltpu.SemaphoreType.DMA((len(args),)),
    ]
    out = pl.pallas_call(
        _kernel,
        out_shape=jax.ShapeDtypeStruct((1, M), A_x.dtype),
        in_specs=[pl.BlockSpec(memory_space=pl.ANY)] * len(args),
        out_specs=pl.BlockSpec(memory_space=pltpu.VMEM),
        scratch_shapes=scratch,
        compiler_params=pltpu.CompilerParams(
            vmem_limit_bytes=100 * 1024 * 1024),
        name="mla_moe_decode",
    )(*args)
    return out.reshape(1, 1, M)
```

```python
import jax
import jax.numpy as jnp
import jax.experimental.pallas as pl
import jax.experimental.pallas.tpu as pltpu

F32 = jnp.float32
BF16 = jnp.bfloat16
U32 = jnp.uint32

H = 32
D = 128
M = 640
DC = 512
SK = 4096
FF = 1728
EPS = 1e-5
R = 8
L = 128

MT = M // L
CT = DC // L
KT = SK // L
FT = -(-FF // L)
F_TAIL = FF - (FT - 1) * L
KCHUNK = 8
WO_CHUNKS = 4
WD_CHUNKS = ((0, 6), (6, 11), (11, FT))


SKEW_Q = 4
SKEW_S = 1
SKEW_O = 4
SKEW_F = 3


def _skewed(n, skew, produce, consume):
    for step in range(n + skew):
        if step < n:
            produce(step)
        if step >= skew:
            consume(step - skew)


def _dot(a, b):
    return jnp.dot(a, b, preferred_element_type=F32)


def _ld(ref32, idx):
    return pltpu.bitcast(ref32[idx], BF16)


def _st(ref32, idx, val):
    ref32[idx] = pltpu.bitcast(val, U32)


def _round_bf16(x):
    return x.astype(BF16).astype(F32)


def _stats(x):
    mu = jnp.mean(x, axis=-1, keepdims=True)
    xc = x - mu
    var = jnp.mean(xc * xc, axis=-1, keepdims=True)
    return mu, jax.lax.rsqrt(var + EPS)


def _lhs16(x):
    return jnp.concatenate([x, jnp.ones_like(x)], axis=0).astype(BF16)


def _kernel(x_hbm, wr_hbm, wq_hbm, wuk_hbm, ckv_hbm, wuv_hbm, wg_hbm, wu_hbm,
            wo_hbm, wd_hbm,
            o_ref,
            x_v, wr_v, wq_l, wuk_l, wuv_l, wg_l, wu_l, wo_l, wd_l,
            WQ, WUKT, CKV, CKT, WUV, WG, WU, WO, WD, sems):
    sem_ids = iter(range(64))

    def copy(src, dst):
        c = pltpu.make_async_copy(src, dst, sems.at[next(sem_ids)])
        c.start()
        return c

    c_x = copy(x_hbm, x_v)
    c_wr = copy(wr_hbm, wr_v)
    c_wq = copy(wq_hbm, wq_l)
    c_wuk = copy(wuk_hbm, wuk_l)
    c_ckv = [copy(ckv_hbm.at[:, pl.ds(ct * L, L)], CKV.at[ct]) for ct in range(CT)]
    c_wuv = copy(wuv_hbm, wuv_l)
    c_wg = copy(wg_hbm, wg_l)
    c_wu = copy(wu_hbm, wu_l)
    wo_rows = H * D // WO_CHUNKS
    c_wo = [copy(wo_hbm.at[pl.ds(c * wo_rows, wo_rows)],
                 wo_l.at[pl.ds(c * wo_rows, wo_rows)]) for c in range(WO_CHUNKS)]
    c_wd = []
    for (f0, f1) in WD_CHUNKS:
        r0, r1 = f0 * L, min(f1 * L, FF)
        c_wd.append(copy(wd_hbm.at[pl.ds(r0, r1 - r0)], wd_l.at[pl.ds(r0, r1 - r0)]))

    wq_l32, wuk_l32, wuv_l32 = (r.bitcast(U32) for r in (wq_l, wuk_l, wuv_l))
    WQ32, WUKT32, CKV32, CKT32, WUV32, WG32, WU32, WO32, WD32 = (
        r.bitcast(U32) for r in (WQ, WUKT, CKV, CKT, WUV, WG, WU, WO, WD))

    def swap_heads(src32, dst32, rows):
        ch = 64

        def body(i, carry):
            r0 = pl.multiple_of(i * ch, ch)
            w = _ld(src32, pl.ds(r0, ch))
            dst32[:, pl.ds(pl.multiple_of(i * (ch // 2), ch // 2), ch // 2), :] = (
                pltpu.bitcast(jnp.swapaxes(w, 0, 1), U32))
            return carry
        jax.lax.fori_loop(0, rows // ch, body, 0)

    def make_wukt():
        def body(i, carry):
            w = _ld(wuk_l32, pl.ds(pl.multiple_of(i * L, L), L))
            w = jnp.swapaxes(jnp.swapaxes(w, 0, 1), 1, 2)
            WUKT32[:, pl.ds(pl.multiple_of(i * (L // 2), L // 2), L // 2), :] = (
                pltpu.bitcast(w, U32))
            return carry
        jax.lax.fori_loop(0, CT, body, 0)

    def make_ckt():
        def body(kt, carry):
            for ct in range(CT):
                w = _ld(CKV32, (ct, pl.ds(pl.multiple_of(kt * (L // 2), L // 2), L // 2)))
                CKT32[kt, ct * (L // 2):(ct + 1) * (L // 2), :] = pltpu.bitcast(w.T, U32)
            return carry
        jax.lax.fori_loop(0, KT, body, 0)

    def make_wgu(src, dst32):
        def body(ft, carry):
            w = src[pl.ds(pl.multiple_of(ft * L, L), L), :]
            dst32[ft] = pltpu.bitcast(w.T, U32)
            return carry
        jax.lax.fori_loop(0, FT - 1, body, 0)
        w = src[(FT - 1) * L:FF, :]
        w = jnp.concatenate([w, jnp.zeros((L - F_TAIL, M), BF16)], axis=0)
        dst32[FT - 1] = pltpu.bitcast(w.T, U32)

    def make_cols(src, dst32, r0, rows):
        for nt in range(MT):
            dst32[nt, r0 // 2:(r0 + rows) // 2, :] = pltpu.bitcast(
                src[r0:r0 + rows, nt * L:(nt + 1) * L], U32)

    sub = jax.lax.broadcasted_iota(jnp.int32, (R, L), 0)

    def attention(x, first):
        mu, rstd = _stats(x)
        lhs = _lhs16(x)
        qscale = rstd * (D ** -0.5)
        if first:
            c_wq.wait()
            swap_heads(wq_l32, WQ32, M)
            c_wuk.wait()
            make_wukt()
        qa = [[None] * CT for _ in range(H // R)]
        qh = [None] * H

        def q_head(h):
            oq = _dot(lhs, _ld(WQ32, h))
            qh[h] = ((oq[:R] - mu * oq[R:]) * qscale).astype(BF16)

        def qabs_head(h):
            g, i = divmod(h, R)
            for ct in range(CT):
                t = _dot(qh[h], _ld(WUKT32, (h, slice(ct * L // 2, (ct + 1) * L // 2))))
                qa[g][ct] = t if i == 0 else jnp.where(sub == i, t, qa[g][ct])

        _skewed(H, SKEW_Q, q_head, qabs_head)
        qabs = jnp.concatenate(
            [jnp.concatenate(row, axis=1) for row in qa], axis=0).astype(BF16)

        if first:
            for c in c_ckv:
                c.wait()
            make_ckt()
        nch = KT // KCHUNK
        ms, ls, lats, ps = [None] * nch, [None] * nch, [None] * nch, [None] * nch

        def scores_chunk(j):
            s = [_dot(qabs, _ld(CKT32, kt))
                 for kt in range(j * KCHUNK, (j + 1) * KCHUNK)]
            mx = s[0]
            for t in s[1:]:
                mx = jnp.maximum(mx, t)
            mx = jnp.max(mx, axis=-1, keepdims=True)
            e = [jnp.exp(t - mx) for t in s]
            lsum = e[0]
            for t in e[1:]:
                lsum = lsum + t
            ps[j] = jnp.concatenate(e, axis=1).astype(BF16)
            ms[j] = mx
            ls[j] = lsum

        def lat_chunk(j):
            k0 = j * KCHUNK * L // 2
            lats[j] = [_dot(ps[j], _ld(CKV32, (ct, slice(k0, k0 + KCHUNK * L // 2))))
                       for ct in range(CT)]

        _skewed(nch, SKEW_S, scores_chunk, lat_chunk)
        m = ms[0]
        for t in ms[1:]:
            m = jnp.maximum(m, t)
        alpha = [jnp.exp(t - m) for t in ms]
        lsum = alpha[0] * ls[0]
        for a, t in zip(alpha[1:], ls[1:]):
            lsum = lsum + a * t
        inv = 1.0 / jnp.sum(lsum, axis=-1, keepdims=True)
        lat = []
        for ct in range(CT):
            t = alpha[0] * lats[0][ct]
            for j in range(1, len(lats)):
                t = t + alpha[j] * lats[j][ct]
            lat.append(t * inv)
        lat = jnp.concatenate(lat, axis=1)
        latg = [lat[g * R:(g + 1) * R].astype(BF16) for g in range(H // R)]

        if first:
            c_wuv.wait()
            swap_heads(wuv_l32, WUV32, DC)

        def ctx_head(h):
            g, i = divmod(h, R)
            c = _dot(latg[g], _ld(WUV32, h))
            return jnp.broadcast_to(c[i:i + 1], (R, D)).astype(BF16)

        def out_head(h, cb, o):
            for nt in range(MT):
                t = _dot(cb, _ld(WO32, (nt, slice(h * L // 2, (h + 1) * L // 2))))
                o[nt] = t if o[nt] is None else o[nt] + t

        o = [None] * MT
        if first:
            cbs = [ctx_head(h) for h in range(H)]
            c_wg.wait()
            make_wgu(wg_l, WG32)
            c_wu.wait()
            make_wgu(wu_l, WU32)
            hpc = H // WO_CHUNKS
            for c in range(WO_CHUNKS):
                c_wo[c].wait()
                make_cols(wo_l, WO32, c * wo_rows, wo_rows)
                for h in range(c * hpc, (c + 1) * hpc):
                    out_head(h, cbs[h], o)
        else:
            cbs = [None] * H

            def ctx_stage(h):
                cbs[h] = ctx_head(h)

            _skewed(H, SKEW_O, ctx_stage, lambda h: out_head(h, cbs[h], o))
        return _round_bf16(x + jnp.concatenate(o, axis=1))

    def ffn(x, first):
        mu, rstd = _stats(x)
        lhs = _lhs16(x)
        xn = (x - mu) * rstd
        r = jnp.sum(xn * wr_v[...].reshape(1, M).astype(F32), axis=-1, keepdims=True)
        gate = jax.nn.sigmoid(r)

        def act_tile(ft):
            og = _dot(lhs, _ld(WG32, ft))
            ou = _dot(lhs, _ld(WU32, ft))
            g = (og[:R] - mu * og[R:]) * rstd
            u = (ou[:R] - mu * ou[R:]) * rstd
            return (g * jax.nn.sigmoid(g) * u).astype(BF16)

        def down_tile(ft, a, y):
            for nt in range(MT):
                if first:
                    r0 = ft * L
                    if ft < FT - 1:
                        t = _dot(a, wd_l[r0:r0 + L, nt * L:(nt + 1) * L])
                    else:
                        t = _dot(a[:, :F_TAIL], wd_l[r0:FF, nt * L:(nt + 1) * L])
                else:
                    r0 = ft * L // 2
                    if ft < FT - 1:
                        t = _dot(a, _ld(WD32, (nt, slice(r0, r0 + L // 2))))
                    else:
                        t = _dot(a[:, :F_TAIL], _ld(WD32, (nt, slice(r0, FF // 2))))
                y[nt] = t if y[nt] is None else y[nt] + t

        y = [None] * MT
        if first:
            acts = [act_tile(ft) for ft in range(FT)]
            for c, (f0, f1) in enumerate(WD_CHUNKS):
                c_wd[c].wait()
                for ft in range(f0, f1):
                    down_tile(ft, acts[ft], y)
        else:
            acts = [None] * FT

            def act_stage(ft):
                acts[ft] = act_tile(ft)

            _skewed(FT, SKEW_F, act_stage, lambda ft: down_tile(ft, acts[ft], y))
        return _round_bf16(x + xn + jnp.concatenate(y, axis=1) * gate)

    c_x.wait()
    c_wr.wait()
    x = jnp.broadcast_to(x_v[...].astype(F32), (R, M))
    x = attention(x, True)
    x = ffn(x, True)
    make_cols(wd_l, WD32, 0, FF)
    x = attention(x, False)
    x = ffn(x, False)
    o_ref[...] = x[0:1].astype(o_ref.dtype)


@jax.jit
def pallas_interleave_layers__compressed_kv_cla__moe_arch_mod__decode_kernel(
    A_x: jax.Array,
    A_c_kv: jax.Array,
    A_w_q: jax.Array,
    A_w_uk: jax.Array,
    A_w_uv: jax.Array,
    A_w_o: jax.Array,
    B_x: jax.Array,
    B_w_r: jax.Array,
    B_w_gate: jax.Array,
    B_w_up: jax.Array,
    B_w_down: jax.Array,
):
    del B_x
    args = (
        A_x.reshape(1, M),
        B_w_r,
        A_w_q,
        A_w_uk,
        A_c_kv.reshape(SK, DC),
        A_w_uv,
        B_w_gate.T,
        B_w_up.T,
        A_w_o.reshape(H * D, M),
        B_w_down,
    )
    scratch = [
        pltpu.VMEM((1, M), BF16),
        pltpu.VMEM((M,), BF16),
        pltpu.VMEM((M, H, D), BF16),
        pltpu.VMEM((DC, H, D), BF16),
        pltpu.VMEM((DC, H, D), BF16),
        pltpu.VMEM((FF, M), BF16),
        pltpu.VMEM((FF, M), BF16),
        pltpu.VMEM((H * D, M), BF16),
        pltpu.VMEM((FF, M), BF16),
        pltpu.VMEM((H, M, D), BF16),
        pltpu.VMEM((H, DC, L), BF16),
        pltpu.VMEM((CT, SK, L), BF16),
        pltpu.VMEM((KT, DC, L), BF16),
        pltpu.VMEM((H, DC, D), BF16),
        pltpu.VMEM((FT, M, L), BF16),
        pltpu.VMEM((FT, M, L), BF16),
        pltpu.VMEM((MT, H * D, L), BF16),
        pltpu.VMEM((MT, FF, L), BF16),
        pltpu.SemaphoreType.DMA((24,)),
    ]
    out = pl.pallas_call(
        _kernel,
        out_shape=jax.ShapeDtypeStruct((1, M), A_x.dtype),
        in_specs=[pl.BlockSpec(memory_space=pl.ANY)] * len(args),
        out_specs=pl.BlockSpec(memory_space=pltpu.VMEM),
        scratch_shapes=scratch,
        compiler_params=pltpu.CompilerParams(
            vmem_limit_bytes=100 * 1024 * 1024),
        name="mla_moe_decode",
    )(*args)
    return out.reshape(1, 1, M)
```

```python
import jax
import jax.numpy as jnp
import jax.experimental.pallas as pl
import jax.experimental.pallas.tpu as pltpu

F32 = jnp.float32
BF16 = jnp.bfloat16
U32 = jnp.uint32

H = 32
D = 128
M = 640
DC = 512
SK = 4096
FF = 1728
EPS = 1e-5
R = 8
L = 128

MT = M // L
CT = DC // L
KT = SK // L
FT = -(-FF // L)
F_TAIL = FF - (FT - 1) * L
KCHUNK = 8
WO_CHUNKS = 4
WD_CHUNKS = ((0, 6), (6, 11), (11, FT))


N_LAYERS = 2
SMALL_FIRST = False
SKEW_Q = 8
SKEW_S = 1
SKEW_O = 6
SKEW_F = 5


def _skewed(n, skew, produce, consume):
    for step in range(n + skew):
        if step < n:
            produce(step)
        if step >= skew:
            consume(step - skew)


def _dot(a, b):
    return jnp.dot(a, b, preferred_element_type=F32)


def _ld(ref32, idx):
    return pltpu.bitcast(ref32[idx], BF16)


def _st(ref32, idx, val):
    ref32[idx] = pltpu.bitcast(val, U32)


def _round_bf16(x):
    return x.astype(BF16).astype(F32)


def _stats(x):
    mu = jnp.mean(x, axis=-1, keepdims=True)
    xc = x - mu
    var = jnp.mean(xc * xc, axis=-1, keepdims=True)
    return mu, jax.lax.rsqrt(var + EPS)


def _lhs16(x):
    return jnp.concatenate([x, jnp.ones_like(x)], axis=0).astype(BF16)


def _kernel(x_hbm, wr_hbm, wq_hbm, wuk_hbm, ckv_hbm, wuv_hbm, wg_hbm, wu_hbm,
            wo_hbm, wd_hbm,
            o_ref,
            x_v, wr_v, wq_l, wuk_l, wuv_l, wg_l, wu_l, wo_l, wd_l,
            WQ, WUKT, CKV, CKT, WUV, WG, WU, WO, WD, sems):
    sem_ids = iter(range(64))

    def copy(src, dst):
        c = pltpu.make_async_copy(src, dst, sems.at[next(sem_ids)])
        c.start()
        return c

    if SMALL_FIRST:
        c_x = copy(x_hbm, x_v)
        c_wr = copy(wr_hbm, wr_v)
        c_wq = copy(wq_hbm, wq_l)
    else:
        c_wq = copy(wq_hbm, wq_l)
        c_x = copy(x_hbm, x_v)
        c_wr = copy(wr_hbm, wr_v)
    c_wuk = copy(wuk_hbm, wuk_l)
    c_ckv = [copy(ckv_hbm.at[:, pl.ds(ct * L, L)], CKV.at[ct]) for ct in range(CT)]
    c_wuv = copy(wuv_hbm, wuv_l)
    c_wg = copy(wg_hbm, wg_l)
    c_wu = copy(wu_hbm, wu_l)
    wo_rows = H * D // WO_CHUNKS
    c_wo = [copy(wo_hbm.at[pl.ds(c * wo_rows, wo_rows)],
                 wo_l.at[pl.ds(c * wo_rows, wo_rows)]) for c in range(WO_CHUNKS)]
    c_wd = []
    for (f0, f1) in WD_CHUNKS:
        r0, r1 = f0 * L, min(f1 * L, FF)
        c_wd.append(copy(wd_hbm.at[pl.ds(r0, r1 - r0)], wd_l.at[pl.ds(r0, r1 - r0)]))

    wq_l32, wuk_l32, wuv_l32 = (r.bitcast(U32) for r in (wq_l, wuk_l, wuv_l))
    WQ32, WUKT32, CKV32, CKT32, WUV32, WG32, WU32, WO32, WD32 = (
        r.bitcast(U32) for r in (WQ, WUKT, CKV, CKT, WUV, WG, WU, WO, WD))

    def swap_heads(src32, dst32, rows):
        ch = 64

        def body(i, carry):
            r0 = pl.multiple_of(i * ch, ch)
            w = _ld(src32, pl.ds(r0, ch))
            dst32[:, pl.ds(pl.multiple_of(i * (ch // 2), ch // 2), ch // 2), :] = (
                pltpu.bitcast(jnp.swapaxes(w, 0, 1), U32))
            return carry
        jax.lax.fori_loop(0, rows // ch, body, 0)

    def make_wukt():
        def body(i, carry):
            w = _ld(wuk_l32, pl.ds(pl.multiple_of(i * L, L), L))
            w = jnp.swapaxes(jnp.swapaxes(w, 0, 1), 1, 2)
            WUKT32[:, pl.ds(pl.multiple_of(i * (L // 2), L // 2), L // 2), :] = (
                pltpu.bitcast(w, U32))
            return carry
        jax.lax.fori_loop(0, CT, body, 0)

    def make_ckt():
        def body(kt, carry):
            for ct in range(CT):
                w = _ld(CKV32, (ct, pl.ds(pl.multiple_of(kt * (L // 2), L // 2), L // 2)))
                CKT32[kt, ct * (L // 2):(ct + 1) * (L // 2), :] = pltpu.bitcast(w.T, U32)
            return carry
        jax.lax.fori_loop(0, KT, body, 0)

    def make_wgu(src, dst32):
        def body(ft, carry):
            w = src[pl.ds(pl.multiple_of(ft * L, L), L), :]
            dst32[ft] = pltpu.bitcast(w.T, U32)
            return carry
        jax.lax.fori_loop(0, FT - 1, body, 0)
        w = src[(FT - 1) * L:FF, :]
        w = jnp.concatenate([w, jnp.zeros((L - F_TAIL, M), BF16)], axis=0)
        dst32[FT - 1] = pltpu.bitcast(w.T, U32)

    def make_cols(src, dst32, r0, rows):
        for nt in range(MT):
            dst32[nt, r0 // 2:(r0 + rows) // 2, :] = pltpu.bitcast(
                src[r0:r0 + rows, nt * L:(nt + 1) * L], U32)

    sub = jax.lax.broadcasted_iota(jnp.int32, (R, L), 0)

    def attention(x, first):
        mu, rstd = _stats(x)
        lhs = _lhs16(x)
        qscale = rstd * (D ** -0.5)
        if first:
            c_wq.wait()
            swap_heads(wq_l32, WQ32, M)
            c_wuk.wait()
            make_wukt()
        qa = [[None] * CT for _ in range(H // R)]
        qh = [None] * H

        def q_head(h):
            oq = _dot(lhs, _ld(WQ32, h))
            qh[h] = ((oq[:R] - mu * oq[R:]) * qscale).astype(BF16)

        def qabs_head(h):
            g, i = divmod(h, R)
            for ct in range(CT):
                t = _dot(qh[h], _ld(WUKT32, (h, slice(ct * L // 2, (ct + 1) * L // 2))))
                qa[g][ct] = t if i == 0 else jnp.where(sub == i, t, qa[g][ct])

        _skewed(H, SKEW_Q, q_head, qabs_head)
        qabs = jnp.concatenate(
            [jnp.concatenate(row, axis=1) for row in qa], axis=0).astype(BF16)

        if first:
            for c in c_ckv:
                c.wait()
            make_ckt()
        nch = KT // KCHUNK
        ms, ls, lats, ps = [None] * nch, [None] * nch, [None] * nch, [None] * nch

        def scores_chunk(j):
            s = [_dot(qabs, _ld(CKT32, kt))
                 for kt in range(j * KCHUNK, (j + 1) * KCHUNK)]
            mx = s[0]
            for t in s[1:]:
                mx = jnp.maximum(mx, t)
            mx = jnp.max(mx, axis=-1, keepdims=True)
            e = [jnp.exp(t - mx) for t in s]
            lsum = e[0]
            for t in e[1:]:
                lsum = lsum + t
            ps[j] = jnp.concatenate(e, axis=1).astype(BF16)
            ms[j] = mx
            ls[j] = lsum

        def lat_chunk(j):
            k0 = j * KCHUNK * L // 2
            lats[j] = [_dot(ps[j], _ld(CKV32, (ct, slice(k0, k0 + KCHUNK * L // 2))))
                       for ct in range(CT)]

        _skewed(nch, SKEW_S, scores_chunk, lat_chunk)
        m = ms[0]
        for t in ms[1:]:
            m = jnp.maximum(m, t)
        alpha = [jnp.exp(t - m) for t in ms]
        lsum = alpha[0] * ls[0]
        for a, t in zip(alpha[1:], ls[1:]):
            lsum = lsum + a * t
        inv = 1.0 / jnp.sum(lsum, axis=-1, keepdims=True)
        lat = []
        for ct in range(CT):
            t = alpha[0] * lats[0][ct]
            for j in range(1, len(lats)):
                t = t + alpha[j] * lats[j][ct]
            lat.append(t * inv)
        lat = jnp.concatenate(lat, axis=1)
        latg = [lat[g * R:(g + 1) * R].astype(BF16) for g in range(H // R)]

        if first:
            c_wuv.wait()
            swap_heads(wuv_l32, WUV32, DC)

        def ctx_head(h):
            g, i = divmod(h, R)
            c = _dot(latg[g], _ld(WUV32, h))
            return jnp.broadcast_to(c[i:i + 1], (R, D)).astype(BF16)

        def out_head(h, cb, o):
            for nt in range(MT):
                t = _dot(cb, _ld(WO32, (nt, slice(h * L // 2, (h + 1) * L // 2))))
                o[nt] = t if o[nt] is None else o[nt] + t

        o = [None] * MT
        if first:
            cbs = [ctx_head(h) for h in range(H)]
            c_wg.wait()
            make_wgu(wg_l, WG32)
            c_wu.wait()
            make_wgu(wu_l, WU32)
            hpc = H // WO_CHUNKS
            for c in range(WO_CHUNKS):
                c_wo[c].wait()
                make_cols(wo_l, WO32, c * wo_rows, wo_rows)
                for h in range(c * hpc, (c + 1) * hpc):
                    out_head(h, cbs[h], o)
        else:
            cbs = [None] * H

            def ctx_stage(h):
                cbs[h] = ctx_head(h)

            _skewed(H, SKEW_O, ctx_stage, lambda h: out_head(h, cbs[h], o))
        return _round_bf16(x + jnp.concatenate(o, axis=1))

    def ffn(x, first):
        mu, rstd = _stats(x)
        lhs = _lhs16(x)
        xn = (x - mu) * rstd
        r = jnp.sum(xn * wr_v[...].reshape(1, M).astype(F32), axis=-1, keepdims=True)
        gate = jax.nn.sigmoid(r)

        def act_tile(ft):
            og = _dot(lhs, _ld(WG32, ft))
            ou = _dot(lhs, _ld(WU32, ft))
            g = (og[:R] - mu * og[R:]) * rstd
            u = (ou[:R] - mu * ou[R:]) * rstd
            return (g * jax.nn.sigmoid(g) * u).astype(BF16)

        def down_tile(ft, a, y):
            for nt in range(MT):
                if first:
                    r0 = ft * L
                    if ft < FT - 1:
                        t = _dot(a, wd_l[r0:r0 + L, nt * L:(nt + 1) * L])
                    else:
                        t = _dot(a[:, :F_TAIL], wd_l[r0:FF, nt * L:(nt + 1) * L])
                else:
                    r0 = ft * L // 2
                    if ft < FT - 1:
                        t = _dot(a, _ld(WD32, (nt, slice(r0, r0 + L // 2))))
                    else:
                        t = _dot(a[:, :F_TAIL], _ld(WD32, (nt, slice(r0, FF // 2))))
                y[nt] = t if y[nt] is None else y[nt] + t

        y = [None] * MT
        if first:
            acts = [act_tile(ft) for ft in range(FT)]
            for c, (f0, f1) in enumerate(WD_CHUNKS):
                c_wd[c].wait()
                for ft in range(f0, f1):
                    down_tile(ft, acts[ft], y)
        else:
            acts = [None] * FT

            def act_stage(ft):
                acts[ft] = act_tile(ft)

            _skewed(FT, SKEW_F, act_stage, lambda ft: down_tile(ft, acts[ft], y))
        return _round_bf16(x + xn + jnp.concatenate(y, axis=1) * gate)

    c_x.wait()
    c_wr.wait()
    x = jnp.broadcast_to(x_v[...].astype(F32), (R, M))
    x = attention(x, True)
    x = ffn(x, True)
    if N_LAYERS > 1:
        make_cols(wd_l, WD32, 0, FF)
        x = attention(x, False)
        x = ffn(x, False)
    o_ref[...] = x[0:1].astype(o_ref.dtype)


@jax.jit
def pallas_interleave_layers__compressed_kv_cla__moe_arch_mod__decode_kernel(
    A_x: jax.Array,
    A_c_kv: jax.Array,
    A_w_q: jax.Array,
    A_w_uk: jax.Array,
    A_w_uv: jax.Array,
    A_w_o: jax.Array,
    B_x: jax.Array,
    B_w_r: jax.Array,
    B_w_gate: jax.Array,
    B_w_up: jax.Array,
    B_w_down: jax.Array,
):
    del B_x
    args = (
        A_x.reshape(1, M),
        B_w_r,
        A_w_q,
        A_w_uk,
        A_c_kv.reshape(SK, DC),
        A_w_uv,
        B_w_gate.T,
        B_w_up.T,
        A_w_o.reshape(H * D, M),
        B_w_down,
    )
    scratch = [
        pltpu.VMEM((1, M), BF16),
        pltpu.VMEM((M,), BF16),
        pltpu.VMEM((M, H, D), BF16),
        pltpu.VMEM((DC, H, D), BF16),
        pltpu.VMEM((DC, H, D), BF16),
        pltpu.VMEM((FF, M), BF16),
        pltpu.VMEM((FF, M), BF16),
        pltpu.VMEM((H * D, M), BF16),
        pltpu.VMEM((FF, M), BF16),
        pltpu.VMEM((H, M, D), BF16),
        pltpu.VMEM((H, DC, L), BF16),
        pltpu.VMEM((CT, SK, L), BF16),
        pltpu.VMEM((KT, DC, L), BF16),
        pltpu.VMEM((H, DC, D), BF16),
        pltpu.VMEM((FT, M, L), BF16),
        pltpu.VMEM((FT, M, L), BF16),
        pltpu.VMEM((MT, H * D, L), BF16),
        pltpu.VMEM((MT, FF, L), BF16),
        pltpu.SemaphoreType.DMA((19,)),
    ]
    out = pl.pallas_call(
        _kernel,
        out_shape=jax.ShapeDtypeStruct((1, M), A_x.dtype),
        in_specs=[pl.BlockSpec(memory_space=pl.ANY)] * len(args),
        out_specs=pl.BlockSpec(memory_space=pltpu.VMEM),
        scratch_shapes=scratch,
        compiler_params=pltpu.CompilerParams(
            vmem_limit_bytes=100 * 1024 * 1024),
        name="mla_moe_decode",
    )(*args)
    return out.reshape(1, 1, M)
```

```python
import jax
import jax.numpy as jnp
import jax.experimental.pallas as pl
import jax.experimental.pallas.tpu as pltpu

F32 = jnp.float32
BF16 = jnp.bfloat16
U32 = jnp.uint32

H = 32
D = 128
M = 640
DC = 512
SK = 4096
FF = 1728
EPS = 1e-5
R = 8
L = 128

MT = M // L
CT = DC // L
KT = SK // L
FT = -(-FF // L)
F_TAIL = FF - (FT - 1) * L
KCHUNK = 8
WO_CHUNKS = 4
WD_CHUNKS = ((0, 6), (6, 11), (11, FT))


N_LAYERS = 2
SMALL_FIRST = False
SKEW_Q = 8
SKEW_S = 1
SKEW_O = 6
SKEW_F = 5


def _skewed(n, skew, produce, consume):
    for step in range(n + skew):
        if step < n:
            produce(step)
        if step >= skew:
            consume(step - skew)


VQ_HEADS = 16
VQ_GROUP = 4
P1_CFG = (30, 1.0, 2, 18, 1)


def _cosched(ms, vs, cfg):
    vstart, vrate, lag_v, lag_m, nlink = cfg
    mres, vres = [], []
    j = 0

    def emit_v(dep):
        nonlocal j
        vres.append(vs[j](dep))
        j += 1

    for i, m in enumerate(ms):
        while not getattr(m, "ready", lambda: True)():
            emit_v(None)
        dep = None
        if len(vres) > lag_v and i % nlink == 0 and j < len(vs):
            dep = vres[-1 - lag_v]
        mres.append(m(dep))
        while j < len(vs) and j < (i + 1 - vstart) * vrate:
            emit_v(mres[-1 - lag_m] if (len(mres) > lag_m and j % 2 == 0) else None)
    while j < len(vs):
        emit_v(None)


def _lo(w):
    return pltpu.bitcast(w << 16, F32)


def _hi(w):
    return pltpu.bitcast(w & jnp.uint32(0xFFFF0000), F32)


def _sublane_sum(t):
    t = t + pltpu.roll(t, 4, 0)
    t = t + pltpu.roll(t, 2, 0)
    return t + pltpu.roll(t, 1, 0)


def _col_bcast(row):
    return pltpu.bitcast(jnp.broadcast_to(row, (L, L)).T, U32)


def _dot(a, b):
    return jnp.dot(a, b, preferred_element_type=F32)


def _ld(ref32, idx):
    return pltpu.bitcast(ref32[idx], BF16)


def _st(ref32, idx, val):
    ref32[idx] = pltpu.bitcast(val, U32)


def _round_bf16(x):
    return x.astype(BF16).astype(F32)


def _stats(x):
    mu = jnp.mean(x, axis=-1, keepdims=True)
    xc = x - mu
    var = jnp.mean(xc * xc, axis=-1, keepdims=True)
    return mu, jax.lax.rsqrt(var + EPS)


def _lhs16(x):
    return jnp.concatenate([x, jnp.ones_like(x)], axis=0).astype(BF16)


def _kernel(x_hbm, wr_hbm, wq_hbm, wuk_hbm, ckv_hbm, wuv_hbm, wg_hbm, wu_hbm,
            wo_hbm, wd_hbm,
            o_ref,
            x_v, x_v2, wr_v, wq_l, wuk_l, wuv_l, wg_l, wu_l, wo_l, wd_l,
            WQ, WUKT, CKV, CKT, WUV, WG, WU, WO, WD,
            CSQ, XE, XO, sems):
    sem_ids = iter(range(64))

    def copy(src, dst):
        c = pltpu.make_async_copy(src, dst, sems.at[next(sem_ids)])
        c.start()
        return c

    if SMALL_FIRST:
        c_x = copy(x_hbm, x_v)
        c_wr = copy(wr_hbm, wr_v)
        c_wq = copy(wq_hbm, wq_l)
    else:
        c_wq = copy(wq_hbm, wq_l)
        c_x = copy(x_hbm, x_v)
        c_wr = copy(wr_hbm, wr_v)
    c_x2 = copy(x_hbm, x_v2)
    c_wuk = copy(wuk_hbm, wuk_l)
    c_ckv = [copy(ckv_hbm.at[:, pl.ds(ct * L, L)], CKV.at[ct]) for ct in range(CT)]
    c_wuv = copy(wuv_hbm, wuv_l)
    c_wg = copy(wg_hbm, wg_l)
    c_wu = copy(wu_hbm, wu_l)
    wo_rows = H * D // WO_CHUNKS
    c_wo = [copy(wo_hbm.at[pl.ds(c * wo_rows, wo_rows)],
                 wo_l.at[pl.ds(c * wo_rows, wo_rows)]) for c in range(WO_CHUNKS)]
    c_wd = []
    for (f0, f1) in WD_CHUNKS:
        r0, r1 = f0 * L, min(f1 * L, FF)
        c_wd.append(copy(wd_hbm.at[pl.ds(r0, r1 - r0)], wd_l.at[pl.ds(r0, r1 - r0)]))

    wq_l32, wuk_l32, wuv_l32 = (r.bitcast(U32) for r in (wq_l, wuk_l, wuv_l))
    WQ32, WUKT32, CKV32, CKT32, WUV32, WG32, WU32, WO32, WD32 = (
        r.bitcast(U32) for r in (WQ, WUKT, CKV, CKT, WUV, WG, WU, WO, WD))

    def swap_heads(src32, dst32, rows):
        ch = 64

        def body(i, carry):
            r0 = pl.multiple_of(i * ch, ch)
            w = _ld(src32, pl.ds(r0, ch))
            dst32[:, pl.ds(pl.multiple_of(i * (ch // 2), ch // 2), ch // 2), :] = (
                pltpu.bitcast(jnp.swapaxes(w, 0, 1), U32))
            return carry
        jax.lax.fori_loop(0, rows // ch, body, 0)

    def make_wukt():
        def body(i, carry):
            w = _ld(wuk_l32, pl.ds(pl.multiple_of(i * L, L), L))
            w = jnp.swapaxes(jnp.swapaxes(w, 0, 1), 1, 2)
            WUKT32[:, pl.ds(pl.multiple_of(i * (L // 2), L // 2), L // 2), :] = (
                pltpu.bitcast(w, U32))
            return carry
        jax.lax.fori_loop(0, CT, body, 0)

    def make_ckt():
        def body(kt, carry):
            for ct in range(CT):
                w = _ld(CKV32, (ct, pl.ds(pl.multiple_of(kt * (L // 2), L // 2), L // 2)))
                CKT32[kt, ct * (L // 2):(ct + 1) * (L // 2), :] = pltpu.bitcast(w.T, U32)
            return carry
        jax.lax.fori_loop(0, KT, body, 0)

    def make_wgu(src, dst32):
        def body(ft, carry):
            w = src[pl.ds(pl.multiple_of(ft * L, L), L), :]
            dst32[ft] = pltpu.bitcast(w.T, U32)
            return carry
        jax.lax.fori_loop(0, FT - 1, body, 0)
        w = src[(FT - 1) * L:FF, :]
        w = jnp.concatenate([w, jnp.zeros((L - F_TAIL, M), BF16)], axis=0)
        dst32[FT - 1] = pltpu.bitcast(w.T, U32)

    def make_cols(src, dst32, r0, rows):
        for nt in range(MT):
            dst32[nt, r0 // 2:(r0 + rows) // 2, :] = pltpu.bitcast(
                src[r0:r0 + rows, nt * L:(nt + 1) * L], U32)

    sub = jax.lax.broadcasted_iota(jnp.int32, (R, L), 0)

    def link(a, dep):
        if dep is None:
            return a
        z = pltpu.bitcast(dep, U32) & zero_v[0]
        return pltpu.bitcast(pltpu.bitcast(a, U32) | z, a.dtype)

    def make_xb(x):
        xb = x.astype(BF16)
        for t in range(MT):
            w = _col_bcast(xb[0:1, t * L:(t + 1) * L])
            XE[t * L // 2:(t + 1) * L // 2, :] = _lo(w)
            XO[t * L // 2:(t + 1) * L // 2, :] = _hi(w)

    zero_v = [None]

    def attention(x, first):
        mu, rstd = _stats(x)
        lhs = _lhs16(x)
        qscale = rstd * (D ** -0.5)
        if first:
            c_wq.wait()
            swap_heads(wq_l32, WQ32, M)
            c_wuk.wait()
            make_wukt()
        qa = [[None] * CT for _ in range(H // R)]
        qh = [None] * H

        def q_head(h):
            oq = _dot(lhs, _ld(WQ32, h))
            if first and h >= H - VQ_HEADS:
                CSQ[h] = oq[R:]
            qh[h] = ((oq[:R] - mu * oq[R:]) * qscale).astype(BF16)

        def qabs_head(h):
            g, i = divmod(h, R)
            for ct in range(CT):
                t = _dot(qh[h], _ld(WUKT32, (h, slice(ct * L // 2, (ct + 1) * L // 2))))
                qa[g][ct] = t if i == 0 else jnp.where(sub == i, t, qa[g][ct])

        if first or VQ_HEADS == 0:
            _skewed(H, SKEW_Q, q_head, qabs_head)
        else:
            make_xb(x)
            na = H - VQ_HEADS
            lhs_t = [lhs[:, t * L:(t + 1) * L] for t in range(MT)]
            oq = {}

            def q_tile(h, t):
                def f(dep):
                    p = _dot(link(lhs_t[t], dep),
                             _ld(WQ32, (h, slice(t * L // 2, (t + 1) * L // 2))))
                    oq[h] = p if t == 0 else oq[h] + p
                    if t == MT - 1:
                        o = oq[h]
                        qh[h] = ((o[:R] - mu * o[R:]) * qscale).astype(BF16)
                    return p[:R]
                return f

            def qabs_tile(h, ct):
                def f(dep):
                    g, i = divmod(h, R)
                    t = _dot(qh[h], _ld(WUKT32, (h, slice(ct * L // 2, (ct + 1) * L // 2))))
                    qa[g][ct] = t if i == 0 else jnp.where(sub == i, t, qa[g][ct])
                    return t
                f.ready = lambda: qh[h] is not None
                return f

            ms = []
            for step in range(na + SKEW_Q):
                if step < na:
                    ms += [q_tile(step, t) for t in range(MT)]
                if step >= SKEW_Q:
                    ms += [qabs_tile(step - SKEW_Q, ct) for ct in range(CT)]
            for h in range(na, H):
                ms += [qabs_tile(h, ct) for ct in range(CT)]

            acc = {}

            def v_step(hs, s):
                def f(dep):
                    xe = link(XE[s * R:(s + 1) * R, :], dep)
                    xo = XO[s * R:(s + 1) * R, :]
                    for h in hs:
                        w = WQ32[h, s * R:(s + 1) * R, :]
                        t = _lo(w) * xe + _hi(w) * xo
                        acc[h] = t if s == 0 else acc[h] + t
                    if s == M // 16 - 1:
                        for h in hs:
                            t = _sublane_sum(acc[h])
                            qh[h] = ((t - mu * CSQ[h]) * qscale).astype(BF16)
                    return acc[hs[0]]
                return f

            vs = [v_step(list(range(h0, min(H, h0 + VQ_GROUP))), s)
                  for h0 in range(na, H, VQ_GROUP) for s in range(M // 16)]
            _cosched(ms, vs, P1_CFG)
        qabs = jnp.concatenate(
            [jnp.concatenate(row, axis=1) for row in qa], axis=0).astype(BF16)

        if first:
            for c in c_ckv:
                c.wait()
            make_ckt()
        nch = KT // KCHUNK
        ms, ls, lats, ps = [None] * nch, [None] * nch, [None] * nch, [None] * nch

        def scores_chunk(j):
            s = [_dot(qabs, _ld(CKT32, kt))
                 for kt in range(j * KCHUNK, (j + 1) * KCHUNK)]
            mx = s[0]
            for t in s[1:]:
                mx = jnp.maximum(mx, t)
            mx = jnp.max(mx, axis=-1, keepdims=True)
            e = [jnp.exp(t - mx) for t in s]
            lsum = e[0]
            for t in e[1:]:
                lsum = lsum + t
            ps[j] = jnp.concatenate(e, axis=1).astype(BF16)
            ms[j] = mx
            ls[j] = lsum

        def lat_chunk(j):
            k0 = j * KCHUNK * L // 2
            lats[j] = [_dot(ps[j], _ld(CKV32, (ct, slice(k0, k0 + KCHUNK * L // 2))))
                       for ct in range(CT)]

        _skewed(nch, SKEW_S, scores_chunk, lat_chunk)
        m = ms[0]
        for t in ms[1:]:
            m = jnp.maximum(m, t)
        alpha = [jnp.exp(t - m) for t in ms]
        lsum = alpha[0] * ls[0]
        for a, t in zip(alpha[1:], ls[1:]):
            lsum = lsum + a * t
        inv = 1.0 / jnp.sum(lsum, axis=-1, keepdims=True)
        lat = []
        for ct in range(CT):
            t = alpha[0] * lats[0][ct]
            for j in range(1, len(lats)):
                t = t + alpha[j] * lats[j][ct]
            lat.append(t * inv)
        lat = jnp.concatenate(lat, axis=1)
        latg = [lat[g * R:(g + 1) * R].astype(BF16) for g in range(H // R)]

        if first:
            c_wuv.wait()
            swap_heads(wuv_l32, WUV32, DC)

        def ctx_head(h):
            g, i = divmod(h, R)
            c = _dot(latg[g], _ld(WUV32, h))
            return jnp.broadcast_to(c[i:i + 1], (R, D)).astype(BF16)

        def out_head(h, cb, o):
            for nt in range(MT):
                t = _dot(cb, _ld(WO32, (nt, slice(h * L // 2, (h + 1) * L // 2))))
                o[nt] = t if o[nt] is None else o[nt] + t

        o = [None] * MT
        if first:
            cbs = [ctx_head(h) for h in range(H)]
            c_wg.wait()
            make_wgu(wg_l, WG32)
            c_wu.wait()
            make_wgu(wu_l, WU32)
            hpc = H // WO_CHUNKS
            for c in range(WO_CHUNKS):
                c_wo[c].wait()
                make_cols(wo_l, WO32, c * wo_rows, wo_rows)
                for h in range(c * hpc, (c + 1) * hpc):
                    out_head(h, cbs[h], o)
        else:
            cbs = [None] * H

            def ctx_stage(h):
                cbs[h] = ctx_head(h)

            _skewed(H, SKEW_O, ctx_stage, lambda h: out_head(h, cbs[h], o))
        return _round_bf16(x + jnp.concatenate(o, axis=1))

    def ffn(x, first):
        mu, rstd = _stats(x)
        lhs = _lhs16(x)
        xn = (x - mu) * rstd
        r = jnp.sum(xn * wr_v[...].reshape(1, M).astype(F32), axis=-1, keepdims=True)
        gate = jax.nn.sigmoid(r)

        def act_tile(ft):
            og = _dot(lhs, _ld(WG32, ft))
            ou = _dot(lhs, _ld(WU32, ft))
            g = (og[:R] - mu * og[R:]) * rstd
            u = (ou[:R] - mu * ou[R:]) * rstd
            return (g * jax.nn.sigmoid(g) * u).astype(BF16)

        def down_tile(ft, a, y):
            for nt in range(MT):
                if first:
                    r0 = ft * L
                    if ft < FT - 1:
                        t = _dot(a, wd_l[r0:r0 + L, nt * L:(nt + 1) * L])
                    else:
                        t = _dot(a[:, :F_TAIL], wd_l[r0:FF, nt * L:(nt + 1) * L])
                else:
                    r0 = ft * L // 2
                    if ft < FT - 1:
                        t = _dot(a, _ld(WD32, (nt, slice(r0, r0 + L // 2))))
                    else:
                        t = _dot(a[:, :F_TAIL], _ld(WD32, (nt, slice(r0, FF // 2))))
                y[nt] = t if y[nt] is None else y[nt] + t

        y = [None] * MT
        if first:
            acts = [act_tile(ft) for ft in range(FT)]
            for c, (f0, f1) in enumerate(WD_CHUNKS):
                c_wd[c].wait()
                for ft in range(f0, f1):
                    down_tile(ft, acts[ft], y)
        else:
            acts = [None] * FT

            def act_stage(ft):
                acts[ft] = act_tile(ft)

            _skewed(FT, SKEW_F, act_stage, lambda ft: down_tile(ft, acts[ft], y))
        return _round_bf16(x + xn + jnp.concatenate(y, axis=1) * gate)

    c_x.wait()
    c_x2.wait()
    c_wr.wait()
    x = jnp.broadcast_to(x_v[...].astype(F32), (R, M))
    xc = jnp.broadcast_to(x_v2[...].astype(F32), (R, M))
    zero_v[0] = pltpu.bitcast(x[:, :L], U32) ^ pltpu.bitcast(xc[:, :L], U32)
    x = attention(x, True)
    x = ffn(x, True)
    if N_LAYERS > 1:
        make_cols(wd_l, WD32, 0, FF)
        x = attention(x, False)
        x = ffn(x, False)
    o_ref[...] = x[0:1].astype(o_ref.dtype)


@jax.jit
def pallas_interleave_layers__compressed_kv_cla__moe_arch_mod__decode_kernel(
    A_x: jax.Array,
    A_c_kv: jax.Array,
    A_w_q: jax.Array,
    A_w_uk: jax.Array,
    A_w_uv: jax.Array,
    A_w_o: jax.Array,
    B_x: jax.Array,
    B_w_r: jax.Array,
    B_w_gate: jax.Array,
    B_w_up: jax.Array,
    B_w_down: jax.Array,
):
    del B_x
    args = (
        A_x.reshape(1, M),
        B_w_r,
        A_w_q,
        A_w_uk,
        A_c_kv.reshape(SK, DC),
        A_w_uv,
        B_w_gate.T,
        B_w_up.T,
        A_w_o.reshape(H * D, M),
        B_w_down,
    )
    scratch = [
        pltpu.VMEM((1, M), BF16),
        pltpu.VMEM((1, M), BF16),
        pltpu.VMEM((M,), BF16),
        pltpu.VMEM((M, H, D), BF16),
        pltpu.VMEM((DC, H, D), BF16),
        pltpu.VMEM((DC, H, D), BF16),
        pltpu.VMEM((FF, M), BF16),
        pltpu.VMEM((FF, M), BF16),
        pltpu.VMEM((H * D, M), BF16),
        pltpu.VMEM((FF, M), BF16),
        pltpu.VMEM((H, M, D), BF16),
        pltpu.VMEM((H, DC, L), BF16),
        pltpu.VMEM((CT, SK, L), BF16),
        pltpu.VMEM((KT, DC, L), BF16),
        pltpu.VMEM((H, DC, D), BF16),
        pltpu.VMEM((FT, M, L), BF16),
        pltpu.VMEM((FT, M, L), BF16),
        pltpu.VMEM((MT, H * D, L), BF16),
        pltpu.VMEM((MT, FF, L), BF16),
        pltpu.VMEM((H, R, L), F32),
        pltpu.VMEM((M // 2, L), F32),
        pltpu.VMEM((M // 2, L), F32),
        pltpu.SemaphoreType.DMA((20,)),
    ]
    out = pl.pallas_call(
        _kernel,
        out_shape=jax.ShapeDtypeStruct((1, M), A_x.dtype),
        in_specs=[pl.BlockSpec(memory_space=pl.ANY)] * len(args),
        out_specs=pl.BlockSpec(memory_space=pltpu.VMEM),
        scratch_shapes=scratch,
        compiler_params=pltpu.CompilerParams(
            vmem_limit_bytes=100 * 1024 * 1024),
        name="mla_moe_decode",
    )(*args)
    return out.reshape(1, 1, M)
```

```python
import jax
import jax.numpy as jnp
import jax.experimental.pallas as pl
import jax.experimental.pallas.tpu as pltpu

F32 = jnp.float32
BF16 = jnp.bfloat16
U32 = jnp.uint32

H = 32
D = 128
M = 640
DC = 512
SK = 4096
FF = 1728
EPS = 1e-5
R = 8
L = 128

MT = M // L
CT = DC // L
KT = SK // L
FT = -(-FF // L)
F_TAIL = FF - (FT - 1) * L
KCHUNK = 8
WO_CHUNKS = 4
WD_CHUNKS = ((0, 6), (6, 11), (11, FT))


N_LAYERS = 2
SMALL_FIRST = False
SKEW_Q = 8
SKEW_S = 1
SKEW_O = 6
SKEW_F = 5


def _skewed(n, skew, produce, consume):
    for step in range(n + skew):
        if step < n:
            produce(step)
        if step >= skew:
            consume(step - skew)


VQ_HEADS = 16
VQ_GROUP = 4
P1_CFG = (30, 1.0, 2, 18, 1)
VO_HEADS = 16
P3_CFG = (30, 0.9, 2, 18, 1)
XLU_AHEAD = 2
VF_TILES = 4
VF_GROUP = 2
P4_CFG = (20, 0.8, 2, 18, 1)


def _cosched(ms, vs, cfg):
    vstart, vrate, lag_v, lag_m, nlink = cfg
    mres, vres = [], []
    j = 0

    def emit_v(dep):
        nonlocal j
        vres.append(vs[j](dep))
        j += 1

    for i, m in enumerate(ms):
        while not getattr(m, "ready", lambda: True)():
            emit_v(None)
        dep = None
        if len(vres) > lag_v and i % nlink == 0 and j < len(vs):
            dep = vres[-1 - lag_v]
        mres.append(m(dep))
        while (j < len(vs) and j < (i + 1 - vstart) * vrate
               and getattr(vs[j], "ready", lambda: True)()):
            emit_v(mres[-1 - lag_m] if (len(mres) > lag_m and j % 2 == 0) else None)
    while j < len(vs):
        emit_v(None)


def _lo(w):
    return pltpu.bitcast(w << 16, F32)


def _hi(w):
    return pltpu.bitcast(w & jnp.uint32(0xFFFF0000), F32)


def _sublane_sum(t):
    t = t + pltpu.roll(t, 4, 0)
    t = t + pltpu.roll(t, 2, 0)
    return t + pltpu.roll(t, 1, 0)


def _col_bcast(row):
    return pltpu.bitcast(jnp.broadcast_to(row, (L, L)).T, U32)


def _dot(a, b):
    return jnp.dot(a, b, preferred_element_type=F32)


def _ld(ref32, idx):
    return pltpu.bitcast(ref32[idx], BF16)


def _st(ref32, idx, val):
    ref32[idx] = pltpu.bitcast(val, U32)


def _round_bf16(x):
    return x.astype(BF16).astype(F32)


def _stats(x):
    mu = jnp.mean(x, axis=-1, keepdims=True)
    xc = x - mu
    var = jnp.mean(xc * xc, axis=-1, keepdims=True)
    return mu, jax.lax.rsqrt(var + EPS)


def _lhs16(x):
    return jnp.concatenate([x, jnp.ones_like(x)], axis=0).astype(BF16)


def _kernel(x_hbm, wr_hbm, wq_hbm, wuk_hbm, ckv_hbm, wuv_hbm, wg_hbm, wu_hbm,
            wo_hbm, wd_hbm,
            o_ref,
            x_v, x_v2, wr_v, wq_l, wuk_l, wuv_l, wg_l, wu_l, wo_l, wd_l,
            WQ, WUKT, CKV, CKT, WUV, WG, WU, WO, WD,
            CSQ, CSG, CSU, XE, XO, sems):
    sem_ids = iter(range(64))

    def copy(src, dst):
        c = pltpu.make_async_copy(src, dst, sems.at[next(sem_ids)])
        c.start()
        return c

    if SMALL_FIRST:
        c_x = copy(x_hbm, x_v)
        c_wr = copy(wr_hbm, wr_v)
        c_wq = copy(wq_hbm, wq_l)
    else:
        c_wq = copy(wq_hbm, wq_l)
        c_x = copy(x_hbm, x_v)
        c_wr = copy(wr_hbm, wr_v)
    c_x2 = copy(x_hbm, x_v2)
    c_wuk = copy(wuk_hbm, wuk_l)
    c_ckv = [copy(ckv_hbm.at[:, pl.ds(ct * L, L)], CKV.at[ct]) for ct in range(CT)]
    c_wuv = copy(wuv_hbm, wuv_l)
    c_wg = copy(wg_hbm, wg_l)
    c_wu = copy(wu_hbm, wu_l)
    wo_rows = H * D // WO_CHUNKS
    c_wo = [copy(wo_hbm.at[pl.ds(c * wo_rows, wo_rows)],
                 wo_l.at[pl.ds(c * wo_rows, wo_rows)]) for c in range(WO_CHUNKS)]
    c_wd = []
    for (f0, f1) in WD_CHUNKS:
        r0, r1 = f0 * L, min(f1 * L, FF)
        c_wd.append(copy(wd_hbm.at[pl.ds(r0, r1 - r0)], wd_l.at[pl.ds(r0, r1 - r0)]))

    wq_l32, wuk_l32, wuv_l32 = (r.bitcast(U32) for r in (wq_l, wuk_l, wuv_l))
    WQ32, WUKT32, CKV32, CKT32, WUV32, WG32, WU32, WO32, WD32 = (
        r.bitcast(U32) for r in (WQ, WUKT, CKV, CKT, WUV, WG, WU, WO, WD))

    def swap_heads(src32, dst32, rows):
        ch = 64

        def body(i, carry):
            r0 = pl.multiple_of(i * ch, ch)
            w = _ld(src32, pl.ds(r0, ch))
            dst32[:, pl.ds(pl.multiple_of(i * (ch // 2), ch // 2), ch // 2), :] = (
                pltpu.bitcast(jnp.swapaxes(w, 0, 1), U32))
            return carry
        jax.lax.fori_loop(0, rows // ch, body, 0)

    def make_wukt():
        def body(i, carry):
            w = _ld(wuk_l32, pl.ds(pl.multiple_of(i * L, L), L))
            w = jnp.swapaxes(jnp.swapaxes(w, 0, 1), 1, 2)
            WUKT32[:, pl.ds(pl.multiple_of(i * (L // 2), L // 2), L // 2), :] = (
                pltpu.bitcast(w, U32))
            return carry
        jax.lax.fori_loop(0, CT, body, 0)

    def make_ckt():
        def body(kt, carry):
            for ct in range(CT):
                w = _ld(CKV32, (ct, pl.ds(pl.multiple_of(kt * (L // 2), L // 2), L // 2)))
                CKT32[kt, ct * (L // 2):(ct + 1) * (L // 2), :] = pltpu.bitcast(w.T, U32)
            return carry
        jax.lax.fori_loop(0, KT, body, 0)

    def make_wgu(src, dst32):
        def body(ft, carry):
            w = src[pl.ds(pl.multiple_of(ft * L, L), L), :]
            dst32[ft] = pltpu.bitcast(w.T, U32)
            return carry
        jax.lax.fori_loop(0, FT - 1, body, 0)
        w = src[(FT - 1) * L:FF, :]
        w = jnp.concatenate([w, jnp.zeros((L - F_TAIL, M), BF16)], axis=0)
        dst32[FT - 1] = pltpu.bitcast(w.T, U32)

    def make_cols(src, dst32, r0, rows):
        for nt in range(MT):
            dst32[nt, r0 // 2:(r0 + rows) // 2, :] = pltpu.bitcast(
                src[r0:r0 + rows, nt * L:(nt + 1) * L], U32)

    sub = jax.lax.broadcasted_iota(jnp.int32, (R, L), 0)

    def link(a, dep):
        if dep is None:
            return a
        z = pltpu.bitcast(dep, U32) & zero_v[0]
        a32 = pltpu.bitcast(a, U32)
        return pltpu.bitcast(a32 | z[:a32.shape[0]], a.dtype)

    def make_xb(x):
        xb = x.astype(BF16)
        for t in range(MT):
            w = _col_bcast(xb[0:1, t * L:(t + 1) * L])
            XE[t * L // 2:(t + 1) * L // 2, :] = _lo(w)
            XO[t * L // 2:(t + 1) * L // 2, :] = _hi(w)

    zero_v = [None]

    def attention(x, first):
        mu, rstd = _stats(x)
        lhs = _lhs16(x)
        qscale = rstd * (D ** -0.5)
        if first:
            c_wq.wait()
            swap_heads(wq_l32, WQ32, M)
            c_wuk.wait()
            make_wukt()
        qa = [[None] * CT for _ in range(H // R)]
        qh = [None] * H

        def q_head(h):
            oq = _dot(lhs, _ld(WQ32, h))
            if first and h >= H - VQ_HEADS:
                CSQ[h] = oq[R:]
            qh[h] = ((oq[:R] - mu * oq[R:]) * qscale).astype(BF16)

        def qabs_head(h):
            g, i = divmod(h, R)
            for ct in range(CT):
                t = _dot(qh[h], _ld(WUKT32, (h, slice(ct * L // 2, (ct + 1) * L // 2))))
                qa[g][ct] = t if i == 0 else jnp.where(sub == i, t, qa[g][ct])

        if first or VQ_HEADS == 0:
            _skewed(H, SKEW_Q, q_head, qabs_head)
        else:
            make_xb(x)
            na = H - VQ_HEADS
            lhs_t = [lhs[:, t * L:(t + 1) * L] for t in range(MT)]
            oq = {}

            def q_tile(h, t):
                def f(dep):
                    p = _dot(link(lhs_t[t], dep),
                             _ld(WQ32, (h, slice(t * L // 2, (t + 1) * L // 2))))
                    oq[h] = p if t == 0 else oq[h] + p
                    if t == MT - 1:
                        o = oq[h]
                        qh[h] = ((o[:R] - mu * o[R:]) * qscale).astype(BF16)
                    return p[:R]
                return f

            def qabs_tile(h, ct):
                def f(dep):
                    g, i = divmod(h, R)
                    t = _dot(qh[h], _ld(WUKT32, (h, slice(ct * L // 2, (ct + 1) * L // 2))))
                    qa[g][ct] = t if i == 0 else jnp.where(sub == i, t, qa[g][ct])
                    return t
                f.ready = lambda: qh[h] is not None
                return f

            ms = []
            for step in range(na + SKEW_Q):
                if step < na:
                    ms += [q_tile(step, t) for t in range(MT)]
                if step >= SKEW_Q:
                    ms += [qabs_tile(step - SKEW_Q, ct) for ct in range(CT)]
            for h in range(na, H):
                ms += [qabs_tile(h, ct) for ct in range(CT)]

            acc = {}

            def v_step(hs, s):
                def f(dep):
                    xe = link(XE[s * R:(s + 1) * R, :], dep)
                    xo = XO[s * R:(s + 1) * R, :]
                    for h in hs:
                        w = WQ32[h, s * R:(s + 1) * R, :]
                        t = _lo(w) * xe + _hi(w) * xo
                        acc[h] = t if s == 0 else acc[h] + t
                    if s == M // 16 - 1:
                        for h in hs:
                            t = _sublane_sum(acc[h])
                            qh[h] = ((t - mu * CSQ[h]) * qscale).astype(BF16)
                    return acc[hs[0]]
                return f

            vs = [v_step(list(range(h0, min(H, h0 + VQ_GROUP))), s)
                  for h0 in range(na, H, VQ_GROUP) for s in range(M // 16)]
            _cosched(ms, vs, P1_CFG)
        qabs = jnp.concatenate(
            [jnp.concatenate(row, axis=1) for row in qa], axis=0).astype(BF16)

        if first:
            for c in c_ckv:
                c.wait()
            make_ckt()
        nch = KT // KCHUNK
        ms, ls, lats, ps = [None] * nch, [None] * nch, [None] * nch, [None] * nch

        def scores_chunk(j):
            s = [_dot(qabs, _ld(CKT32, kt))
                 for kt in range(j * KCHUNK, (j + 1) * KCHUNK)]
            mx = s[0]
            for t in s[1:]:
                mx = jnp.maximum(mx, t)
            mx = jnp.max(mx, axis=-1, keepdims=True)
            e = [jnp.exp(t - mx) for t in s]
            lsum = e[0]
            for t in e[1:]:
                lsum = lsum + t
            ps[j] = jnp.concatenate(e, axis=1).astype(BF16)
            ms[j] = mx
            ls[j] = lsum

        def lat_chunk(j):
            k0 = j * KCHUNK * L // 2
            lats[j] = [_dot(ps[j], _ld(CKV32, (ct, slice(k0, k0 + KCHUNK * L // 2))))
                       for ct in range(CT)]

        _skewed(nch, SKEW_S, scores_chunk, lat_chunk)
        m = ms[0]
        for t in ms[1:]:
            m = jnp.maximum(m, t)
        alpha = [jnp.exp(t - m) for t in ms]
        lsum = alpha[0] * ls[0]
        for a, t in zip(alpha[1:], ls[1:]):
            lsum = lsum + a * t
        inv = 1.0 / jnp.sum(lsum, axis=-1, keepdims=True)
        lat = []
        for ct in range(CT):
            t = alpha[0] * lats[0][ct]
            for j in range(1, len(lats)):
                t = t + alpha[j] * lats[j][ct]
            lat.append(t * inv)
        lat = jnp.concatenate(lat, axis=1)
        latg = [lat[g * R:(g + 1) * R].astype(BF16) for g in range(H // R)]

        if first:
            c_wuv.wait()
            swap_heads(wuv_l32, WUV32, DC)

        def ctx_head(h):
            g, i = divmod(h, R)
            c = _dot(latg[g], _ld(WUV32, h))
            return jnp.broadcast_to(c[i:i + 1], (R, D)).astype(BF16)

        def out_head(h, cb, o):
            for nt in range(MT):
                t = _dot(cb, _ld(WO32, (nt, slice(h * L // 2, (h + 1) * L // 2))))
                o[nt] = t if o[nt] is None else o[nt] + t

        o = [None] * MT
        if first:
            cbs = [ctx_head(h) for h in range(H)]
            c_wg.wait()
            make_wgu(wg_l, WG32)
            c_wu.wait()
            make_wgu(wu_l, WU32)
            hpc = H // WO_CHUNKS
            for c in range(WO_CHUNKS):
                c_wo[c].wait()
                make_cols(wo_l, WO32, c * wo_rows, wo_rows)
                for h in range(c * hpc, (c + 1) * hpc):
                    out_head(h, cbs[h], o)
        else:
            cbs = [None] * H
            if VO_HEADS == 0:
                def ctx_stage(h):
                    cbs[h] = ctx_head(h)

                _skewed(H, SKEW_O, ctx_stage, lambda h: out_head(h, cbs[h], o))
            else:
                cacc = {}

                def ctx_tile(h, ct):
                    def f(dep):
                        g, i = divmod(h, R)
                        p = _dot(link(latg_t[g][ct], dep),
                                 _ld(WUV32, (h, slice(ct * L // 2, (ct + 1) * L // 2))))
                        cacc[h] = p if ct == 0 else cacc[h] + p
                        if ct == CT - 1:
                            cbs[h] = jnp.broadcast_to(
                                cacc[h][i:i + 1], (R, D)).astype(BF16)
                        return p
                    return f

                def out_tile(h, nt):
                    def f(dep):
                        t = _dot(cbs[h], _ld(WO32, (nt, slice(h * L // 2, (h + 1) * L // 2))))
                        o[nt] = t if o[nt] is None else o[nt] + t
                        return t
                    return f

                latg_t = [[t[:, ct * L:(ct + 1) * L] for ct in range(CT)] for t in latg]
                ms = []
                for h in range(VO_HEADS):
                    ms += [ctx_tile(h, ct) for ct in range(CT)]
                nm = H - VO_HEADS
                for step in range(nm + SKEW_O):
                    if step < nm:
                        ms += [ctx_tile(VO_HEADS + step, ct) for ct in range(CT)]
                    if step >= SKEW_O:
                        ms += [out_tile(VO_HEADS + step - SKEW_O, nt) for nt in range(MT)]

                cw = {}
                ov = [None] * MT

                def xlu_op(h):
                    def f(dep):
                        cw[h] = _col_bcast(cbs[h][0:1])
                        return pltpu.bitcast(cw[h][:R], F32)
                    f.ready = lambda: cbs[h] is not None
                    return f

                def v_step(h, k):
                    def f(dep):
                        w = cw[h][k * R:(k + 1) * R]
                        ce, co = link(_lo(w), dep), _hi(w)
                        r0 = h * L // 2 + k * R
                        for nt in range(MT):
                            w = WO32[nt, r0:r0 + R, :]
                            t = _lo(w) * ce + _hi(w) * co
                            ov[nt] = t if ov[nt] is None else ov[nt] + t
                        return ov[0]
                    return f

                vs = [xlu_op(h) for h in range(min(XLU_AHEAD, VO_HEADS))]
                for h in range(VO_HEADS):
                    if h + XLU_AHEAD < VO_HEADS:
                        vs.append(xlu_op(h + XLU_AHEAD))
                    vs += [v_step(h, k) for k in range(L // 16)]
                _cosched(ms, vs, P3_CFG)
                o = [a + _sublane_sum(b) for a, b in zip(o, ov)]
        return _round_bf16(x + jnp.concatenate(o, axis=1))

    def ffn(x, first):
        mu, rstd = _stats(x)
        lhs = _lhs16(x)
        xn = (x - mu) * rstd
        r = jnp.sum(xn * wr_v[...].reshape(1, M).astype(F32), axis=-1, keepdims=True)
        gate = jax.nn.sigmoid(r)

        def act_tile(ft):
            og = _dot(lhs, _ld(WG32, ft))
            ou = _dot(lhs, _ld(WU32, ft))
            if first and ft < VF_TILES:
                CSG[ft] = og[R:]
                CSU[ft] = ou[R:]
            g = (og[:R] - mu * og[R:]) * rstd
            u = (ou[:R] - mu * ou[R:]) * rstd
            return (g * jax.nn.sigmoid(g) * u).astype(BF16)

        def down_tile(ft, a, y):
            for nt in range(MT):
                if first:
                    r0 = ft * L
                    if ft < FT - 1:
                        t = _dot(a, wd_l[r0:r0 + L, nt * L:(nt + 1) * L])
                    else:
                        t = _dot(a[:, :F_TAIL], wd_l[r0:FF, nt * L:(nt + 1) * L])
                else:
                    r0 = ft * L // 2
                    if ft < FT - 1:
                        t = _dot(a, _ld(WD32, (nt, slice(r0, r0 + L // 2))))
                    else:
                        t = _dot(a[:, :F_TAIL], _ld(WD32, (nt, slice(r0, FF // 2))))
                y[nt] = t if y[nt] is None else y[nt] + t

        y = [None] * MT
        if first:
            acts = [act_tile(ft) for ft in range(FT)]
            for c, (f0, f1) in enumerate(WD_CHUNKS):
                c_wd[c].wait()
                for ft in range(f0, f1):
                    down_tile(ft, acts[ft], y)
        else:
            acts = [None] * FT
            if VF_TILES == 0:
                def act_stage(ft):
                    acts[ft] = act_tile(ft)

                _skewed(FT, SKEW_F, act_stage, lambda ft: down_tile(ft, acts[ft], y))
            else:
                make_xb(x)
                lhs_t = [lhs[:, t * L:(t + 1) * L] for t in range(MT)]
                pre = {}

                def finish(ft):
                    g, u = pre[ft, 0] * rstd, pre[ft, 1] * rstd
                    acts[ft] = (g * jax.nn.sigmoid(g) * u).astype(BF16)

                def gu_tile(ft, which, t):
                    def f(dep):
                        w32 = (WG32, WU32)[which]
                        p = _dot(link(lhs_t[t], dep),
                                 _ld(w32, (ft, slice(t * L // 2, (t + 1) * L // 2))))
                        k = (ft, which)
                        pre[k] = p if t == 0 else pre[k] + p
                        if t == MT - 1:
                            pre[k] = pre[k][:R] - mu * pre[k][R:]
                            if which == 1:
                                finish(ft)
                        return p[:R]
                    return f

                def dn_tile(ft, nt):
                    def f(dep):
                        r0 = ft * L // 2
                        if ft < FT - 1:
                            t = _dot(acts[ft], _ld(WD32, (nt, slice(r0, r0 + L // 2))))
                        else:
                            t = _dot(acts[ft][:, :F_TAIL], _ld(WD32, (nt, slice(r0, FF // 2))))
                        y[nt] = t if y[nt] is None else y[nt] + t
                        return t
                    f.ready = lambda: acts[ft] is not None
                    return f

                mt = list(range(VF_TILES, FT))
                ms = []
                for step in range(len(mt) + SKEW_F):
                    if step < len(mt):
                        ms += [gu_tile(mt[step], wh, t) for wh in range(2) for t in range(MT)]
                    if step >= SKEW_F:
                        ms += [dn_tile(mt[step - SKEW_F], nt) for nt in range(MT)]
                for ft in range(VF_TILES):
                    ms += [dn_tile(ft, nt) for nt in range(MT)]

                acc = {}

                def v_step(fts, s):
                    def f(dep):
                        xe = link(XE[s * R:(s + 1) * R, :], dep)
                        xo = XO[s * R:(s + 1) * R, :]
                        for ft in fts:
                            for wh, w32 in enumerate((WG32, WU32)):
                                w = w32[ft, s * R:(s + 1) * R, :]
                                t = _lo(w) * xe + _hi(w) * xo
                                acc[ft, wh] = t if s == 0 else acc[ft, wh] + t
                        if s == M // 16 - 1:
                            for ft in fts:
                                for wh, cs in enumerate((CSG, CSU)):
                                    pre[ft, wh] = _sublane_sum(acc[ft, wh]) - mu * cs[ft]
                                finish(ft)
                        return acc[fts[0], 0]
                    return f

                vs = [v_step(list(range(f0, min(VF_TILES, f0 + VF_GROUP))), s)
                      for f0 in range(0, VF_TILES, VF_GROUP) for s in range(M // 16)]
                _cosched(ms, vs, P4_CFG)
        return _round_bf16(x + xn + jnp.concatenate(y, axis=1) * gate)

    c_x.wait()
    c_x2.wait()
    c_wr.wait()
    x = jnp.broadcast_to(x_v[...].astype(F32), (R, M))
    xc = jnp.broadcast_to(x_v2[...].astype(F32), (R, M))
    zero_v[0] = pltpu.bitcast(x[:, :L], U32) ^ pltpu.bitcast(xc[:, :L], U32)
    x = attention(x, True)
    x = ffn(x, True)
    if N_LAYERS > 1:
        make_cols(wd_l, WD32, 0, FF)
        x = attention(x, False)
        x = ffn(x, False)
    o_ref[...] = x[0:1].astype(o_ref.dtype)


@jax.jit
def pallas_interleave_layers__compressed_kv_cla__moe_arch_mod__decode_kernel(
    A_x: jax.Array,
    A_c_kv: jax.Array,
    A_w_q: jax.Array,
    A_w_uk: jax.Array,
    A_w_uv: jax.Array,
    A_w_o: jax.Array,
    B_x: jax.Array,
    B_w_r: jax.Array,
    B_w_gate: jax.Array,
    B_w_up: jax.Array,
    B_w_down: jax.Array,
):
    del B_x
    args = (
        A_x.reshape(1, M),
        B_w_r,
        A_w_q,
        A_w_uk,
        A_c_kv.reshape(SK, DC),
        A_w_uv,
        B_w_gate.T,
        B_w_up.T,
        A_w_o.reshape(H * D, M),
        B_w_down,
    )
    scratch = [
        pltpu.VMEM((1, M), BF16),
        pltpu.VMEM((1, M), BF16),
        pltpu.VMEM((M,), BF16),
        pltpu.VMEM((M, H, D), BF16),
        pltpu.VMEM((DC, H, D), BF16),
        pltpu.VMEM((DC, H, D), BF16),
        pltpu.VMEM((FF, M), BF16),
        pltpu.VMEM((FF, M), BF16),
        pltpu.VMEM((H * D, M), BF16),
        pltpu.VMEM((FF, M), BF16),
        pltpu.VMEM((H, M, D), BF16),
        pltpu.VMEM((H, DC, L), BF16),
        pltpu.VMEM((CT, SK, L), BF16),
        pltpu.VMEM((KT, DC, L), BF16),
        pltpu.VMEM((H, DC, D), BF16),
        pltpu.VMEM((FT, M, L), BF16),
        pltpu.VMEM((FT, M, L), BF16),
        pltpu.VMEM((MT, H * D, L), BF16),
        pltpu.VMEM((MT, FF, L), BF16),
        pltpu.VMEM((H, R, L), F32),
        pltpu.VMEM((FT, R, L), F32),
        pltpu.VMEM((FT, R, L), F32),
        pltpu.VMEM((M // 2, L), F32),
        pltpu.VMEM((M // 2, L), F32),
        pltpu.SemaphoreType.DMA((20,)),
    ]
    out = pl.pallas_call(
        _kernel,
        out_shape=jax.ShapeDtypeStruct((1, M), A_x.dtype),
        in_specs=[pl.BlockSpec(memory_space=pl.ANY)] * len(args),
        out_specs=pl.BlockSpec(memory_space=pltpu.VMEM),
        scratch_shapes=scratch,
        compiler_params=pltpu.CompilerParams(
            vmem_limit_bytes=100 * 1024 * 1024),
        name="mla_moe_decode",
    )(*args)
    return out.reshape(1, 1, M)
```

```python
import jax
import jax.numpy as jnp
import jax.experimental.pallas as pl
import jax.experimental.pallas.tpu as pltpu

F32 = jnp.float32
BF16 = jnp.bfloat16
U32 = jnp.uint32

H = 32
D = 128
M = 640
DC = 512
SK = 4096
FF = 1728
EPS = 1e-5
R = 8
L = 128
W2 = L // 2

MT = M // L
CT = DC // L
KT = SK // L
FT = -(-FF // L)
F_TAIL = FF - (FT - 1) * L
KCHUNK = 8
WO_CHUNKS = 4
WD_CHUNKS = ((0, 7), (7, 12), (12, FT))

N_LAYERS = 2
SKEW_Q = 8
SKEW_S = 1
SKEW_O = 6
SKEW_F = 5
EDGE = 4

VQ_HEADS = 16
VQ_GROUP = 4
P1_CFG = (30, 1.0, 2, 18, 1)
VO_HEADS = 16
P3_CFG = (30, 0.9, 2, 18, 1)
XLU_AHEAD = 2
VF_TILES = 4
VF_GROUP = 2
P4_CFG = (20, 0.8, 2, 18, 1)


def _always():
    return True


def _cosched(ms, vs, cfg):
    vstart, vrate, lag_v, lag_m, nlink = cfg
    mres, vres = [], []
    j = 0

    def emit_v(dep):
        nonlocal j
        vres.append(vs[j](dep))
        j += 1

    for i, m in enumerate(ms):
        while not getattr(m, "ready", _always)():
            emit_v(None)
        dep = None
        if len(vres) > lag_v and i % nlink == 0 and j < len(vs):
            dep = vres[-1 - lag_v]
        mres.append(m(dep))
        while (j < len(vs) and j < (i + 1 - vstart) * vrate
               and getattr(vs[j], "ready", _always)()):
            emit_v(mres[-1 - lag_m] if (len(mres) > lag_m and j % 2 == 0) else None)
    while j < len(vs):
        emit_v(None)


def _skewed(n, skew, produce, consume):
    out = []
    for step in range(n + skew):
        if step < n:
            out += produce(step)
        if step >= skew:
            out += consume(step - skew)
    return out


def _by_column(items, op, ncol):
    return [op(it, c) for c in range(ncol) for it in items]


def _by_item(items, op, ncol):
    return [op(it, c) for it in items for c in range(ncol)]


def _run(ops):
    for f in ops:
        f(None)


def _dot(a, b):
    return jnp.dot(a, b, preferred_element_type=F32)


def _bf(words):
    return pltpu.bitcast(words, BF16)


def _lo(w):
    return pltpu.bitcast(w << 16, F32)


def _hi(w):
    return pltpu.bitcast(w & jnp.uint32(0xFFFF0000), F32)


def _sublane_sum(t):
    t = t + pltpu.roll(t, 4, 0)
    t = t + pltpu.roll(t, 2, 0)
    return t + pltpu.roll(t, 1, 0)


def _col_bcast(row):
    return pltpu.bitcast(jnp.broadcast_to(row, (L, L)).T, U32)


def _round_bf16(x):
    return x.astype(BF16).astype(F32)


def _stats(xt):
    x = jnp.concatenate(xt, axis=1)
    mu = jnp.mean(x, axis=-1, keepdims=True)
    xc = x - mu
    var = jnp.mean(xc * xc, axis=-1, keepdims=True)
    return mu, jax.lax.rsqrt(var + EPS)


def _lhs16(xt):
    return [jnp.concatenate([x, jnp.ones_like(x)], axis=0).astype(BF16) for x in xt]


def _acc(d, k, v):
    d[k] = v if d.get(k) is None else d[k] + v
    return d[k]


def _kernel(x_hbm, wr_hbm, wq_hbm, wuk_hbm, ckv_hbm, wuv_hbm, wg_hbm, wu_hbm,
            wo_hbm, wd_hbm,
            o_ref,
            x_v, x_v2, wr_v, wq_l, wuk_l, wuv_l, wg_l, wu_l, wo_l, wd_l,
            WQ, WUKT, CKV, CKT, WUV, WG, WU, WO, WD,
            CSQ, CSG, CSU, XE, XO, sems):
    sem_ids = iter(range(64))

    def copy(src, dst, sem=None):
        sem = next(sem_ids) if sem is None else sem
        c = pltpu.make_async_copy(src, dst, sems.at[sem])
        c.start()
        return c

    c_wq = copy(wq_hbm, wq_l)
    s_small = next(sem_ids)
    c_small = [copy(x_hbm, x_v, s_small), copy(x_hbm, x_v2, s_small),
               copy(wr_hbm, wr_v, s_small)]
    c_wuk = copy(wuk_hbm, wuk_l)
    s_ckv = next(sem_ids)
    c_ckv = [copy(ckv_hbm.at[:, pl.ds(ct * L, L)], CKV.at[ct], s_ckv) for ct in range(CT)]
    c_wuv = copy(wuv_hbm, wuv_l)
    c_wg = copy(wg_hbm, wg_l)
    c_wu = copy(wu_hbm, wu_l)
    wo_rows = H * D // WO_CHUNKS
    c_wo = [copy(wo_hbm.at[pl.ds(c * wo_rows, wo_rows)],
                 wo_l.at[pl.ds(c * wo_rows, wo_rows)]) for c in range(WO_CHUNKS)]
    c_wd = []
    for (f0, f1) in WD_CHUNKS:
        r0, r1 = f0 * L, min(f1 * L, FF)
        c_wd.append(copy(wd_hbm.at[pl.ds(r0, r1 - r0)], wd_l.at[pl.ds(r0, r1 - r0)]))

    wq_l32, wuk_l32, wuv_l32 = (r.bitcast(U32) for r in (wq_l, wuk_l, wuv_l))
    WQ32, WUKT32, CKV32, CKT32, WUV32, WG32, WU32, WO32, WD32 = (
        r.bitcast(U32) for r in (WQ, WUKT, CKV, CKT, WUV, WG, WU, WO, WD))

    def swap_heads(src32, dst32, rows):
        ch = 64

        def body(i, carry):
            w = _bf(src32[pl.ds(pl.multiple_of(i * ch, ch), ch)])
            dst32[:, pl.ds(pl.multiple_of(i * (ch // 2), ch // 2), ch // 2), :] = (
                pltpu.bitcast(jnp.swapaxes(w, 0, 1), U32))
            return carry
        jax.lax.fori_loop(0, rows // ch, body, 0)

    def make_wukt():
        def body(i, carry):
            w = _bf(wuk_l32[pl.ds(pl.multiple_of(i * L, L), L)])
            w = jnp.swapaxes(jnp.swapaxes(w, 0, 1), 1, 2)
            WUKT32[:, pl.ds(pl.multiple_of(i * W2, W2), W2), :] = pltpu.bitcast(w, U32)
            return carry
        jax.lax.fori_loop(0, CT, body, 0)

    def make_ckt():
        def body(kt, carry):
            for ct in range(CT):
                w = _bf(CKV32[ct, pl.ds(pl.multiple_of(kt * W2, W2), W2)])
                CKT32[kt, ct * W2:(ct + 1) * W2, :] = pltpu.bitcast(w.T, U32)
            return carry
        jax.lax.fori_loop(0, KT, body, 0)

    def make_wgu(src, dst32):
        def body(ft, carry):
            w = src[pl.ds(pl.multiple_of(ft * L, L), L), :]
            dst32[ft] = pltpu.bitcast(w.T, U32)
            return carry
        jax.lax.fori_loop(0, FT - 1, body, 0)
        w = src[(FT - 1) * L:FF, :]
        w = jnp.concatenate([w, jnp.zeros((L - F_TAIL, M), BF16)], axis=0)
        dst32[FT - 1] = pltpu.bitcast(w.T, U32)

    def make_cols(src, dst32, r0, rows):
        for nt in range(MT):
            dst32[nt, r0 // 2:(r0 + rows) // 2, :] = pltpu.bitcast(
                src[r0:r0 + rows, nt * L:(nt + 1) * L], U32)

    sub = jax.lax.broadcasted_iota(jnp.int32, (R, L), 0)
    zero_v = []

    def link(a, dep):
        if dep is None:
            return a
        z = pltpu.bitcast(dep, U32) & zero_v[0]
        a32 = pltpu.bitcast(a, U32)
        return pltpu.bitcast(a32 | z[:a32.shape[0]], a.dtype)

    def make_xb(xt):
        for t in range(MT):
            w = _col_bcast(xt[t].astype(BF16)[0:1])
            XE[t * W2:(t + 1) * W2, :] = _lo(w)
            XO[t * W2:(t + 1) * W2, :] = _hi(w)

    def tile(ref32, lead, t):
        return _bf(ref32[lead, t * W2:(t + 1) * W2, :])

    def vpu_matvec_step(accs, ref_keys, s, dep):
        xe = link(XE[s * R:(s + 1) * R, :], dep)
        xo = XO[s * R:(s + 1) * R, :]
        for ref32, lead in ref_keys:
            w = ref32[lead, s * R:(s + 1) * R, :]
            _acc(accs, (id(ref32), lead), _lo(w) * xe + _hi(w) * xo)

    def attention(xt, first):
        mu, rstd = _stats(xt)
        lhs = _lhs16(xt)
        qscale = rstd * (D ** -0.5)
        nvq = 0 if first else VQ_HEADS
        nvo = 0 if first else VO_HEADS
        if first:
            c_wq.wait()
            swap_heads(wq_l32, WQ32, M)
            c_wuk.wait()
            make_wukt()

        oq, qh, qa = {}, {}, {}

        def q_op(h, t):
            def f(dep):
                p = _dot(link(lhs[t], dep), tile(WQ32, h, t))
                o = _acc(oq, h, p)
                if t == MT - 1:
                    if first and h >= H - VQ_HEADS:
                        CSQ[h] = o[R:]
                    qh[h] = ((o[:R] - mu * o[R:]) * qscale).astype(BF16)
                return p[:R]
            return f

        def qabs_op(h, ct):
            def f(dep):
                g, i = divmod(h, R)
                t = _dot(qh[h], tile(WUKT32, h, ct))
                qa[g, ct] = t if (g, ct) not in qa else jnp.where(sub == i, t, qa[g, ct])
                return t
            f.ready = lambda: h in qh
            return f

        na = H - nvq
        edge = min(EDGE, na)

        def q_produce(h):
            if h == 0:
                return _by_column(range(edge), q_op, MT)
            return [] if h < edge else _by_item([h], q_op, MT)

        def q_consume(h):
            if h >= H - EDGE:
                return _by_column(range(H - EDGE, H), qabs_op, CT) if h == H - 1 else []
            return _by_item([h], qabs_op, CT)

        ms = _skewed(na, max(SKEW_Q, edge), q_produce, q_consume)
        for h in range(na, H):
            ms += q_consume(h)
        qacc = {}

        def q_vstep(hs, s):
            def f(dep):
                vpu_matvec_step(qacc, [(WQ32, h) for h in hs], s, dep)
                if s == M // 16 - 1:
                    for h in hs:
                        t = _sublane_sum(qacc[id(WQ32), h])
                        qh[h] = ((t - mu * CSQ[h]) * qscale).astype(BF16)
                return qacc[id(WQ32), hs[0]]
            return f

        if nvq:
            make_xb(xt)
        vs = [q_vstep(list(range(h0, min(H, h0 + VQ_GROUP))), s)
              for h0 in range(na, H, VQ_GROUP) for s in range(M // 16)]
        _cosched(ms, vs, P1_CFG)
        qabs = [jnp.concatenate([qa[g, ct] for g in range(H // R)], axis=0).astype(BF16)
                for ct in range(CT)]

        if first:
            for c in c_ckv:
                c.wait()
            make_ckt()
        nch = KT // KCHUNK
        sc, ps, lats = {}, {}, {}
        mxs, lss = [None] * nch, [None] * nch

        def score_op(kt, ct):
            def f(dep):
                _acc(sc, kt, _dot(qabs[ct], tile(CKT32, kt, ct)))
                j = kt // KCHUNK
                if ct == CT - 1 and kt == (j + 1) * KCHUNK - 1:
                    kts = range(j * KCHUNK, (j + 1) * KCHUNK)
                    mx = sc[kts[0]]
                    for k in kts[1:]:
                        mx = jnp.maximum(mx, sc[k])
                    mx = jnp.max(mx, axis=-1, keepdims=True)
                    lsum = None
                    for k in kts:
                        e = jnp.exp(sc[k] - mx)
                        lsum = e if lsum is None else lsum + e
                        ps[k] = e.astype(BF16)
                    mxs[j], lss[j] = mx, lsum
            return f

        def lat_op(kt, ct):
            def f(dep):
                _acc(lats, (kt // KCHUNK, ct), _dot(ps[kt], tile(CKV32, ct, kt)))
            return f

        def s_produce(j):
            kts = list(range(j * KCHUNK, (j + 1) * KCHUNK))
            if j == 0:
                return (_by_column(kts[:EDGE], score_op, CT)
                        + _by_item(kts[EDGE:], score_op, CT))
            return _by_item(kts, score_op, CT)

        def s_consume(j):
            return _by_column(range(j * KCHUNK, (j + 1) * KCHUNK), lat_op, CT)

        _run(_skewed(nch, SKEW_S, s_produce, s_consume))
        m = mxs[0]
        for t in mxs[1:]:
            m = jnp.maximum(m, t)
        alpha = [jnp.exp(t - m) for t in mxs]
        lsum = alpha[0] * lss[0]
        for a, t in zip(alpha[1:], lss[1:]):
            lsum = lsum + a * t
        inv = 1.0 / jnp.sum(lsum, axis=-1, keepdims=True)
        alpha = [a * inv for a in alpha]
        latg = {}
        for ct in range(CT):
            t = alpha[0] * lats[0, ct]
            for j in range(1, nch):
                t = t + alpha[j] * lats[j, ct]
            for g in range(H // R):
                latg[g, ct] = t[g * R:(g + 1) * R].astype(BF16)

        if first:
            c_wuv.wait()
            swap_heads(wuv_l32, WUV32, DC)
        cacc, cbs, o = {}, {}, {}

        def ctx_op(h, ct):
            def f(dep):
                g, i = divmod(h, R)
                p = _dot(link(latg[g, ct], dep), tile(WUV32, h, ct))
                c = _acc(cacc, h, p)
                if ct == CT - 1:
                    cbs[h] = jnp.broadcast_to(c[i:i + 1], (R, D)).astype(BF16)
                return p
            return f

        def out_op(h, nt):
            def f(dep):
                t = _dot(cbs[h], tile(WO32, nt, h))
                _acc(o, nt, t)
                return t
            return f

        if first:
            _run(_by_item(range(H), ctx_op, CT))
            c_wg.wait()
            make_wgu(wg_l, WG32)
            c_wu.wait()
            make_wgu(wu_l, WU32)
            hpc = H // WO_CHUNKS
            for c in range(WO_CHUNKS):
                c_wo[c].wait()
                make_cols(wo_l, WO32, c * wo_rows, wo_rows)
                _run(_by_item(range(c * hpc, (c + 1) * hpc), out_op, MT))
            return [_round_bf16(xt[nt] + o[nt]) for nt in range(MT)]

        ms = _by_column(range(EDGE), ctx_op, CT) + _by_item(range(EDGE, nvo), ctx_op, CT)
        h0 = max(nvo, EDGE)

        def o_produce(i):
            return _by_item([h0 + i], ctx_op, CT)

        def o_consume(h):
            if h >= H - EDGE:
                return _by_column(range(H - EDGE, H), out_op, MT) if h == H - 1 else []
            return _by_item([h], out_op, MT)

        for step in range(H - h0 + SKEW_O):
            if step < H - h0:
                ms += o_produce(step)
            if step >= SKEW_O:
                ms += o_consume(h0 + step - SKEW_O)
        for h in range(nvo, h0):
            ms += o_consume(h)
        cw, ov = {}, {}

        def xlu_op(h):
            def f(dep):
                cw[h] = _col_bcast(cbs[h][0:1])
                return pltpu.bitcast(cw[h][:R], F32)
            f.ready = lambda: h in cbs
            return f

        def o_vstep(h, k):
            def f(dep):
                w = cw[h][k * R:(k + 1) * R]
                ce, co = link(_lo(w), dep), _hi(w)
                r0 = h * W2 + k * R
                for nt in range(MT):
                    w = WO32[nt, r0:r0 + R, :]
                    _acc(ov, nt, _lo(w) * ce + _hi(w) * co)
                return ov[0]
            return f

        vs = [xlu_op(h) for h in range(min(XLU_AHEAD, nvo))]
        for h in range(nvo):
            if h + XLU_AHEAD < nvo:
                vs.append(xlu_op(h + XLU_AHEAD))
            vs += [o_vstep(h, k) for k in range(L // 16)]
        _cosched(ms, vs, P3_CFG)
        if nvo:
            o = {nt: o[nt] + _sublane_sum(ov[nt]) for nt in range(MT)}
        return [_round_bf16(xt[nt] + o[nt]) for nt in range(MT)]

    def ffn(xt, first):
        mu, rstd = _stats(xt)
        lhs = _lhs16(xt)
        xn = [(x - mu) * rstd for x in xt]
        wr = wr_v[...].reshape(1, M).astype(F32)
        r = jnp.sum(jnp.concatenate(xn, axis=1) * wr, axis=-1, keepdims=True)
        gate = jax.nn.sigmoid(r)
        nvf = 0 if first else VF_TILES
        pre, acts, y = {}, {}, {}

        def finish(ft):
            g, u = pre[ft, 0] * rstd, pre[ft, 1] * rstd
            acts[ft] = (g * jax.nn.sigmoid(g) * u).astype(BF16)

        def gu_op(key, t):
            ft, which = key

            def f(dep):
                p = _dot(link(lhs[t], dep), tile((WG32, WU32)[which], ft, t))
                o = _acc(pre, key, p)
                if t == MT - 1:
                    if first and ft < VF_TILES:
                        (CSG, CSU)[which][ft] = o[R:]
                    pre[key] = o[:R] - mu * o[R:]
                    if which == 1:
                        finish(ft)
                return p[:R]
            return f

        def dn_op(ft, nt):
            def f(dep):
                rows = L if ft < FT - 1 else F_TAIL
                a = acts[ft] if rows == L else acts[ft][:, :rows]
                if first:
                    w = wd_l[ft * L:ft * L + rows, nt * L:(nt + 1) * L]
                else:
                    w = _bf(WD32[nt, ft * W2:ft * W2 + rows // 2, :])
                t = _dot(a, w)
                _acc(y, nt, t)
                return t
            f.ready = lambda: ft in acts
            return f

        def gu_keys(fts):
            return [(ft, which) for ft in fts for which in range(2)]

        if first:
            _run(_by_item(gu_keys(range(FT)), gu_op, MT))
            for c, (f0, f1) in enumerate(WD_CHUNKS):
                c_wd[c].wait()
                if c == len(WD_CHUNKS) - 1:
                    _run(_by_column(range(f0, f1), dn_op, MT))
                else:
                    _run(_by_item(range(f0, f1), dn_op, MT))
        else:
            mt = list(range(nvf, FT))
            last = (mt + list(range(nvf)))[-2:] if nvf < 2 else list(range(nvf))[-2:]

            def g_produce(i):
                if i == 0:
                    return _by_column(gu_keys(mt[:2]), gu_op, MT)
                return [] if i == 1 else _by_item(gu_keys([mt[i]]), gu_op, MT)

            def g_consume(ft):
                if ft in last:
                    return _by_column(last, dn_op, MT) if ft == last[-1] else []
                return _by_item([ft], dn_op, MT)

            ms = _skewed(len(mt), SKEW_F, g_produce, lambda i: g_consume(mt[i]))
            for ft in range(nvf):
                ms += g_consume(ft)
            facc = {}

            def f_vstep(fts, s):
                def f(dep):
                    keys = [(w, ft) for ft in fts for w in (WG32, WU32)]
                    vpu_matvec_step(facc, keys, s, dep)
                    if s == M // 16 - 1:
                        for ft in fts:
                            for wh, (w, cs) in enumerate(((WG32, CSG), (WU32, CSU))):
                                pre[ft, wh] = _sublane_sum(facc[id(w), ft]) - mu * cs[ft]
                            finish(ft)
                    return facc[id(WG32), fts[0]]
                return f

            if nvf:
                make_xb(xt)
            vs = [f_vstep(list(range(f0, min(nvf, f0 + VF_GROUP))), s)
                  for f0 in range(0, nvf, VF_GROUP) for s in range(M // 16)]
            _cosched(ms, vs, P4_CFG)
        return [_round_bf16(xt[nt] + xn[nt] + y[nt] * gate) for nt in range(MT)]

    for c in c_small:
        c.wait()
    x = jnp.broadcast_to(x_v[...].astype(F32), (R, M))
    xc = jnp.broadcast_to(x_v2[...].astype(F32), (R, M))
    zero_v.append(pltpu.bitcast(x[:, :L], U32) ^ pltpu.bitcast(xc[:, :L], U32))
    xt = [x[:, t * L:(t + 1) * L] for t in range(MT)]
    xt = attention(xt, True)
    xt = ffn(xt, True)
    if N_LAYERS > 1:
        make_cols(wd_l, WD32, 0, FF)
        xt = attention(xt, False)
        xt = ffn(xt, False)
    o_ref[...] = jnp.concatenate(xt, axis=1)[0:1].astype(o_ref.dtype)


@jax.jit
def pallas_interleave_layers__compressed_kv_cla__moe_arch_mod__decode_kernel(
    A_x: jax.Array,
    A_c_kv: jax.Array,
    A_w_q: jax.Array,
    A_w_uk: jax.Array,
    A_w_uv: jax.Array,
    A_w_o: jax.Array,
    B_x: jax.Array,
    B_w_r: jax.Array,
    B_w_gate: jax.Array,
    B_w_up: jax.Array,
    B_w_down: jax.Array,
):
    del B_x
    args = (
        A_x.reshape(1, M),
        B_w_r,
        A_w_q,
        A_w_uk,
        A_c_kv.reshape(SK, DC),
        A_w_uv,
        B_w_gate.T,
        B_w_up.T,
        A_w_o.reshape(H * D, M),
        B_w_down,
    )
    n_sems = 7 + WO_CHUNKS + len(WD_CHUNKS)
    scratch = [
        pltpu.VMEM((1, M), BF16),
        pltpu.VMEM((1, M), BF16),
        pltpu.VMEM((M,), BF16),
        pltpu.VMEM((M, H, D), BF16),
        pltpu.VMEM((DC, H, D), BF16),
        pltpu.VMEM((DC, H, D), BF16),
        pltpu.VMEM((FF, M), BF16),
        pltpu.VMEM((FF, M), BF16),
        pltpu.VMEM((H * D, M), BF16),
        pltpu.VMEM((FF, M), BF16),
        pltpu.VMEM((H, M, D), BF16),
        pltpu.VMEM((H, DC, L), BF16),
        pltpu.VMEM((CT, SK, L), BF16),
        pltpu.VMEM((KT, DC, L), BF16),
        pltpu.VMEM((H, DC, D), BF16),
        pltpu.VMEM((FT, M, L), BF16),
        pltpu.VMEM((FT, M, L), BF16),
        pltpu.VMEM((MT, H * D, L), BF16),
        pltpu.VMEM((MT, FF, L), BF16),
        pltpu.VMEM((H, R, L), F32),
        pltpu.VMEM((FT, R, L), F32),
        pltpu.VMEM((FT, R, L), F32),
        pltpu.VMEM((M // 2, L), F32),
        pltpu.VMEM((M // 2, L), F32),
        pltpu.SemaphoreType.DMA((n_sems,)),
    ]
    out = pl.pallas_call(
        _kernel,
        out_shape=jax.ShapeDtypeStruct((1, M), A_x.dtype),
        in_specs=[pl.BlockSpec(memory_space=pl.ANY)] * len(args),
        out_specs=pl.BlockSpec(memory_space=pltpu.VMEM),
        scratch_shapes=scratch,
        compiler_params=pltpu.CompilerParams(
            vmem_limit_bytes=100 * 1024 * 1024),
        name="mla_moe_decode",
    )(*args)
    return out.reshape(1, 1, M)
```

```python
import jax
import jax.numpy as jnp
import jax.experimental.pallas as pl
import jax.experimental.pallas.tpu as pltpu

F32 = jnp.float32
BF16 = jnp.bfloat16
U32 = jnp.uint32

H = 32
D = 128
M = 640
DC = 512
SK = 4096
FF = 1728
EPS = 1e-5
R = 8
L = 128
W2 = L // 2

MT = M // L
CT = DC // L
KT = SK // L
FT = -(-FF // L)
F_TAIL = FF - (FT - 1) * L
KCHUNK = 8
WO_CHUNKS = 4
WD_CHUNKS = ((0, 7), (7, 12), (12, FT))

N_LAYERS = 2
SKEW_Q = 8
SKEW_S = 1
SKEW_O = 6
SKEW_F = 5
EDGE = 4

VQ_HEADS = 16
VQ_GROUP = 4
P1_CFG = (30, 1.0, 1, 18, 1, 0)
VO_HEADS = 16
P3_CFG = (50, 0.95, 2, 18, 1, 80)
XLU_AHEAD = 2
VF_TILES = 4
VF_GROUP = 2
P4_CFG = (20, 0.7, 2, 18, 1, 0)


def _always():
    return True


def _cosched(ms, vs, cfg):
    vstart, vrate, lag_v, lag_m, nlink, lstart = cfg
    mres, vres = [], []
    j = 0

    def emit_v(dep):
        nonlocal j
        vres.append(vs[j](dep))
        j += 1

    for i, m in enumerate(ms):
        while not getattr(m, "ready", _always)():
            emit_v(None)
        dep = None
        if len(vres) > lag_v and i % nlink == 0 and j < len(vs) and i >= lstart:
            dep = vres[-1 - lag_v]
        mres.append(m(dep))
        while (j < len(vs) and j < (i + 1 - vstart) * vrate
               and getattr(vs[j], "ready", _always)()):
            emit_v(mres[-1 - lag_m] if (len(mres) > lag_m and j % 2 == 0) else None)
    while j < len(vs):
        emit_v(None)


def _skewed(n, skew, produce, consume):
    out = []
    for step in range(n + skew):
        if step < n:
            out += produce(step)
        if step >= skew:
            out += consume(step - skew)
    return out


def _by_column(items, op, ncol):
    return [op(it, c) for c in range(ncol) for it in items]


def _by_item(items, op, ncol):
    return [op(it, c) for it in items for c in range(ncol)]


def _run(ops):
    for f in ops:
        f(None)


def _dot(a, b):
    return jnp.dot(a, b, preferred_element_type=F32)


def _bf(words):
    return pltpu.bitcast(words, BF16)


def _lo(w):
    return pltpu.bitcast(w << 16, F32)


def _hi(w):
    return pltpu.bitcast(w & jnp.uint32(0xFFFF0000), F32)


def _sublane_sum(t):
    t = t + pltpu.roll(t, 4, 0)
    t = t + pltpu.roll(t, 2, 0)
    return t + pltpu.roll(t, 1, 0)


def _col_bcast(row):
    return pltpu.bitcast(jnp.broadcast_to(row, (L, L)).T, U32)


def _round_bf16(x):
    return x.astype(BF16).astype(F32)


def _stats(xt):
    x = jnp.concatenate(xt, axis=1)
    mu = jnp.mean(x, axis=-1, keepdims=True)
    xc = x - mu
    var = jnp.mean(xc * xc, axis=-1, keepdims=True)
    return mu, jax.lax.rsqrt(var + EPS)


def _lhs16(xt):
    return [jnp.concatenate([x, jnp.ones_like(x)], axis=0).astype(BF16) for x in xt]


def _acc(d, k, v):
    d[k] = v if d.get(k) is None else d[k] + v
    return d[k]


def _kernel(x_hbm, wr_hbm, wq_hbm, wuk_hbm, ckv_hbm, wuv_hbm, wg_hbm, wu_hbm,
            wo_hbm, wd_hbm,
            o_ref,
            x_v, x_v2, wr_v, wq_l, wuk_l, wuv_l, wg_l, wu_l, wo_l, wd_l,
            WQ, WUKT, CKV, CKT, WUV, WG, WU, WO, WD,
            CSQ, CSG, CSU, XE, XO, sems):
    sem_ids = iter(range(64))

    def copy(src, dst, sem=None):
        sem = next(sem_ids) if sem is None else sem
        c = pltpu.make_async_copy(src, dst, sems.at[sem])
        c.start()
        return c

    c_wq = copy(wq_hbm, wq_l)
    s_small = next(sem_ids)
    c_small = [copy(x_hbm, x_v, s_small), copy(x_hbm, x_v2, s_small),
               copy(wr_hbm, wr_v, s_small)]
    c_wuk = copy(wuk_hbm, wuk_l)
    s_ckv = next(sem_ids)
    c_ckv = [copy(ckv_hbm.at[:, pl.ds(ct * L, L)], CKV.at[ct], s_ckv) for ct in range(CT)]
    c_wuv = copy(wuv_hbm, wuv_l)
    c_wg = copy(wg_hbm, wg_l)
    c_wu = copy(wu_hbm, wu_l)
    wo_rows = H * D // WO_CHUNKS
    c_wo = [copy(wo_hbm.at[pl.ds(c * wo_rows, wo_rows)],
                 wo_l.at[pl.ds(c * wo_rows, wo_rows)]) for c in range(WO_CHUNKS)]
    c_wd = []
    for (f0, f1) in WD_CHUNKS:
        r0, r1 = f0 * L, min(f1 * L, FF)
        c_wd.append(copy(wd_hbm.at[pl.ds(r0, r1 - r0)], wd_l.at[pl.ds(r0, r1 - r0)]))

    wq_l32, wuk_l32, wuv_l32 = (r.bitcast(U32) for r in (wq_l, wuk_l, wuv_l))
    WQ32, WUKT32, CKV32, CKT32, WUV32, WG32, WU32, WO32, WD32 = (
        r.bitcast(U32) for r in (WQ, WUKT, CKV, CKT, WUV, WG, WU, WO, WD))

    def swap_heads(src32, dst32, rows):
        ch = 64

        def body(i, carry):
            w = _bf(src32[pl.ds(pl.multiple_of(i * ch, ch), ch)])
            dst32[:, pl.ds(pl.multiple_of(i * (ch // 2), ch // 2), ch // 2), :] = (
                pltpu.bitcast(jnp.swapaxes(w, 0, 1), U32))
            return carry
        jax.lax.fori_loop(0, rows // ch, body, 0)

    def make_wukt():
        def body(i, carry):
            w = _bf(wuk_l32[pl.ds(pl.multiple_of(i * L, L), L)])
            w = jnp.swapaxes(jnp.swapaxes(w, 0, 1), 1, 2)
            WUKT32[:, pl.ds(pl.multiple_of(i * W2, W2), W2), :] = pltpu.bitcast(w, U32)
            return carry
        jax.lax.fori_loop(0, CT, body, 0)

    def make_ckt():
        def body(kt, carry):
            for ct in range(CT):
                w = _bf(CKV32[ct, pl.ds(pl.multiple_of(kt * W2, W2), W2)])
                CKT32[kt, ct * W2:(ct + 1) * W2, :] = pltpu.bitcast(w.T, U32)
            return carry
        jax.lax.fori_loop(0, KT, body, 0)

    def make_wgu(src, dst32):
        def body(ft, carry):
            w = src[pl.ds(pl.multiple_of(ft * L, L), L), :]
            dst32[ft] = pltpu.bitcast(w.T, U32)
            return carry
        jax.lax.fori_loop(0, FT - 1, body, 0)
        w = src[(FT - 1) * L:FF, :]
        w = jnp.concatenate([w, jnp.zeros((L - F_TAIL, M), BF16)], axis=0)
        dst32[FT - 1] = pltpu.bitcast(w.T, U32)

    def make_cols(src, dst32, r0, rows):
        for nt in range(MT):
            dst32[nt, r0 // 2:(r0 + rows) // 2, :] = pltpu.bitcast(
                src[r0:r0 + rows, nt * L:(nt + 1) * L], U32)

    sub = jax.lax.broadcasted_iota(jnp.int32, (R, L), 0)
    zero_v = []

    def link(a, dep):
        if dep is None:
            return a
        z = pltpu.bitcast(dep, U32) & zero_v[0]
        a32 = pltpu.bitcast(a, U32)
        return pltpu.bitcast(a32 | z[:a32.shape[0]], a.dtype)

    def make_xb(xt):
        for t in range(MT):
            w = _col_bcast(xt[t].astype(BF16)[0:1])
            XE[t * W2:(t + 1) * W2, :] = _lo(w)
            XO[t * W2:(t + 1) * W2, :] = _hi(w)

    def tile(ref32, lead, t):
        return _bf(ref32[lead, t * W2:(t + 1) * W2, :])

    def vpu_matvec_step(accs, ref_keys, s, dep):
        xe = link(XE[s * R:(s + 1) * R, :], dep)
        xo = XO[s * R:(s + 1) * R, :]
        for ref32, lead in ref_keys:
            w = ref32[lead, s * R:(s + 1) * R, :]
            _acc(accs, (id(ref32), lead), _lo(w) * xe + _hi(w) * xo)

    def attention(xt, first):
        mu, rstd = _stats(xt)
        lhs = _lhs16(xt)
        qscale = rstd * (D ** -0.5)
        nvq = 0 if first else VQ_HEADS
        nvo = 0 if first else VO_HEADS
        if first:
            c_wq.wait()
            swap_heads(wq_l32, WQ32, M)
            c_wuk.wait()
            make_wukt()

        oq, qh, qa = {}, {}, {}

        def q_op(h, t):
            def f(dep):
                p = _dot(link(lhs[t], dep), tile(WQ32, h, t))
                o = _acc(oq, h, p)
                if t == MT - 1:
                    if first and h >= H - VQ_HEADS:
                        CSQ[h] = o[R:]
                    qh[h] = ((o[:R] - mu * o[R:]) * qscale).astype(BF16)
                return p[:R]
            return f

        def qabs_op(h, ct):
            def f(dep):
                g, i = divmod(h, R)
                t = _dot(qh[h], tile(WUKT32, h, ct))
                qa[g, ct] = t if (g, ct) not in qa else jnp.where(sub == i, t, qa[g, ct])
                return t
            f.ready = lambda: h in qh
            return f

        na = H - nvq
        edge = min(EDGE, na)

        def q_produce(h):
            if h == 0:
                return _by_column(range(edge), q_op, MT)
            return [] if h < edge else _by_item([h], q_op, MT)

        def q_consume(h):
            if h >= H - EDGE:
                return _by_column(range(H - EDGE, H), qabs_op, CT) if h == H - 1 else []
            return _by_item([h], qabs_op, CT)

        ms = _skewed(na, max(SKEW_Q, edge), q_produce, q_consume)
        for h in range(na, H):
            ms += q_consume(h)
        qacc = {}

        def q_vstep(hs, s):
            def f(dep):
                vpu_matvec_step(qacc, [(WQ32, h) for h in hs], s, dep)
                if s == M // 16 - 1:
                    for h in hs:
                        t = _sublane_sum(qacc[id(WQ32), h])
                        qh[h] = ((t - mu * CSQ[h]) * qscale).astype(BF16)
                return qacc[id(WQ32), hs[0]]
            return f

        if nvq:
            make_xb(xt)
        vs = [q_vstep(list(range(h0, min(H, h0 + VQ_GROUP))), s)
              for h0 in range(na, H, VQ_GROUP) for s in range(M // 16)]
        _cosched(ms, vs, P1_CFG)
        qabs = [jnp.concatenate([qa[g, ct] for g in range(H // R)], axis=0).astype(BF16)
                for ct in range(CT)]

        if first:
            for c in c_ckv:
                c.wait()
            make_ckt()
        nch = KT // KCHUNK
        sc, ps, lats = {}, {}, {}
        mxs, lss = [None] * nch, [None] * nch

        def score_op(kt, ct):
            def f(dep):
                _acc(sc, kt, _dot(qabs[ct], tile(CKT32, kt, ct)))
                j = kt // KCHUNK
                if ct == CT - 1 and kt == (j + 1) * KCHUNK - 1:
                    kts = range(j * KCHUNK, (j + 1) * KCHUNK)
                    mx = sc[kts[0]]
                    for k in kts[1:]:
                        mx = jnp.maximum(mx, sc[k])
                    mx = jnp.max(mx, axis=-1, keepdims=True)
                    lsum = None
                    for k in kts:
                        e = jnp.exp(sc[k] - mx)
                        lsum = e if lsum is None else lsum + e
                        ps[k] = e.astype(BF16)
                    mxs[j], lss[j] = mx, lsum
            return f

        def lat_op(kt, ct):
            def f(dep):
                _acc(lats, (kt // KCHUNK, ct), _dot(ps[kt], tile(CKV32, ct, kt)))
            return f

        def s_produce(j):
            kts = list(range(j * KCHUNK, (j + 1) * KCHUNK))
            if j == 0:
                return (_by_column(kts[:EDGE], score_op, CT)
                        + _by_item(kts[EDGE:], score_op, CT))
            return _by_item(kts, score_op, CT)

        def s_consume(j):
            return _by_column(range(j * KCHUNK, (j + 1) * KCHUNK), lat_op, CT)

        _run(_skewed(nch, SKEW_S, s_produce, s_consume))
        m = mxs[0]
        for t in mxs[1:]:
            m = jnp.maximum(m, t)
        alpha = [jnp.exp(t - m) for t in mxs]
        lsum = alpha[0] * lss[0]
        for a, t in zip(alpha[1:], lss[1:]):
            lsum = lsum + a * t
        inv = 1.0 / jnp.sum(lsum, axis=-1, keepdims=True)
        alpha = [a * inv for a in alpha]
        latg = {}
        for ct in range(CT):
            t = alpha[0] * lats[0, ct]
            for j in range(1, nch):
                t = t + alpha[j] * lats[j, ct]
            for g in range(H // R):
                latg[g, ct] = t[g * R:(g + 1) * R].astype(BF16)

        if first:
            c_wuv.wait()
            swap_heads(wuv_l32, WUV32, DC)
        cacc, cbs, o = {}, {}, {}

        def ctx_op(h, ct):
            def f(dep):
                g, i = divmod(h, R)
                p = _dot(link(latg[g, ct], dep), tile(WUV32, h, ct))
                c = _acc(cacc, h, p)
                if ct == CT - 1:
                    cbs[h] = jnp.broadcast_to(c[i:i + 1], (R, D)).astype(BF16)
                return p
            return f

        def out_op(h, nt):
            def f(dep):
                t = _dot(cbs[h], tile(WO32, nt, h))
                _acc(o, nt, t)
                return t
            return f

        if first:
            _run(_by_item(range(H), ctx_op, CT))
            c_wg.wait()
            make_wgu(wg_l, WG32)
            c_wu.wait()
            make_wgu(wu_l, WU32)
            hpc = H // WO_CHUNKS
            for c in range(WO_CHUNKS):
                c_wo[c].wait()
                make_cols(wo_l, WO32, c * wo_rows, wo_rows)
                _run(_by_item(range(c * hpc, (c + 1) * hpc), out_op, MT))
            return [_round_bf16(xt[nt] + o[nt]) for nt in range(MT)]

        ms = _by_column(range(EDGE), ctx_op, CT) + _by_item(range(EDGE, nvo), ctx_op, CT)
        h0 = max(nvo, EDGE)

        def o_produce(i):
            return _by_item([h0 + i], ctx_op, CT)

        def o_consume(h):
            if h >= H - EDGE:
                return _by_column(range(H - EDGE, H), out_op, MT) if h == H - 1 else []
            return _by_item([h], out_op, MT)

        for step in range(H - h0 + SKEW_O):
            if step < H - h0:
                ms += o_produce(step)
            if step >= SKEW_O:
                ms += o_consume(h0 + step - SKEW_O)
        for h in range(nvo, h0):
            ms += o_consume(h)
        cw, ov = {}, {}

        def xlu_op(h):
            def f(dep):
                cw[h] = _col_bcast(cbs[h][0:1])
                return pltpu.bitcast(cw[h][:R], F32)
            f.ready = lambda: h in cbs
            return f

        def o_vstep(h, k):
            def f(dep):
                w = cw[h][k * R:(k + 1) * R]
                ce, co = link(_lo(w), dep), _hi(w)
                r0 = h * W2 + k * R
                for nt in range(MT):
                    w = WO32[nt, r0:r0 + R, :]
                    _acc(ov, nt, _lo(w) * ce + _hi(w) * co)
                return ov[0]
            return f

        vs = [xlu_op(h) for h in range(min(XLU_AHEAD, nvo))]
        for h in range(nvo):
            if h + XLU_AHEAD < nvo:
                vs.append(xlu_op(h + XLU_AHEAD))
            vs += [o_vstep(h, k) for k in range(L // 16)]
        _cosched(ms, vs, P3_CFG)
        if nvo:
            o = {nt: o[nt] + _sublane_sum(ov[nt]) for nt in range(MT)}
        return [_round_bf16(xt[nt] + o[nt]) for nt in range(MT)]

    def ffn(xt, first):
        mu, rstd = _stats(xt)
        lhs = _lhs16(xt)
        xn = [(x - mu) * rstd for x in xt]
        wr = wr_v[...].reshape(1, M).astype(F32)
        r = jnp.sum(jnp.concatenate(xn, axis=1) * wr, axis=-1, keepdims=True)
        gate = jax.nn.sigmoid(r)
        nvf = 0 if first else VF_TILES
        pre, acts, y = {}, {}, {}

        def finish(ft):
            g, u = pre[ft, 0] * rstd, pre[ft, 1] * rstd
            acts[ft] = (g * jax.nn.sigmoid(g) * u).astype(BF16)

        def gu_op(key, t):
            ft, which = key

            def f(dep):
                p = _dot(link(lhs[t], dep), tile((WG32, WU32)[which], ft, t))
                o = _acc(pre, key, p)
                if t == MT - 1:
                    if first and ft < VF_TILES:
                        (CSG, CSU)[which][ft] = o[R:]
                    pre[key] = o[:R] - mu * o[R:]
                    if which == 1:
                        finish(ft)
                return p[:R]
            return f

        def dn_op(ft, nt):
            def f(dep):
                rows = L if ft < FT - 1 else F_TAIL
                a = acts[ft] if rows == L else acts[ft][:, :rows]
                if first:
                    w = wd_l[ft * L:ft * L + rows, nt * L:(nt + 1) * L]
                else:
                    w = _bf(WD32[nt, ft * W2:ft * W2 + rows // 2, :])
                t = _dot(a, w)
                _acc(y, nt, t)
                return t
            f.ready = lambda: ft in acts
            return f

        def gu_keys(fts):
            return [(ft, which) for ft in fts for which in range(2)]

        if first:
            _run(_by_item(gu_keys(range(FT)), gu_op, MT))
            for c, (f0, f1) in enumerate(WD_CHUNKS):
                c_wd[c].wait()
                if c == len(WD_CHUNKS) - 1:
                    _run(_by_column(range(f0, f1), dn_op, MT))
                else:
                    _run(_by_item(range(f0, f1), dn_op, MT))
        else:
            mt = list(range(nvf, FT))
            last = (mt + list(range(nvf)))[-2:] if nvf < 2 else list(range(nvf))[-2:]

            def g_produce(i):
                if i == 0:
                    return _by_column(gu_keys(mt[:2]), gu_op, MT)
                return [] if i == 1 else _by_item(gu_keys([mt[i]]), gu_op, MT)

            def g_consume(ft):
                if ft in last:
                    return _by_column(last, dn_op, MT) if ft == last[-1] else []
                return _by_item([ft], dn_op, MT)

            ms = _skewed(len(mt), SKEW_F, g_produce, lambda i: g_consume(mt[i]))
            for ft in range(nvf):
                ms += g_consume(ft)
            facc = {}

            def f_vstep(fts, s):
                def f(dep):
                    keys = [(w, ft) for ft in fts for w in (WG32, WU32)]
                    vpu_matvec_step(facc, keys, s, dep)
                    if s == M // 16 - 1:
                        for ft in fts:
                            for wh, (w, cs) in enumerate(((WG32, CSG), (WU32, CSU))):
                                pre[ft, wh] = _sublane_sum(facc[id(w), ft]) - mu * cs[ft]
                            finish(ft)
                    return facc[id(WG32), fts[0]]
                return f

            if nvf:
                make_xb(xt)
            vs = [f_vstep(list(range(f0, min(nvf, f0 + VF_GROUP))), s)
                  for f0 in range(0, nvf, VF_GROUP) for s in range(M // 16)]
            _cosched(ms, vs, P4_CFG)
        return [_round_bf16(xt[nt] + xn[nt] + y[nt] * gate) for nt in range(MT)]

    for c in c_small:
        c.wait()
    x = jnp.broadcast_to(x_v[...].astype(F32), (R, M))
    xc = jnp.broadcast_to(x_v2[...].astype(F32), (R, M))
    zero_v.append(pltpu.bitcast(x[:, :L], U32) ^ pltpu.bitcast(xc[:, :L], U32))
    xt = [x[:, t * L:(t + 1) * L] for t in range(MT)]
    xt = attention(xt, True)
    xt = ffn(xt, True)
    if N_LAYERS > 1:
        make_cols(wd_l, WD32, 0, FF)
        xt = attention(xt, False)
        xt = ffn(xt, False)
    o_ref[...] = jnp.concatenate(xt, axis=1)[0:1].astype(o_ref.dtype)


@jax.jit
def pallas_interleave_layers__compressed_kv_cla__moe_arch_mod__decode_kernel(
    A_x: jax.Array,
    A_c_kv: jax.Array,
    A_w_q: jax.Array,
    A_w_uk: jax.Array,
    A_w_uv: jax.Array,
    A_w_o: jax.Array,
    B_x: jax.Array,
    B_w_r: jax.Array,
    B_w_gate: jax.Array,
    B_w_up: jax.Array,
    B_w_down: jax.Array,
):
    del B_x
    args = (
        A_x.reshape(1, M),
        B_w_r,
        A_w_q,
        A_w_uk,
        A_c_kv.reshape(SK, DC),
        A_w_uv,
        B_w_gate.T,
        B_w_up.T,
        A_w_o.reshape(H * D, M),
        B_w_down,
    )
    n_sems = 7 + WO_CHUNKS + len(WD_CHUNKS)
    scratch = [
        pltpu.VMEM((1, M), BF16),
        pltpu.VMEM((1, M), BF16),
        pltpu.VMEM((M,), BF16),
        pltpu.VMEM((M, H, D), BF16),
        pltpu.VMEM((DC, H, D), BF16),
        pltpu.VMEM((DC, H, D), BF16),
        pltpu.VMEM((FF, M), BF16),
        pltpu.VMEM((FF, M), BF16),
        pltpu.VMEM((H * D, M), BF16),
        pltpu.VMEM((FF, M), BF16),
        pltpu.VMEM((H, M, D), BF16),
        pltpu.VMEM((H, DC, L), BF16),
        pltpu.VMEM((CT, SK, L), BF16),
        pltpu.VMEM((KT, DC, L), BF16),
        pltpu.VMEM((H, DC, D), BF16),
        pltpu.VMEM((FT, M, L), BF16),
        pltpu.VMEM((FT, M, L), BF16),
        pltpu.VMEM((MT, H * D, L), BF16),
        pltpu.VMEM((MT, FF, L), BF16),
        pltpu.VMEM((H, R, L), F32),
        pltpu.VMEM((FT, R, L), F32),
        pltpu.VMEM((FT, R, L), F32),
        pltpu.VMEM((M // 2, L), F32),
        pltpu.VMEM((M // 2, L), F32),
        pltpu.SemaphoreType.DMA((n_sems,)),
    ]
    out = pl.pallas_call(
        _kernel,
        out_shape=jax.ShapeDtypeStruct((1, M), A_x.dtype),
        in_specs=[pl.BlockSpec(memory_space=pl.ANY)] * len(args),
        out_specs=pl.BlockSpec(memory_space=pltpu.VMEM),
        scratch_shapes=scratch,
        compiler_params=pltpu.CompilerParams(
            vmem_limit_bytes=100 * 1024 * 1024),
        name="mla_moe_decode",
    )(*args)
    return out.reshape(1, 1, M)
```

```python
import jax
import jax.numpy as jnp
import jax.experimental.pallas as pl
import jax.experimental.pallas.tpu as pltpu

F32 = jnp.float32
BF16 = jnp.bfloat16
U32 = jnp.uint32

H = 32
D = 128
M = 640
DC = 512
SK = 4096
FF = 1728
EPS = 1e-5
R = 8
L = 128
W2 = L // 2

MT = M // L
CT = DC // L
KT = SK // L
FT = -(-FF // L)
F_TAIL = FF - (FT - 1) * L
KCHUNK = 8
WO_CHUNKS = 4
WD_CHUNKS = ((0, 7), (7, 12), (12, FT))

N_LAYERS = 2
SKEW_Q = 8
SKEW_S = 1
SKEW_O = 6
SKEW_F = 5
EDGE = 4

VQ_HEADS = 16
VQ_GROUP = 4
P1_CFG = (30, 1.0, 1, 18, 1, 0)
VO_HEADS = 16
P3_CFG = (50, 0.95, 2, 18, 1, 80)
XLU_AHEAD = 2
VF_TILES = 4
VF_GROUP = 2
P4_CFG = (20, 0.7, 2, 18, 1, 0)


def _always():
    return True


def _cosched(ms, vs, cfg):
    vstart, vrate, lag_v, lag_m, nlink, lstart = cfg
    mres, vres = [], []
    j = 0

    def emit_v(dep):
        nonlocal j
        vres.append(vs[j](dep))
        j += 1

    for i, m in enumerate(ms):
        while not getattr(m, "ready", _always)():
            emit_v(None)
        dep = None
        if len(vres) > lag_v and i % nlink == 0 and j < len(vs) and i >= lstart:
            dep = vres[-1 - lag_v]
        mres.append(m(dep))
        while (j < len(vs) and j < (i + 1 - vstart) * vrate
               and getattr(vs[j], "ready", _always)()):
            emit_v(mres[-1 - lag_m] if (len(mres) > lag_m and j % 2 == 0) else None)
    while j < len(vs):
        emit_v(None)


def _skewed(n, skew, produce, consume):
    out = []
    for step in range(n + skew):
        if step < n:
            out += produce(step)
        if step >= skew:
            out += consume(step - skew)
    return out


def _by_column(items, op, ncol):
    return [op(it, c) for c in range(ncol) for it in items]


def _by_item(items, op, ncol):
    return [op(it, c) for it in items for c in range(ncol)]


def _run(ops):
    for f in ops:
        f(None)


def _dot(a, b):
    return jnp.dot(a, b, preferred_element_type=F32)


def _bf(words):
    return pltpu.bitcast(words, BF16)


def _lo(w):
    return pltpu.bitcast(w << 16, F32)


def _hi(w):
    return pltpu.bitcast(w & jnp.uint32(0xFFFF0000), F32)


def _sublane_sum(t):
    t = t + pltpu.roll(t, 4, 0)
    t = t + pltpu.roll(t, 2, 0)
    return t + pltpu.roll(t, 1, 0)


def _col_bcast(row):
    return pltpu.bitcast(jnp.broadcast_to(row, (L, L)).T, U32)


def _round_bf16(x):
    return x.astype(BF16).astype(F32)


def _stats(xt):
    x = jnp.concatenate(xt, axis=1)
    mu = jnp.mean(x, axis=-1, keepdims=True)
    xc = x - mu
    var = jnp.mean(xc * xc, axis=-1, keepdims=True)
    return mu, jax.lax.rsqrt(var + EPS)


def _lhs16(xt):
    return [jnp.concatenate([x, jnp.ones_like(x)], axis=0).astype(BF16) for x in xt]


def _acc(d, k, v):
    d[k] = v if d.get(k) is None else d[k] + v
    return d[k]


def _kernel(x_hbm, wr_hbm, wq_hbm, wuk_hbm, ckv_hbm, wuv_hbm, wg_hbm, wu_hbm,
            wo_hbm, wd_hbm,
            o_ref,
            x_v, wr_v, wq_l, wuk_l, wuv_l, wg_l, wu_l, wo_l, wd_l,
            WQ, WUKT, CKV, CKT, WUV, WG, WU, WO, WD,
            CSQ, CSG, CSU, XE, XO, sems):
    sem_ids = iter(range(64))

    def copy(src, dst, sem=None):
        sem = next(sem_ids) if sem is None else sem
        c = pltpu.make_async_copy(src, dst, sems.at[sem])
        c.start()
        return c

    c_wq = copy(wq_hbm, wq_l)
    s_small = next(sem_ids)
    c_small = [copy(x_hbm, x_v, s_small), copy(wr_hbm, wr_v, s_small)]
    c_wuk = copy(wuk_hbm, wuk_l)
    s_ckv = next(sem_ids)
    c_ckv = [copy(ckv_hbm.at[:, pl.ds(ct * L, L)], CKV.at[ct], s_ckv) for ct in range(CT)]
    c_wuv = copy(wuv_hbm, wuv_l)
    c_wg = copy(wg_hbm, wg_l)
    c_wu = copy(wu_hbm, wu_l)
    wo_rows = H * D // WO_CHUNKS
    c_wo = [copy(wo_hbm.at[pl.ds(c * wo_rows, wo_rows)],
                 wo_l.at[pl.ds(c * wo_rows, wo_rows)]) for c in range(WO_CHUNKS)]
    c_wd = []
    for (f0, f1) in WD_CHUNKS:
        r0, r1 = f0 * L, min(f1 * L, FF)
        c_wd.append(copy(wd_hbm.at[pl.ds(r0, r1 - r0)], wd_l.at[pl.ds(r0, r1 - r0)]))

    wq_l32, wuk_l32, wuv_l32 = (r.bitcast(U32) for r in (wq_l, wuk_l, wuv_l))
    WQ32, WUKT32, CKV32, CKT32, WUV32, WG32, WU32, WO32, WD32 = (
        r.bitcast(U32) for r in (WQ, WUKT, CKV, CKT, WUV, WG, WU, WO, WD))

    def swap_heads(src32, dst32, rows):
        ch = 64

        def body(i, carry):
            w = _bf(src32[pl.ds(pl.multiple_of(i * ch, ch), ch)])
            dst32[:, pl.ds(pl.multiple_of(i * (ch // 2), ch // 2), ch // 2), :] = (
                pltpu.bitcast(jnp.swapaxes(w, 0, 1), U32))
            return carry
        jax.lax.fori_loop(0, rows // ch, body, 0)

    def make_wukt():
        def body(i, carry):
            w = _bf(wuk_l32[pl.ds(pl.multiple_of(i * L, L), L)])
            w = jnp.swapaxes(jnp.swapaxes(w, 0, 1), 1, 2)
            WUKT32[:, pl.ds(pl.multiple_of(i * W2, W2), W2), :] = pltpu.bitcast(w, U32)
            return carry
        jax.lax.fori_loop(0, CT, body, 0)

    def make_ckt():
        def body(kt, carry):
            for ct in range(CT):
                w = _bf(CKV32[ct, pl.ds(pl.multiple_of(kt * W2, W2), W2)])
                CKT32[kt, ct * W2:(ct + 1) * W2, :] = pltpu.bitcast(w.T, U32)
            return carry
        jax.lax.fori_loop(0, KT, body, 0)

    def make_wgu(src, dst32):
        def body(ft, carry):
            w = src[pl.ds(pl.multiple_of(ft * L, L), L), :]
            dst32[ft] = pltpu.bitcast(w.T, U32)
            return carry
        jax.lax.fori_loop(0, FT - 1, body, 0)
        w = src[(FT - 1) * L:FF, :]
        w = jnp.concatenate([w, jnp.zeros((L - F_TAIL, M), BF16)], axis=0)
        dst32[FT - 1] = pltpu.bitcast(w.T, U32)

    def make_cols(src, dst32, r0, rows):
        for nt in range(MT):
            dst32[nt, r0 // 2:(r0 + rows) // 2, :] = pltpu.bitcast(
                src[r0:r0 + rows, nt * L:(nt + 1) * L], U32)

    sub = jax.lax.broadcasted_iota(jnp.int32, (R, L), 0)
    zero_v = []

    def link(a, dep):
        if dep is None:
            return a
        z = pltpu.bitcast(dep, U32) & zero_v[0]
        a32 = pltpu.bitcast(a, U32)
        return pltpu.bitcast(a32 | z[:a32.shape[0]], a.dtype)

    def make_xb(xt):
        for t in range(MT):
            w = _col_bcast(xt[t].astype(BF16)[0:1])
            XE[t * W2:(t + 1) * W2, :] = _lo(w)
            XO[t * W2:(t + 1) * W2, :] = _hi(w)

    def tile(ref32, lead, t):
        return _bf(ref32[lead, t * W2:(t + 1) * W2, :])

    def vpu_matvec_step(accs, ref_keys, s, dep):
        xe = link(XE[s * R:(s + 1) * R, :], dep)
        xo = XO[s * R:(s + 1) * R, :]
        for ref32, lead in ref_keys:
            w = ref32[lead, s * R:(s + 1) * R, :]
            _acc(accs, (id(ref32), lead), _lo(w) * xe + _hi(w) * xo)

    def attention(xt, first):
        mu, rstd = _stats(xt)
        lhs = _lhs16(xt)
        qscale = rstd * (D ** -0.5)
        nvq = 0 if first else VQ_HEADS
        nvo = 0 if first else VO_HEADS
        if first:
            c_wq.wait()
            swap_heads(wq_l32, WQ32, M)
            c_wuk.wait()
            make_wukt()

        oq, qh, qa = {}, {}, {}

        def q_op(h, t):
            def f(dep):
                p = _dot(link(lhs[t], dep), tile(WQ32, h, t))
                o = _acc(oq, h, p)
                if t == MT - 1:
                    if first and h >= H - VQ_HEADS:
                        CSQ[h] = o[R:]
                    qh[h] = ((o[:R] - mu * o[R:]) * qscale).astype(BF16)
                return p[:R]
            return f

        def qabs_op(h, ct):
            def f(dep):
                g, i = divmod(h, R)
                t = _dot(qh[h], tile(WUKT32, h, ct))
                qa[g, ct] = t if (g, ct) not in qa else jnp.where(sub == i, t, qa[g, ct])
                return t
            f.ready = lambda: h in qh
            return f

        na = H - nvq
        edge = min(EDGE, na)

        def q_produce(h):
            if h == 0:
                return _by_column(range(edge), q_op, MT)
            return [] if h < edge else _by_item([h], q_op, MT)

        def q_consume(h):
            if h >= H - EDGE:
                return _by_column(range(H - EDGE, H), qabs_op, CT) if h == H - 1 else []
            return _by_item([h], qabs_op, CT)

        ms = _skewed(na, max(SKEW_Q, edge), q_produce, q_consume)
        for h in range(na, H):
            ms += q_consume(h)
        qacc = {}

        def q_vstep(hs, s):
            def f(dep):
                vpu_matvec_step(qacc, [(WQ32, h) for h in hs], s, dep)
                if s == M // 16 - 1:
                    for h in hs:
                        t = _sublane_sum(qacc[id(WQ32), h])
                        qh[h] = ((t - mu * CSQ[h]) * qscale).astype(BF16)
                return qacc[id(WQ32), hs[0]]
            return f

        if nvq:
            make_xb(xt)
        vs = [q_vstep(list(range(h0, min(H, h0 + VQ_GROUP))), s)
              for h0 in range(na, H, VQ_GROUP) for s in range(M // 16)]
        _cosched(ms, vs, P1_CFG)
        qabs = [jnp.concatenate([qa[g, ct] for g in range(H // R)], axis=0).astype(BF16)
                for ct in range(CT)]

        if first:
            for c in c_ckv:
                c.wait()
            make_ckt()
        nch = KT // KCHUNK
        sc, ps, lats = {}, {}, {}
        mxs, lss = [None] * nch, [None] * nch

        def score_op(kt, ct):
            def f(dep):
                _acc(sc, kt, _dot(qabs[ct], tile(CKT32, kt, ct)))
                j = kt // KCHUNK
                if ct == CT - 1 and kt == (j + 1) * KCHUNK - 1:
                    kts = range(j * KCHUNK, (j + 1) * KCHUNK)
                    mx = sc[kts[0]]
                    for k in kts[1:]:
                        mx = jnp.maximum(mx, sc[k])
                    mx = jnp.max(mx, axis=-1, keepdims=True)
                    lsum = None
                    for k in kts:
                        e = jnp.exp(sc[k] - mx)
                        lsum = e if lsum is None else lsum + e
                        ps[k] = e.astype(BF16)
                    mxs[j], lss[j] = mx, lsum
            return f

        def lat_op(kt, ct):
            def f(dep):
                _acc(lats, (kt // KCHUNK, ct), _dot(ps[kt], tile(CKV32, ct, kt)))
            return f

        def s_produce(j):
            kts = list(range(j * KCHUNK, (j + 1) * KCHUNK))
            if j == 0:
                return (_by_column(kts[:EDGE], score_op, CT)
                        + _by_item(kts[EDGE:], score_op, CT))
            return _by_item(kts, score_op, CT)

        def s_consume(j):
            return _by_column(range(j * KCHUNK, (j + 1) * KCHUNK), lat_op, CT)

        _run(_skewed(nch, SKEW_S, s_produce, s_consume))
        m = mxs[0]
        for t in mxs[1:]:
            m = jnp.maximum(m, t)
        alpha = [jnp.exp(t - m) for t in mxs]
        lsum = alpha[0] * lss[0]
        for a, t in zip(alpha[1:], lss[1:]):
            lsum = lsum + a * t
        inv = 1.0 / jnp.sum(lsum, axis=-1, keepdims=True)
        alpha = [a * inv for a in alpha]
        latg = {}
        for ct in range(CT):
            t = alpha[0] * lats[0, ct]
            for j in range(1, nch):
                t = t + alpha[j] * lats[j, ct]
            for g in range(H // R):
                latg[g, ct] = t[g * R:(g + 1) * R].astype(BF16)

        if first:
            c_wuv.wait()
            swap_heads(wuv_l32, WUV32, DC)
        cacc, cbs, o = {}, {}, {}

        def ctx_op(h, ct):
            def f(dep):
                g, i = divmod(h, R)
                p = _dot(link(latg[g, ct], dep), tile(WUV32, h, ct))
                c = _acc(cacc, h, p)
                if ct == CT - 1:
                    cbs[h] = jnp.broadcast_to(c[i:i + 1], (R, D)).astype(BF16)
                return p
            return f

        def out_op(h, nt):
            def f(dep):
                t = _dot(cbs[h], tile(WO32, nt, h))
                _acc(o, nt, t)
                return t
            return f

        if first:
            _run(_by_item(range(H), ctx_op, CT))
            c_wg.wait()
            make_wgu(wg_l, WG32)
            c_wu.wait()
            make_wgu(wu_l, WU32)
            hpc = H // WO_CHUNKS
            for c in range(WO_CHUNKS):
                c_wo[c].wait()
                make_cols(wo_l, WO32, c * wo_rows, wo_rows)
                _run(_by_item(range(c * hpc, (c + 1) * hpc), out_op, MT))
            return [_round_bf16(xt[nt] + o[nt]) for nt in range(MT)]

        ms = _by_column(range(EDGE), ctx_op, CT) + _by_item(range(EDGE, nvo), ctx_op, CT)
        h0 = max(nvo, EDGE)

        def o_produce(i):
            return _by_item([h0 + i], ctx_op, CT)

        def o_consume(h):
            if h >= H - EDGE:
                return _by_column(range(H - EDGE, H), out_op, MT) if h == H - 1 else []
            return _by_item([h], out_op, MT)

        for step in range(H - h0 + SKEW_O):
            if step < H - h0:
                ms += o_produce(step)
            if step >= SKEW_O:
                ms += o_consume(h0 + step - SKEW_O)
        for h in range(nvo, h0):
            ms += o_consume(h)
        cw, ov = {}, {}

        def xlu_op(h):
            def f(dep):
                cw[h] = _col_bcast(cbs[h][0:1])
                return pltpu.bitcast(cw[h][:R], F32)
            f.ready = lambda: h in cbs
            return f

        def o_vstep(h, k):
            def f(dep):
                w = cw[h][k * R:(k + 1) * R]
                ce, co = link(_lo(w), dep), _hi(w)
                r0 = h * W2 + k * R
                for nt in range(MT):
                    w = WO32[nt, r0:r0 + R, :]
                    _acc(ov, nt, _lo(w) * ce + _hi(w) * co)
                return ov[0]
            return f

        vs = [xlu_op(h) for h in range(min(XLU_AHEAD, nvo))]
        for h in range(nvo):
            if h + XLU_AHEAD < nvo:
                vs.append(xlu_op(h + XLU_AHEAD))
            vs += [o_vstep(h, k) for k in range(L // 16)]
        _cosched(ms, vs, P3_CFG)
        if nvo:
            o = {nt: o[nt] + _sublane_sum(ov[nt]) for nt in range(MT)}
        return [_round_bf16(xt[nt] + o[nt]) for nt in range(MT)]

    def ffn(xt, first):
        mu, rstd = _stats(xt)
        lhs = _lhs16(xt)
        xn = [(x - mu) * rstd for x in xt]
        wr = wr_v[...].reshape(1, M).astype(F32)
        r = jnp.sum(jnp.concatenate(xn, axis=1) * wr, axis=-1, keepdims=True)
        gate = jax.nn.sigmoid(r)
        nvf = 0 if first else VF_TILES
        pre, acts, y = {}, {}, {}

        def finish(ft):
            g, u = pre[ft, 0] * rstd, pre[ft, 1] * rstd
            acts[ft] = (g * jax.nn.sigmoid(g) * u).astype(BF16)

        def gu_op(key, t):
            ft, which = key

            def f(dep):
                p = _dot(link(lhs[t], dep), tile((WG32, WU32)[which], ft, t))
                o = _acc(pre, key, p)
                if t == MT - 1:
                    if first and ft < VF_TILES:
                        (CSG, CSU)[which][ft] = o[R:]
                    pre[key] = o[:R] - mu * o[R:]
                    if which == 1:
                        finish(ft)
                return p[:R]
            return f

        def dn_op(ft, nt):
            def f(dep):
                rows = L if ft < FT - 1 else F_TAIL
                a = acts[ft] if rows == L else acts[ft][:, :rows]
                if first:
                    w = wd_l[ft * L:ft * L + rows, nt * L:(nt + 1) * L]
                else:
                    w = _bf(WD32[nt, ft * W2:ft * W2 + rows // 2, :])
                t = _dot(a, w)
                _acc(y, nt, t)
                return t
            f.ready = lambda: ft in acts
            return f

        def gu_keys(fts):
            return [(ft, which) for ft in fts for which in range(2)]

        if first:
            _run(_by_item(gu_keys(range(FT)), gu_op, MT))
            for c, (f0, f1) in enumerate(WD_CHUNKS):
                c_wd[c].wait()
                if c == len(WD_CHUNKS) - 1:
                    _run(_by_column(range(f0, f1), dn_op, MT))
                else:
                    _run(_by_item(range(f0, f1), dn_op, MT))
        else:
            mt = list(range(nvf, FT))
            last = (mt + list(range(nvf)))[-2:] if nvf < 2 else list(range(nvf))[-2:]

            def g_produce(i):
                if i == 0:
                    return _by_column(gu_keys(mt[:2]), gu_op, MT)
                return [] if i == 1 else _by_item(gu_keys([mt[i]]), gu_op, MT)

            def g_consume(ft):
                if ft in last:
                    return _by_column(last, dn_op, MT) if ft == last[-1] else []
                return _by_item([ft], dn_op, MT)

            ms = _skewed(len(mt), SKEW_F, g_produce, lambda i: g_consume(mt[i]))
            for ft in range(nvf):
                ms += g_consume(ft)
            facc = {}

            def f_vstep(fts, s):
                def f(dep):
                    keys = [(w, ft) for ft in fts for w in (WG32, WU32)]
                    vpu_matvec_step(facc, keys, s, dep)
                    if s == M // 16 - 1:
                        for ft in fts:
                            for wh, (w, cs) in enumerate(((WG32, CSG), (WU32, CSU))):
                                pre[ft, wh] = _sublane_sum(facc[id(w), ft]) - mu * cs[ft]
                            finish(ft)
                    return facc[id(WG32), fts[0]]
                return f

            if nvf:
                make_xb(xt)
            vs = [f_vstep(list(range(f0, min(nvf, f0 + VF_GROUP))), s)
                  for f0 in range(0, nvf, VF_GROUP) for s in range(M // 16)]
            _cosched(ms, vs, P4_CFG)
        return [_round_bf16(xt[nt] + xn[nt] + y[nt] * gate) for nt in range(MT)]

    for c in c_small:
        c.wait()
    x = jnp.broadcast_to(x_v[...].astype(F32), (R, M))
    zero_v.append(jnp.full((R, L), pl.semaphore_read(sems.at[s_small]), jnp.int32).astype(U32))
    xt = [x[:, t * L:(t + 1) * L] for t in range(MT)]
    xt = attention(xt, True)
    xt = ffn(xt, True)
    if N_LAYERS > 1:
        make_cols(wd_l, WD32, 0, FF)
        xt = attention(xt, False)
        xt = ffn(xt, False)
    o_ref[...] = jnp.concatenate(xt, axis=1)[0:1].astype(o_ref.dtype)


@jax.jit
def pallas_interleave_layers__compressed_kv_cla__moe_arch_mod__decode_kernel(
    A_x: jax.Array,
    A_c_kv: jax.Array,
    A_w_q: jax.Array,
    A_w_uk: jax.Array,
    A_w_uv: jax.Array,
    A_w_o: jax.Array,
    B_x: jax.Array,
    B_w_r: jax.Array,
    B_w_gate: jax.Array,
    B_w_up: jax.Array,
    B_w_down: jax.Array,
):
    del B_x
    args = (
        A_x.reshape(1, M),
        B_w_r,
        A_w_q,
        A_w_uk,
        A_c_kv.reshape(SK, DC),
        A_w_uv,
        B_w_gate.T,
        B_w_up.T,
        A_w_o.reshape(H * D, M),
        B_w_down,
    )
    n_sems = 7 + WO_CHUNKS + len(WD_CHUNKS)
    scratch = [
        pltpu.VMEM((1, M), BF16),
        pltpu.VMEM((M,), BF16),
        pltpu.VMEM((M, H, D), BF16),
        pltpu.VMEM((DC, H, D), BF16),
        pltpu.VMEM((DC, H, D), BF16),
        pltpu.VMEM((FF, M), BF16),
        pltpu.VMEM((FF, M), BF16),
        pltpu.VMEM((H * D, M), BF16),
        pltpu.VMEM((FF, M), BF16),
        pltpu.VMEM((H, M, D), BF16),
        pltpu.VMEM((H, DC, L), BF16),
        pltpu.VMEM((CT, SK, L), BF16),
        pltpu.VMEM((KT, DC, L), BF16),
        pltpu.VMEM((H, DC, D), BF16),
        pltpu.VMEM((FT, M, L), BF16),
        pltpu.VMEM((FT, M, L), BF16),
        pltpu.VMEM((MT, H * D, L), BF16),
        pltpu.VMEM((MT, FF, L), BF16),
        pltpu.VMEM((H, R, L), F32),
        pltpu.VMEM((FT, R, L), F32),
        pltpu.VMEM((FT, R, L), F32),
        pltpu.VMEM((M // 2, L), F32),
        pltpu.VMEM((M // 2, L), F32),
        pltpu.SemaphoreType.DMA((n_sems,)),
    ]
    out = pl.pallas_call(
        _kernel,
        out_shape=jax.ShapeDtypeStruct((1, M), A_x.dtype),
        in_specs=[pl.BlockSpec(memory_space=pl.ANY)] * len(args),
        out_specs=pl.BlockSpec(memory_space=pltpu.VMEM),
        scratch_shapes=scratch,
        compiler_params=pltpu.CompilerParams(
            vmem_limit_bytes=100 * 1024 * 1024,
            disable_semaphore_checks=True),
        name="mla_moe_decode",
    )(*args)
    return out.reshape(1, 1, M)
```

```python
import jax
import jax.numpy as jnp
import jax.experimental.pallas as pl
import jax.experimental.pallas.tpu as pltpu

F32 = jnp.float32
BF16 = jnp.bfloat16
U32 = jnp.uint32

H = 32
D = 128
M = 640
DC = 512
SK = 4096
FF = 1728
EPS = 1e-5
R = 8
L = 128
W2 = L // 2

MT = M // L
CT = DC // L
KT = SK // L
FT = -(-FF // L)
F_TAIL = FF - (FT - 1) * L
KCHUNK = 8
WO_CHUNKS = 4
WD_CHUNKS = ((0, 7), (7, 12), (12, FT))

N_LAYERS = 2
SKEW_Q = 8
SKEW_S = 1
SKEW_O = 6
SKEW_F = 5
EDGE = 4

VQ_HEADS = 16
VQ_GROUP = 4
P1_CFG = (30, 1.0, 1, 18, 1, 0)
VO_HEADS = 16
P3_CFG = (50, 0.95, 2, 18, 1, 80)
XLU_AHEAD = 2
VF_TILES = 4
VF_GROUP = 2
P4_CFG = (20, 0.7, 2, 18, 1, 0)


def _always():
    return True


def _cosched(ms, vs, cfg):
    vstart, vrate, lag_v, lag_m, nlink, lstart = cfg
    mres, vres = [], []
    j = 0

    def emit_v(dep):
        nonlocal j
        vres.append(vs[j](dep))
        j += 1

    for i, m in enumerate(ms):
        while not getattr(m, "ready", _always)():
            emit_v(None)
        dep = None
        if len(vres) > lag_v and i % nlink == 0 and j < len(vs) and i >= lstart:
            dep = vres[-1 - lag_v]
        mres.append(m(dep))
        while (j < len(vs) and j < (i + 1 - vstart) * vrate
               and getattr(vs[j], "ready", _always)()):
            emit_v(mres[-1 - lag_m] if (len(mres) > lag_m and j % 2 == 0) else None)
    while j < len(vs):
        emit_v(None)


def _skewed(n, skew, produce, consume):
    out = []
    for step in range(n + skew):
        if step < n:
            out += produce(step)
        if step >= skew:
            out += consume(step - skew)
    return out


def _by_column(items, op, ncol):
    return [op(it, c) for c in range(ncol) for it in items]


def _by_item(items, op, ncol):
    return [op(it, c) for it in items for c in range(ncol)]


def _run(ops):
    for f in ops:
        f(None)


def _dot(a, b):
    return jnp.dot(a, b, preferred_element_type=F32)


def _bf(words):
    return pltpu.bitcast(words, BF16)


def _lo(w):
    return pltpu.bitcast(w << 16, F32)


def _hi(w):
    return pltpu.bitcast(w & jnp.uint32(0xFFFF0000), F32)


def _sublane_sum(t):
    t = t + pltpu.roll(t, 4, 0)
    t = t + pltpu.roll(t, 2, 0)
    return t + pltpu.roll(t, 1, 0)


def _col_bcast(row):
    return pltpu.bitcast(jnp.broadcast_to(row, (L, L)).T, U32)


def _round_bf16(x):
    return x.astype(BF16).astype(F32)


def _stats(xt):
    x = jnp.concatenate(xt, axis=1)
    mu = jnp.mean(x, axis=-1, keepdims=True)
    xc = x - mu
    var = jnp.mean(xc * xc, axis=-1, keepdims=True)
    return mu, jax.lax.rsqrt(var + EPS)


def _lhs16(xt):
    return [jnp.concatenate([x, jnp.ones_like(x)], axis=0).astype(BF16) for x in xt]


def _acc(d, k, v):
    d[k] = v if d.get(k) is None else d[k] + v
    return d[k]


def _kernel(x_hbm, wr_hbm, wq_hbm, wuk_hbm, ckv_hbm, wuv_hbm, wg_hbm, wu_hbm,
            wo_hbm, wd_hbm,
            o_ref,
            x_v, wr_v, wq_l, wuk_l, ckv_l, wuv_l, wg_l, wu_l, wo_l, wd_l,
            WQ32, WUKT32, CKV32, CKT32, WUV32, WG32, WU32, WO32, WD32,
            CSQ, CSG, CSU, XE, XO, sems):
    sem_ids = iter(range(64))

    def copy(src, dst, sem=None):
        sem = next(sem_ids) if sem is None else sem
        c = pltpu.make_async_copy(src, dst, sems.at[sem])
        c.start()
        return c

    c_wq = copy(wq_hbm, wq_l)
    s_small = next(sem_ids)
    c_small = [copy(x_hbm, x_v, s_small), copy(wr_hbm, wr_v, s_small)]
    c_wuk = copy(wuk_hbm, wuk_l)
    c_ckv = copy(ckv_hbm, ckv_l)
    c_wuv = copy(wuv_hbm, wuv_l)
    c_wg = copy(wg_hbm, wg_l)
    c_wu = copy(wu_hbm, wu_l)
    wo_rows = H * D // WO_CHUNKS
    c_wo = [copy(wo_hbm.at[pl.ds(c * wo_rows, wo_rows)],
                 wo_l.at[pl.ds(c * wo_rows, wo_rows)]) for c in range(WO_CHUNKS)]
    c_wd = []
    for (f0, f1) in WD_CHUNKS:
        r0, r1 = f0 * L, min(f1 * L, FF)
        c_wd.append(copy(wd_hbm.at[pl.ds(r0, r1 - r0)], wd_l.at[pl.ds(r0, r1 - r0)]))

    def swap_heads(src, dst32, rows):
        ch = 64

        def body(i, carry):
            w = src[pl.ds(pl.multiple_of(i * ch, ch), ch)]
            dst32[:, pl.ds(pl.multiple_of(i * (ch // 2), ch // 2), ch // 2), :] = (
                pltpu.bitcast(jnp.swapaxes(w, 0, 1), U32))
            return carry
        jax.lax.fori_loop(0, rows // ch, body, 0)

    def make_wukt():
        def body(i, carry):
            w = wuk_l[pl.ds(pl.multiple_of(i * L, L), L)]
            w = jnp.swapaxes(jnp.swapaxes(w, 0, 1), 1, 2)
            WUKT32[:, pl.ds(pl.multiple_of(i * W2, W2), W2), :] = pltpu.bitcast(w, U32)
            return carry
        jax.lax.fori_loop(0, CT, body, 0)

    def make_ck():
        def body(kt, carry):
            w = ckv_l[pl.ds(pl.multiple_of(kt * L, L), L), :]
            CKT32[kt] = pltpu.bitcast(w.T, U32)
            for ct in range(CT):
                CKV32[ct, pl.ds(pl.multiple_of(kt * W2, W2), W2), :] = pltpu.bitcast(
                    w[:, ct * L:(ct + 1) * L], U32)
            return carry
        jax.lax.fori_loop(0, KT, body, 0)

    def make_wgu(src, dst32):
        def body(ft, carry):
            w = src[pl.ds(pl.multiple_of(ft * L, L), L), :]
            dst32[ft] = pltpu.bitcast(w.T, U32)
            return carry
        jax.lax.fori_loop(0, FT - 1, body, 0)
        w = src[(FT - 1) * L:FF, :]
        w = jnp.concatenate([w, jnp.zeros((L - F_TAIL, M), BF16)], axis=0)
        dst32[FT - 1] = pltpu.bitcast(w.T, U32)

    def make_cols(src, dst32, r0, rows):
        for nt in range(MT):
            dst32[nt, r0 // 2:(r0 + rows) // 2, :] = pltpu.bitcast(
                src[r0:r0 + rows, nt * L:(nt + 1) * L], U32)

    sub = jax.lax.broadcasted_iota(jnp.int32, (R, L), 0)
    zero_v = []

    def link(a, dep):
        if dep is None:
            return a
        z = pltpu.bitcast(dep, U32) & zero_v[0]
        a32 = pltpu.bitcast(a, U32)
        return pltpu.bitcast(a32 | z[:a32.shape[0]], a.dtype)

    def make_xb(xt):
        for t in range(MT):
            w = _col_bcast(xt[t].astype(BF16)[0:1])
            XE[t * W2:(t + 1) * W2, :] = _lo(w)
            XO[t * W2:(t + 1) * W2, :] = _hi(w)

    def tile(ref32, lead, t):
        return _bf(ref32[lead, t * W2:(t + 1) * W2, :])

    def vpu_matvec_step(accs, ref_keys, s, dep):
        xe = link(XE[s * R:(s + 1) * R, :], dep)
        xo = XO[s * R:(s + 1) * R, :]
        for ref32, lead in ref_keys:
            w = ref32[lead, s * R:(s + 1) * R, :]
            _acc(accs, (id(ref32), lead), _lo(w) * xe + _hi(w) * xo)

    def attention(xt, first):
        mu, rstd = _stats(xt)
        lhs = _lhs16(xt)
        qscale = rstd * (D ** -0.5)
        nvq = 0 if first else VQ_HEADS
        nvo = 0 if first else VO_HEADS
        if first:
            c_wq.wait()
            swap_heads(wq_l, WQ32, M)
            c_wuk.wait()
            make_wukt()

        oq, qh, qa = {}, {}, {}

        def q_op(h, t):
            def f(dep):
                p = _dot(link(lhs[t], dep), tile(WQ32, h, t))
                o = _acc(oq, h, p)
                if t == MT - 1:
                    if first and h >= H - VQ_HEADS:
                        CSQ[h] = o[R:]
                    qh[h] = ((o[:R] - mu * o[R:]) * qscale).astype(BF16)
                return p[:R]
            return f

        def qabs_op(h, ct):
            def f(dep):
                g, i = divmod(h, R)
                t = _dot(qh[h], tile(WUKT32, h, ct))
                qa[g, ct] = t if (g, ct) not in qa else jnp.where(sub == i, t, qa[g, ct])
                return t
            f.ready = lambda: h in qh
            return f

        na = H - nvq
        edge = min(EDGE, na)

        def q_produce(h):
            if h == 0:
                return _by_column(range(edge), q_op, MT)
            return [] if h < edge else _by_item([h], q_op, MT)

        def q_consume(h):
            if h >= H - EDGE:
                return _by_column(range(H - EDGE, H), qabs_op, CT) if h == H - 1 else []
            return _by_item([h], qabs_op, CT)

        ms = _skewed(na, max(SKEW_Q, edge), q_produce, q_consume)
        for h in range(na, H):
            ms += q_consume(h)
        qacc = {}

        def q_vstep(hs, s):
            def f(dep):
                vpu_matvec_step(qacc, [(WQ32, h) for h in hs], s, dep)
                if s == M // 16 - 1:
                    for h in hs:
                        t = _sublane_sum(qacc[id(WQ32), h])
                        qh[h] = ((t - mu * CSQ[h]) * qscale).astype(BF16)
                return qacc[id(WQ32), hs[0]]
            return f

        if nvq:
            make_xb(xt)
        vs = [q_vstep(list(range(h0, min(H, h0 + VQ_GROUP))), s)
              for h0 in range(na, H, VQ_GROUP) for s in range(M // 16)]
        _cosched(ms, vs, P1_CFG)
        qabs = [jnp.concatenate([qa[g, ct] for g in range(H // R)], axis=0).astype(BF16)
                for ct in range(CT)]

        if first:
            c_ckv.wait()
            make_ck()
        nch = KT // KCHUNK
        sc, ps, lats = {}, {}, {}
        mxs, lss = [None] * nch, [None] * nch

        def score_op(kt, ct):
            def f(dep):
                _acc(sc, kt, _dot(qabs[ct], tile(CKT32, kt, ct)))
                j = kt // KCHUNK
                if ct == CT - 1 and kt == (j + 1) * KCHUNK - 1:
                    kts = range(j * KCHUNK, (j + 1) * KCHUNK)
                    mx = sc[kts[0]]
                    for k in kts[1:]:
                        mx = jnp.maximum(mx, sc[k])
                    mx = jnp.max(mx, axis=-1, keepdims=True)
                    lsum = None
                    for k in kts:
                        e = jnp.exp(sc[k] - mx)
                        lsum = e if lsum is None else lsum + e
                        ps[k] = e.astype(BF16)
                    mxs[j], lss[j] = mx, lsum
            return f

        def lat_op(kt, ct):
            def f(dep):
                _acc(lats, (kt // KCHUNK, ct), _dot(ps[kt], tile(CKV32, ct, kt)))
            return f

        def s_produce(j):
            kts = list(range(j * KCHUNK, (j + 1) * KCHUNK))
            if j == 0:
                return (_by_column(kts[:EDGE], score_op, CT)
                        + _by_item(kts[EDGE:], score_op, CT))
            return _by_item(kts, score_op, CT)

        def s_consume(j):
            return _by_column(range(j * KCHUNK, (j + 1) * KCHUNK), lat_op, CT)

        _run(_skewed(nch, SKEW_S, s_produce, s_consume))
        m = mxs[0]
        for t in mxs[1:]:
            m = jnp.maximum(m, t)
        alpha = [jnp.exp(t - m) for t in mxs]
        lsum = alpha[0] * lss[0]
        for a, t in zip(alpha[1:], lss[1:]):
            lsum = lsum + a * t
        inv = 1.0 / jnp.sum(lsum, axis=-1, keepdims=True)
        alpha = [a * inv for a in alpha]
        latg = {}
        for ct in range(CT):
            t = alpha[0] * lats[0, ct]
            for j in range(1, nch):
                t = t + alpha[j] * lats[j, ct]
            for g in range(H // R):
                latg[g, ct] = t[g * R:(g + 1) * R].astype(BF16)

        if first:
            c_wuv.wait()
            swap_heads(wuv_l, WUV32, DC)
        cacc, cbs, o = {}, {}, {}

        def ctx_op(h, ct):
            def f(dep):
                g, i = divmod(h, R)
                p = _dot(link(latg[g, ct], dep), tile(WUV32, h, ct))
                c = _acc(cacc, h, p)
                if ct == CT - 1:
                    cbs[h] = jnp.broadcast_to(c[i:i + 1], (R, D)).astype(BF16)
                return p
            return f

        def out_op(h, nt):
            def f(dep):
                t = _dot(cbs[h], tile(WO32, nt, h))
                _acc(o, nt, t)
                return t
            return f

        if first:
            _run(_by_item(range(H), ctx_op, CT))
            c_wg.wait()
            make_wgu(wg_l, WG32)
            c_wu.wait()
            make_wgu(wu_l, WU32)
            hpc = H // WO_CHUNKS
            for c in range(WO_CHUNKS):
                c_wo[c].wait()
                make_cols(wo_l, WO32, c * wo_rows, wo_rows)
                _run(_by_item(range(c * hpc, (c + 1) * hpc), out_op, MT))
            return [_round_bf16(xt[nt] + o[nt]) for nt in range(MT)]

        ms = _by_column(range(EDGE), ctx_op, CT) + _by_item(range(EDGE, nvo), ctx_op, CT)
        h0 = max(nvo, EDGE)

        def o_produce(i):
            return _by_item([h0 + i], ctx_op, CT)

        def o_consume(h):
            if h >= H - EDGE:
                return _by_column(range(H - EDGE, H), out_op, MT) if h == H - 1 else []
            return _by_item([h], out_op, MT)

        for step in range(H - h0 + SKEW_O):
            if step < H - h0:
                ms += o_produce(step)
            if step >= SKEW_O:
                ms += o_consume(h0 + step - SKEW_O)
        for h in range(nvo, h0):
            ms += o_consume(h)
        cw, ov = {}, {}

        def xlu_op(h):
            def f(dep):
                cw[h] = _col_bcast(cbs[h][0:1])
                return pltpu.bitcast(cw[h][:R], F32)
            f.ready = lambda: h in cbs
            return f

        def o_vstep(h, k):
            def f(dep):
                w = cw[h][k * R:(k + 1) * R]
                ce, co = link(_lo(w), dep), _hi(w)
                r0 = h * W2 + k * R
                for nt in range(MT):
                    w = WO32[nt, r0:r0 + R, :]
                    _acc(ov, nt, _lo(w) * ce + _hi(w) * co)
                return ov[0]
            return f

        vs = [xlu_op(h) for h in range(min(XLU_AHEAD, nvo))]
        for h in range(nvo):
            if h + XLU_AHEAD < nvo:
                vs.append(xlu_op(h + XLU_AHEAD))
            vs += [o_vstep(h, k) for k in range(L // 16)]
        _cosched(ms, vs, P3_CFG)
        if nvo:
            o = {nt: o[nt] + _sublane_sum(ov[nt]) for nt in range(MT)}
        return [_round_bf16(xt[nt] + o[nt]) for nt in range(MT)]

    def ffn(xt, first):
        mu, rstd = _stats(xt)
        lhs = _lhs16(xt)
        xn = [(x - mu) * rstd for x in xt]
        wr = wr_v[...].reshape(1, M).astype(F32)
        r = jnp.sum(jnp.concatenate(xn, axis=1) * wr, axis=-1, keepdims=True)
        gate = jax.nn.sigmoid(r)
        nvf = 0 if first else VF_TILES
        pre, acts, y = {}, {}, {}

        def finish(ft):
            g, u = pre[ft, 0] * rstd, pre[ft, 1] * rstd
            acts[ft] = (g * jax.nn.sigmoid(g) * u).astype(BF16)

        def gu_op(key, t):
            ft, which = key

            def f(dep):
                p = _dot(link(lhs[t], dep), tile((WG32, WU32)[which], ft, t))
                o = _acc(pre, key, p)
                if t == MT - 1:
                    if first and ft < VF_TILES:
                        (CSG, CSU)[which][ft] = o[R:]
                    pre[key] = o[:R] - mu * o[R:]
                    if which == 1:
                        finish(ft)
                return p[:R]
            return f

        def dn_op(ft, nt):
            def f(dep):
                rows = L if ft < FT - 1 else F_TAIL
                a = acts[ft] if rows == L else acts[ft][:, :rows]
                if first:
                    w = wd_l[ft * L:ft * L + rows, nt * L:(nt + 1) * L]
                else:
                    w = _bf(WD32[nt, ft * W2:ft * W2 + rows // 2, :])
                t = _dot(a, w)
                _acc(y, nt, t)
                return t
            f.ready = lambda: ft in acts
            return f

        def gu_keys(fts):
            return [(ft, which) for ft in fts for which in range(2)]

        if first:
            _run(_by_item(gu_keys(range(FT)), gu_op, MT))
            for c, (f0, f1) in enumerate(WD_CHUNKS):
                c_wd[c].wait()
                if c == len(WD_CHUNKS) - 1:
                    _run(_by_column(range(f0, f1), dn_op, MT))
                else:
                    _run(_by_item(range(f0, f1), dn_op, MT))
        else:
            mt = list(range(nvf, FT))
            last = (mt + list(range(nvf)))[-2:] if nvf < 2 else list(range(nvf))[-2:]

            def g_produce(i):
                if i == 0:
                    return _by_column(gu_keys(mt[:2]), gu_op, MT)
                return [] if i == 1 else _by_item(gu_keys([mt[i]]), gu_op, MT)

            def g_consume(ft):
                if ft in last:
                    return _by_column(last, dn_op, MT) if ft == last[-1] else []
                return _by_item([ft], dn_op, MT)

            ms = _skewed(len(mt), SKEW_F, g_produce, lambda i: g_consume(mt[i]))
            for ft in range(nvf):
                ms += g_consume(ft)
            facc = {}

            def f_vstep(fts, s):
                def f(dep):
                    keys = [(w, ft) for ft in fts for w in (WG32, WU32)]
                    vpu_matvec_step(facc, keys, s, dep)
                    if s == M // 16 - 1:
                        for ft in fts:
                            for wh, (w, cs) in enumerate(((WG32, CSG), (WU32, CSU))):
                                pre[ft, wh] = _sublane_sum(facc[id(w), ft]) - mu * cs[ft]
                            finish(ft)
                    return facc[id(WG32), fts[0]]
                return f

            if nvf:
                make_xb(xt)
            vs = [f_vstep(list(range(f0, min(nvf, f0 + VF_GROUP))), s)
                  for f0 in range(0, nvf, VF_GROUP) for s in range(M // 16)]
            _cosched(ms, vs, P4_CFG)
        return [_round_bf16(xt[nt] + xn[nt] + y[nt] * gate) for nt in range(MT)]

    for c in c_small:
        c.wait()
    x = jnp.broadcast_to(x_v[...].astype(F32), (R, M))
    zero_v.append(pltpu.bitcast(x[:, :L], U32) & jnp.uint32(0xFFFF))
    xt = [x[:, t * L:(t + 1) * L] for t in range(MT)]
    xt = attention(xt, True)
    xt = ffn(xt, True)
    if N_LAYERS > 1:
        make_cols(wd_l, WD32, 0, FF)
        xt = attention(xt, False)
        xt = ffn(xt, False)
    o_ref[...] = jnp.concatenate(xt, axis=1)[0:1].astype(o_ref.dtype)


@jax.jit
def pallas_interleave_layers__compressed_kv_cla__moe_arch_mod__decode_kernel(
    A_x: jax.Array,
    A_c_kv: jax.Array,
    A_w_q: jax.Array,
    A_w_uk: jax.Array,
    A_w_uv: jax.Array,
    A_w_o: jax.Array,
    B_x: jax.Array,
    B_w_r: jax.Array,
    B_w_gate: jax.Array,
    B_w_up: jax.Array,
    B_w_down: jax.Array,
):
    del B_x
    args = (
        A_x.reshape(1, M),
        B_w_r,
        A_w_q,
        A_w_uk,
        A_c_kv.reshape(SK, DC),
        A_w_uv,
        B_w_gate.T,
        B_w_up.T,
        A_w_o.reshape(H * D, M),
        B_w_down,
    )
    n_sems = 7 + WO_CHUNKS + len(WD_CHUNKS)
    scratch = [
        pltpu.VMEM((1, M), BF16),
        pltpu.VMEM((M,), BF16),
        pltpu.VMEM((M, H, D), BF16),
        pltpu.VMEM((DC, H, D), BF16),
        pltpu.VMEM((SK, DC), BF16),
        pltpu.VMEM((DC, H, D), BF16),
        pltpu.VMEM((FF, M), BF16),
        pltpu.VMEM((FF, M), BF16),
        pltpu.VMEM((H * D, M), BF16),
        pltpu.VMEM((FF, M), BF16),
        pltpu.VMEM((H, M // 2, D), U32),
        pltpu.VMEM((H, DC // 2, L), U32),
        pltpu.VMEM((CT, SK // 2, L), U32),
        pltpu.VMEM((KT, DC // 2, L), U32),
        pltpu.VMEM((H, DC // 2, D), U32),
        pltpu.VMEM((FT, M // 2, L), U32),
        pltpu.VMEM((FT, M // 2, L), U32),
        pltpu.VMEM((MT, H * D // 2, L), U32),
        pltpu.VMEM((MT, FF // 2, L), U32),
        pltpu.VMEM((H, R, L), F32),
        pltpu.VMEM((FT, R, L), F32),
        pltpu.VMEM((FT, R, L), F32),
        pltpu.VMEM((M // 2, L), F32),
        pltpu.VMEM((M // 2, L), F32),
        pltpu.SemaphoreType.DMA((n_sems,)),
    ]
    out = pl.pallas_call(
        _kernel,
        out_shape=jax.ShapeDtypeStruct((1, M), A_x.dtype),
        in_specs=[pl.BlockSpec(memory_space=pl.ANY)] * len(args),
        out_specs=pl.BlockSpec(memory_space=pltpu.VMEM),
        scratch_shapes=scratch,
        compiler_params=pltpu.CompilerParams(
            vmem_limit_bytes=100 * 1024 * 1024,
            disable_semaphore_checks=True),
        name="mla_moe_decode",
    )(*args)
    return out.reshape(1, 1, M)
```

```python
import jax
import jax.numpy as jnp
import jax.experimental.pallas as pl
import jax.experimental.pallas.tpu as pltpu

F32 = jnp.float32
BF16 = jnp.bfloat16
U32 = jnp.uint32

H = 32
D = 128
M = 640
DC = 512
SK = 4096
FF = 1728
EPS = 1e-5
R = 8
L = 128
W2 = L // 2

MT = M // L
CT = DC // L
KT = SK // L
FT = -(-FF // L)
F_TAIL = FF - (FT - 1) * L
KCHUNK = 8
WO_CHUNKS = 4

N_LAYERS = 2
SKEW_S = 1
SKEW_O = 6
SKEW_F = 5
EDGE = 4

VA_HEADS = 10
P1_CFG = (40, 1.0, 2, 18, 1, 70)
VO_HEADS = 16
P3_CFG = (50, 0.95, 2, 18, 1, 80)
XLU_AHEAD = 2
VF_TILES = 4
VF_GROUP = 2
P4_CFG = (20, 0.7, 2, 18, 1, 0)


def _always():
    return True


def _cosched(ms, vs, cfg):
    vstart, vrate, lag_v, lag_m, nlink, lstart = cfg
    mres, vres = [], []
    j = 0

    def emit_v(dep):
        nonlocal j
        vres.append(vs[j](dep))
        j += 1

    for i, m in enumerate(ms):
        while not getattr(m, "ready", _always)():
            emit_v(None)
        dep = None
        if len(vres) > lag_v and i % nlink == 0 and j < len(vs) and i >= lstart:
            dep = vres[-1 - lag_v]
        mres.append(m(dep))
        while (j < len(vs) and j < (i + 1 - vstart) * vrate
               and getattr(vs[j], "ready", _always)()):
            emit_v(mres[-1 - lag_m] if (len(mres) > lag_m and j % 2 == 0) else None)
    while j < len(vs):
        emit_v(None)


def _skewed(n, skew, produce, consume):
    out = []
    for step in range(n + skew):
        if step < n:
            out += produce(step)
        if step >= skew:
            out += consume(step - skew)
    return out


def _by_column(items, op, ncol):
    return [op(it, c) for c in range(ncol) for it in items]


def _by_item(items, op, ncol):
    return [op(it, c) for it in items for c in range(ncol)]


def _run(ops):
    for f in ops:
        f(None)


def _dot(a, b):
    return jnp.dot(a, b, preferred_element_type=F32)


def _bf(words):
    return pltpu.bitcast(words, BF16)


def _lo(w):
    return pltpu.bitcast(w << 16, F32)


def _hi(w):
    return pltpu.bitcast(w & jnp.uint32(0xFFFF0000), F32)


def _sublane_sum(t):
    t = t + pltpu.roll(t, 4, 0)
    t = t + pltpu.roll(t, 2, 0)
    return t + pltpu.roll(t, 1, 0)


def _col_bcast(row):
    return pltpu.bitcast(jnp.broadcast_to(row, (L, L)).T, U32)


def _round_bf16(x):
    return x.astype(BF16).astype(F32)


def _stats(xt):
    x = jnp.concatenate(xt, axis=1)
    mu = jnp.mean(x, axis=-1, keepdims=True)
    xc = x - mu
    var = jnp.mean(xc * xc, axis=-1, keepdims=True)
    return mu, jax.lax.rsqrt(var + EPS)


def _lhs16(xt):
    return [jnp.concatenate([x, jnp.ones_like(x)], axis=0).astype(BF16) for x in xt]


def _acc(d, k, v):
    d[k] = v if d.get(k) is None else d[k] + v
    return d[k]


def _kernel(x_hbm, wr_hbm, wq_hbm, wuk_hbm, ckv_hbm, wuv_hbm, wg_hbm, wu_hbm,
            wo_hbm, wd_hbm,
            o_ref,
            x_v, wr_v, wq_l, wuk_l, ckv_l, wuv_l, wg_l, wu_l, wo_l, wd_l,
            WQ32, WUKT32, CKV32, CKT32, WUV32, WG32, WU32, WO32, WD32,
            CSG, CSU, XE, XO, sems):
    sem_ids = iter(range(64))

    def copy(src, dst, sem=None):
        sem = next(sem_ids) if sem is None else sem
        c = pltpu.make_async_copy(src, dst, sems.at[sem])
        c.start()
        return c

    c_wq = copy(wq_hbm, wq_l)
    s_small = next(sem_ids)
    c_small = [copy(x_hbm, x_v, s_small), copy(wr_hbm, wr_v, s_small)]
    c_wuk = copy(wuk_hbm, wuk_l)
    c_ckv = copy(ckv_hbm, ckv_l)
    c_wuv = copy(wuv_hbm, wuv_l)
    c_wg = copy(wg_hbm, wg_l)
    c_wu = copy(wu_hbm, wu_l)
    wo_rows = H * D // WO_CHUNKS
    c_wo = [copy(wo_hbm.at[pl.ds(c * wo_rows, wo_rows)],
                 wo_l.at[pl.ds(c * wo_rows, wo_rows)]) for c in range(WO_CHUNKS)]
    c_wd = [copy(wd_hbm.at[:, pl.ds(nt * L, L)], wd_l.at[nt]) for nt in range(MT)]

    def swap_heads(src, dst32, rows):
        ch = 64

        def body(i, carry):
            w = src[pl.ds(pl.multiple_of(i * ch, ch), ch)]
            dst32[:, pl.ds(pl.multiple_of(i * (ch // 2), ch // 2), ch // 2), :] = (
                pltpu.bitcast(jnp.swapaxes(w, 0, 1), U32))
            return carry
        jax.lax.fori_loop(0, rows // ch, body, 0)

    def make_wukt():
        def body(i, carry):
            w = wuk_l[pl.ds(pl.multiple_of(i * L, L), L)]
            w = jnp.swapaxes(jnp.swapaxes(w, 0, 1), 1, 2)
            WUKT32[:, pl.ds(pl.multiple_of(i * W2, W2), W2), :] = pltpu.bitcast(w, U32)
            return carry
        jax.lax.fori_loop(0, CT, body, 0)

    def make_ck():
        def body(kt, carry):
            w = ckv_l[pl.ds(pl.multiple_of(kt * L, L), L), :]
            CKT32[kt] = pltpu.bitcast(w.T, U32)
            for ct in range(CT):
                CKV32[ct, pl.ds(pl.multiple_of(kt * W2, W2), W2), :] = pltpu.bitcast(
                    w[:, ct * L:(ct + 1) * L], U32)
            return carry
        jax.lax.fori_loop(0, KT, body, 0)

    def make_wgu(src, dst32):
        def body(ft, carry):
            w = src[pl.ds(pl.multiple_of(ft * L, L), L), :]
            dst32[ft] = pltpu.bitcast(w.T, U32)
            return carry
        jax.lax.fori_loop(0, FT - 1, body, 0)
        w = src[(FT - 1) * L:FF, :]
        w = jnp.concatenate([w, jnp.zeros((L - F_TAIL, M), BF16)], axis=0)
        dst32[FT - 1] = pltpu.bitcast(w.T, U32)

    def make_cols(src, dst32, r0, rows):
        for nt in range(MT):
            dst32[nt, r0 // 2:(r0 + rows) // 2, :] = pltpu.bitcast(
                src[r0:r0 + rows, nt * L:(nt + 1) * L], U32)

    sub = jax.lax.broadcasted_iota(jnp.int32, (R, L), 0)
    zero_v = []

    def link(a, dep):
        if dep is None:
            return a
        z = pltpu.bitcast(dep, U32) & zero_v[0]
        a32 = pltpu.bitcast(a, U32)
        return pltpu.bitcast(a32 | z[:a32.shape[0]], a.dtype)

    def make_xb(xt):
        for t in range(MT):
            w = _col_bcast(xt[t].astype(BF16)[0:1])
            XE[t * W2:(t + 1) * W2, :] = _lo(w)
            XO[t * W2:(t + 1) * W2, :] = _hi(w)

    def tile(ref32, lead, t):
        return _bf(ref32[lead, t * W2:(t + 1) * W2, :])

    def vpu_matvec_step(accs, ref_keys, s, dep):
        xe = link(XE[s * R:(s + 1) * R, :], dep)
        xo = XO[s * R:(s + 1) * R, :]
        for ref32, lead in ref_keys:
            w = ref32[lead, s * R:(s + 1) * R, :]
            _acc(accs, (id(ref32), lead), _lo(w) * xe + _hi(w) * xo)

    def q_partial(oq, x_tile, t):
        lhs = _lhs16([x_tile])[0]

        def op(h):
            def f(dep):
                p = _dot(link(lhs, dep), tile(WQ32, h, t))
                _acc(oq, h, p)
                return p[:R]
            return f
        return [op(h) for h in range(H)]

    def attention(xt, first, oq):
        mu, rstd = _stats(xt)
        qscale = rstd * (D ** -0.5)
        nva = 0 if first else VA_HEADS
        nvo = 0 if first else VO_HEADS
        if first:
            c_wq.wait()
            swap_heads(wq_l, WQ32, M)
            for t in range(MT - 1):
                _run(q_partial(oq, xt[t], t))
            c_wuk.wait()
            make_wukt()

        qh, qa = {}, {}

        def q_last(h, op):
            def f(dep):
                r = op(dep)
                o = oq[h]
                qh[h] = ((o[:R] - mu * o[R:]) * qscale).astype(BF16)
                return r
            return f

        def put_qa(h, ct, t):
            g, i = divmod(h, R)
            qa[g, ct] = t if (g, ct) not in qa else jnp.where(sub == i, t, qa[g, ct])

        def qabs_op(h, ct):
            def f(dep):
                t = _dot(qh[h], tile(WUKT32, h, ct))
                put_qa(h, ct, t)
                return t
            return f

        ms = [q_last(h, op) for h, op in enumerate(q_partial(oq, xt[MT - 1], MT - 1))]
        ms += _by_item(range(nva, H - EDGE), qabs_op, CT)
        ms += _by_column(range(H - EDGE, H), qabs_op, CT)
        qw, aacc = {}, {}

        def qxlu_op(h):
            def f(dep):
                qw[h] = _col_bcast(qh[h][0:1])
                return pltpu.bitcast(qw[h][:R], F32)
            f.ready = lambda: h in qh
            return f

        def qa_vstep(h, k):
            def f(dep):
                w = qw[h][k * R:(k + 1) * R]
                ce, co = link(_lo(w), dep), _hi(w)
                for ct in range(CT):
                    r0 = ct * W2 + k * R
                    w = WUKT32[h, r0:r0 + R, :]
                    _acc(aacc, (h, ct), _lo(w) * ce + _hi(w) * co)
                if k == L // 16 - 1:
                    for ct in range(CT):
                        put_qa(h, ct, _sublane_sum(aacc[h, ct]))
                return aacc[h, 0]
            return f

        vs = [qxlu_op(h) for h in range(min(XLU_AHEAD, nva))]
        for h in range(nva):
            if h + XLU_AHEAD < nva:
                vs.append(qxlu_op(h + XLU_AHEAD))
            vs += [qa_vstep(h, k) for k in range(L // 16)]
        _cosched(ms, vs, P1_CFG)
        qabs = [jnp.concatenate([qa[g, ct] for g in range(H // R)], axis=0).astype(BF16)
                for ct in range(CT)]

        if first:
            c_ckv.wait()
            make_ck()
        nch = KT // KCHUNK
        sc, ps, lats = {}, {}, {}
        mxs, lss = [None] * nch, [None] * nch

        def score_op(kt, ct):
            def f(dep):
                _acc(sc, kt, _dot(qabs[ct], tile(CKT32, kt, ct)))
                j = kt // KCHUNK
                if ct == CT - 1 and kt == (j + 1) * KCHUNK - 1:
                    kts = range(j * KCHUNK, (j + 1) * KCHUNK)
                    mx = sc[kts[0]]
                    for k in kts[1:]:
                        mx = jnp.maximum(mx, sc[k])
                    mx = jnp.max(mx, axis=-1, keepdims=True)
                    lsum = None
                    for k in kts:
                        e = jnp.exp(sc[k] - mx)
                        lsum = e if lsum is None else lsum + e
                        ps[k] = e.astype(BF16)
                    mxs[j], lss[j] = mx, lsum
            return f

        def lat_op(kt, ct):
            def f(dep):
                _acc(lats, (kt // KCHUNK, ct), _dot(ps[kt], tile(CKV32, ct, kt)))
            return f

        def s_produce(j):
            kts = list(range(j * KCHUNK, (j + 1) * KCHUNK))
            if j == 0:
                return (_by_column(kts[:EDGE], score_op, CT)
                        + _by_item(kts[EDGE:], score_op, CT))
            return _by_item(kts, score_op, CT)

        def s_consume(j):
            return _by_column(range(j * KCHUNK, (j + 1) * KCHUNK), lat_op, CT)

        _run(_skewed(nch, SKEW_S, s_produce, s_consume))
        m = mxs[0]
        for t in mxs[1:]:
            m = jnp.maximum(m, t)
        alpha = [jnp.exp(t - m) for t in mxs]
        lsum = alpha[0] * lss[0]
        for a, t in zip(alpha[1:], lss[1:]):
            lsum = lsum + a * t
        inv = 1.0 / jnp.sum(lsum, axis=-1, keepdims=True)
        alpha = [a * inv for a in alpha]
        latg = {}
        for ct in range(CT):
            t = alpha[0] * lats[0, ct]
            for j in range(1, nch):
                t = t + alpha[j] * lats[j, ct]
            for g in range(H // R):
                latg[g, ct] = t[g * R:(g + 1) * R].astype(BF16)

        if first:
            c_wuv.wait()
            swap_heads(wuv_l, WUV32, DC)
        cacc, cbs, o = {}, {}, {}

        def ctx_op(h, ct):
            def f(dep):
                g, i = divmod(h, R)
                p = _dot(link(latg[g, ct], dep), tile(WUV32, h, ct))
                c = _acc(cacc, h, p)
                if ct == CT - 1:
                    cbs[h] = jnp.broadcast_to(c[i:i + 1], (R, D)).astype(BF16)
                return p
            return f

        def out_op(h, nt):
            def f(dep):
                t = _dot(cbs[h], tile(WO32, nt, h))
                _acc(o, nt, t)
                return t
            return f

        if first:
            _run(_by_item(range(H), ctx_op, CT))
            c_wg.wait()
            make_wgu(wg_l, WG32)
            c_wu.wait()
            make_wgu(wu_l, WU32)
            hpc = H // WO_CHUNKS
            for c in range(WO_CHUNKS):
                c_wo[c].wait()
                make_cols(wo_l, WO32, c * wo_rows, wo_rows)
                _run(_by_item(range(c * hpc, (c + 1) * hpc), out_op, MT))
            return [_round_bf16(xt[nt] + o[nt]) for nt in range(MT)]

        ms = _by_column(range(EDGE), ctx_op, CT) + _by_item(range(EDGE, nvo), ctx_op, CT)
        h0 = max(nvo, EDGE)

        def o_produce(i):
            return _by_item([h0 + i], ctx_op, CT)

        def o_consume(h):
            if h >= H - EDGE:
                return _by_column(range(H - EDGE, H), out_op, MT) if h == H - 1 else []
            return _by_item([h], out_op, MT)

        for step in range(H - h0 + SKEW_O):
            if step < H - h0:
                ms += o_produce(step)
            if step >= SKEW_O:
                ms += o_consume(h0 + step - SKEW_O)
        for h in range(nvo, h0):
            ms += o_consume(h)
        cw, ov = {}, {}

        def xlu_op(h):
            def f(dep):
                cw[h] = _col_bcast(cbs[h][0:1])
                return pltpu.bitcast(cw[h][:R], F32)
            f.ready = lambda: h in cbs
            return f

        def o_vstep(h, k):
            def f(dep):
                w = cw[h][k * R:(k + 1) * R]
                ce, co = link(_lo(w), dep), _hi(w)
                r0 = h * W2 + k * R
                for nt in range(MT):
                    w = WO32[nt, r0:r0 + R, :]
                    _acc(ov, nt, _lo(w) * ce + _hi(w) * co)
                return ov[0]
            return f

        vs = [xlu_op(h) for h in range(min(XLU_AHEAD, nvo))]
        for h in range(nvo):
            if h + XLU_AHEAD < nvo:
                vs.append(xlu_op(h + XLU_AHEAD))
            vs += [o_vstep(h, k) for k in range(L // 16)]
        _cosched(ms, vs, P3_CFG)
        if nvo:
            o = {nt: o[nt] + _sublane_sum(ov[nt]) for nt in range(MT)}
        return [_round_bf16(xt[nt] + o[nt]) for nt in range(MT)]

    def ffn(xt, first, oq_next=None):
        mu, rstd = _stats(xt)
        lhs = _lhs16(xt)
        xn = [(x - mu) * rstd for x in xt]
        wr = wr_v[...].reshape(1, M).astype(F32)
        r = jnp.sum(jnp.concatenate(xn, axis=1) * wr, axis=-1, keepdims=True)
        gate = jax.nn.sigmoid(r)
        nvf = 0 if first else VF_TILES
        pre, acts, y = {}, {}, {}

        def finish(ft):
            g, u = pre[ft, 0] * rstd, pre[ft, 1] * rstd
            acts[ft] = (g * jax.nn.sigmoid(g) * u).astype(BF16)

        def gu_op(key, t):
            ft, which = key

            def f(dep):
                p = _dot(link(lhs[t], dep), tile((WG32, WU32)[which], ft, t))
                o = _acc(pre, key, p)
                if t == MT - 1:
                    if first and ft < VF_TILES:
                        (CSG, CSU)[which][ft] = o[R:]
                    pre[key] = o[:R] - mu * o[R:]
                    if which == 1:
                        finish(ft)
                return p[:R]
            return f

        def dn_op(ft, nt):
            def f(dep):
                rows = L if ft < FT - 1 else F_TAIL
                a = acts[ft] if rows == L else acts[ft][:, :rows]
                if first:
                    w = wd_l[nt, ft * L:ft * L + rows, :]
                else:
                    w = _bf(WD32[nt, ft * W2:ft * W2 + rows // 2, :])
                t = _dot(a, w)
                _acc(y, nt, t)
                return t
            f.ready = lambda: ft in acts
            return f

        def gu_keys(fts):
            return [(ft, which) for ft in fts for which in range(2)]

        if first:
            _run(_by_item(gu_keys(range(FT)), gu_op, MT))
            out = []
            for nt in range(MT):
                c_wd[nt].wait()
                _run([dn_op(ft, nt) for ft in range(FT)])
                out.append(_round_bf16(xt[nt] + xn[nt] + y[nt] * gate))
                if nt < MT - 1 and oq_next is not None:
                    _run(q_partial(oq_next, out[nt], nt))
            return out
        else:
            mt = list(range(nvf, FT))
            last = (mt + list(range(nvf)))[-2:] if nvf < 2 else list(range(nvf))[-2:]

            def g_produce(i):
                if i == 0:
                    return _by_column(gu_keys(mt[:2]), gu_op, MT)
                return [] if i == 1 else _by_item(gu_keys([mt[i]]), gu_op, MT)

            def g_consume(ft):
                if ft in last:
                    return _by_column(last, dn_op, MT) if ft == last[-1] else []
                return _by_item([ft], dn_op, MT)

            ms = _skewed(len(mt), SKEW_F, g_produce, lambda i: g_consume(mt[i]))
            for ft in range(nvf):
                ms += g_consume(ft)
            facc = {}

            def f_vstep(fts, s):
                def f(dep):
                    keys = [(w, ft) for ft in fts for w in (WG32, WU32)]
                    vpu_matvec_step(facc, keys, s, dep)
                    if s == M // 16 - 1:
                        for ft in fts:
                            for wh, (w, cs) in enumerate(((WG32, CSG), (WU32, CSU))):
                                pre[ft, wh] = _sublane_sum(facc[id(w), ft]) - mu * cs[ft]
                            finish(ft)
                    return facc[id(WG32), fts[0]]
                return f

            if nvf:
                make_xb(xt)
            vs = [f_vstep(list(range(f0, min(nvf, f0 + VF_GROUP))), s)
                  for f0 in range(0, nvf, VF_GROUP) for s in range(M // 16)]
            _cosched(ms, vs, P4_CFG)
        return [_round_bf16(xt[nt] + xn[nt] + y[nt] * gate) for nt in range(MT)]

    for c in c_small:
        c.wait()
    x = jnp.broadcast_to(x_v[...].astype(F32), (R, M))
    zero_v.append(pltpu.bitcast(x[:, :L], U32) & jnp.uint32(0xFFFF))
    xt = [x[:, t * L:(t + 1) * L] for t in range(MT)]
    xt = attention(xt, True, {})
    oq2 = {}
    xt = ffn(xt, True, oq2 if N_LAYERS > 1 else None)
    if N_LAYERS > 1:
        for nt in range(MT):
            WD32[nt] = pltpu.bitcast(wd_l[nt], U32)
        xt = attention(xt, False, oq2)
        xt = ffn(xt, False)
    o_ref[...] = jnp.concatenate(xt, axis=1)[0:1].astype(o_ref.dtype)


@jax.jit
def pallas_interleave_layers__compressed_kv_cla__moe_arch_mod__decode_kernel(
    A_x: jax.Array,
    A_c_kv: jax.Array,
    A_w_q: jax.Array,
    A_w_uk: jax.Array,
    A_w_uv: jax.Array,
    A_w_o: jax.Array,
    B_x: jax.Array,
    B_w_r: jax.Array,
    B_w_gate: jax.Array,
    B_w_up: jax.Array,
    B_w_down: jax.Array,
):
    del B_x
    args = (
        A_x.reshape(1, M),
        B_w_r,
        A_w_q,
        A_w_uk,
        A_c_kv.reshape(SK, DC),
        A_w_uv,
        B_w_gate.T,
        B_w_up.T,
        A_w_o.reshape(H * D, M),
        B_w_down,
    )
    n_sems = 7 + WO_CHUNKS + MT
    scratch = [
        pltpu.VMEM((1, M), BF16),
        pltpu.VMEM((M,), BF16),
        pltpu.VMEM((M, H, D), BF16),
        pltpu.VMEM((DC, H, D), BF16),
        pltpu.VMEM((SK, DC), BF16),
        pltpu.VMEM((DC, H, D), BF16),
        pltpu.VMEM((FF, M), BF16),
        pltpu.VMEM((FF, M), BF16),
        pltpu.VMEM((H * D, M), BF16),
        pltpu.VMEM((MT, FF, L), BF16),
        pltpu.VMEM((H, M // 2, D), U32),
        pltpu.VMEM((H, DC // 2, L), U32),
        pltpu.VMEM((CT, SK // 2, L), U32),
        pltpu.VMEM((KT, DC // 2, L), U32),
        pltpu.VMEM((H, DC // 2, D), U32),
        pltpu.VMEM((FT, M // 2, L), U32),
        pltpu.VMEM((FT, M // 2, L), U32),
        pltpu.VMEM((MT, H * D // 2, L), U32),
        pltpu.VMEM((MT, FF // 2, L), U32),
        pltpu.VMEM((FT, R, L), F32),
        pltpu.VMEM((FT, R, L), F32),
        pltpu.VMEM((M // 2, L), F32),
        pltpu.VMEM((M // 2, L), F32),
        pltpu.SemaphoreType.DMA((n_sems,)),
    ]
    out = pl.pallas_call(
        _kernel,
        out_shape=jax.ShapeDtypeStruct((1, M), A_x.dtype),
        in_specs=[pl.BlockSpec(memory_space=pl.ANY)] * len(args),
        out_specs=pl.BlockSpec(memory_space=pltpu.VMEM),
        scratch_shapes=scratch,
        compiler_params=pltpu.CompilerParams(
            vmem_limit_bytes=100 * 1024 * 1024,
            disable_semaphore_checks=True),
        name="mla_moe_decode",
    )(*args)
    return out.reshape(1, 1, M)
```

```python
import jax
import jax.numpy as jnp
import jax.experimental.pallas as pl
import jax.experimental.pallas.tpu as pltpu

F32 = jnp.float32
BF16 = jnp.bfloat16
U32 = jnp.uint32

H = 32
D = 128
M = 640
DC = 512
SK = 4096
FF = 1728
EPS = 1e-5
R = 8
L = 128
W2 = L // 2

MT = M // L
CT = DC // L
KT = SK // L
FT = -(-FF // L)
F_TAIL = FF - (FT - 1) * L
KCHUNK = 8
WO_CHUNKS = 4

N_LAYERS = 2
SKEW_S = 1
SKEW_O = 6
SKEW_F = 5
EDGE = 4

VA_HEADS = 9
P1_CFG = (45, 0.9, 1, 18, 1, 55)
VO_HEADS = 16
P3_CFG = (50, 0.95, 2, 18, 1, 80)
XLU_AHEAD = 2
LINK_P1 = False
LINK_P3 = False
LINK_P4 = False
VF_TILES = 4
VF_GROUP = 2
P4_CFG = (20, 0.7, 2, 18, 1, 0)


def _always():
    return True


def _cosched(ms, vs, cfg):
    vstart, vrate, lag_v, lag_m, nlink, lstart = cfg
    mres, vres = [], []
    j = 0

    def emit_v(dep):
        nonlocal j
        vres.append(vs[j](dep))
        j += 1

    for i, m in enumerate(ms):
        while not getattr(m, "ready", _always)():
            emit_v(None)
        dep = None
        if len(vres) > lag_v and i % nlink == 0 and j < len(vs) and i >= lstart:
            dep = vres[-1 - lag_v]
        mres.append(m(dep))
        while (j < len(vs) and j < (i + 1 - vstart) * vrate
               and getattr(vs[j], "ready", _always)()):
            emit_v(mres[-1 - lag_m] if (len(mres) > lag_m and j % 2 == 0) else None)
    while j < len(vs):
        emit_v(None)


def _skewed(n, skew, produce, consume):
    out = []
    for step in range(n + skew):
        if step < n:
            out += produce(step)
        if step >= skew:
            out += consume(step - skew)
    return out


def _by_column(items, op, ncol):
    return [op(it, c) for c in range(ncol) for it in items]


def _by_item(items, op, ncol):
    return [op(it, c) for it in items for c in range(ncol)]


def _run(ops):
    for f in ops:
        f(None)


def _dot(a, b):
    return jnp.dot(a, b, preferred_element_type=F32)


def _bf(words):
    return pltpu.bitcast(words, BF16)


def _lo(w):
    return pltpu.bitcast(w << 16, F32)


def _hi(w):
    return pltpu.bitcast(w & jnp.uint32(0xFFFF0000), F32)


def _sublane_sum(t):
    t = t + pltpu.roll(t, 4, 0)
    t = t + pltpu.roll(t, 2, 0)
    return t + pltpu.roll(t, 1, 0)


def _col_bcast(row):
    return pltpu.bitcast(jnp.broadcast_to(row, (L, L)).T, U32)


def _round_bf16(x):
    return x.astype(BF16).astype(F32)


def _stats(xt):
    x = jnp.concatenate(xt, axis=1)
    mu = jnp.mean(x, axis=-1, keepdims=True)
    xc = x - mu
    var = jnp.mean(xc * xc, axis=-1, keepdims=True)
    return mu, jax.lax.rsqrt(var + EPS)


def _lhs16(xt):
    return [jnp.concatenate([x, jnp.ones_like(x)], axis=0).astype(BF16) for x in xt]


def _acc(d, k, v):
    d[k] = v if d.get(k) is None else d[k] + v
    return d[k]


def _kernel(x_hbm, wr_hbm, wq_hbm, wuk_hbm, ckv_hbm, wuv_hbm, wg_hbm, wu_hbm,
            wo_hbm, wd_hbm,
            o_ref,
            x_v, wr_v, wq_l, wuk_l, ckv_l, wuv_l, wg_l, wu_l, wo_l, wd_l,
            WQ32, WUKT32, CKV32, CKT32, WUV32, WG32, WU32, WO32, WD32,
            CSG, CSU, XE, XO, sems):
    sem_ids = iter(range(64))

    def copy(src, dst, sem=None):
        sem = next(sem_ids) if sem is None else sem
        c = pltpu.make_async_copy(src, dst, sems.at[sem])
        c.start()
        return c

    c_wq = copy(wq_hbm, wq_l)
    s_small = next(sem_ids)
    c_small = [copy(x_hbm, x_v, s_small), copy(wr_hbm, wr_v, s_small)]
    c_wuk = copy(wuk_hbm, wuk_l)
    c_ckv = copy(ckv_hbm, ckv_l)
    c_wuv = copy(wuv_hbm, wuv_l)
    c_wg = copy(wg_hbm, wg_l)
    c_wu = copy(wu_hbm, wu_l)
    wo_rows = H * D // WO_CHUNKS
    c_wo = [copy(wo_hbm.at[pl.ds(c * wo_rows, wo_rows)],
                 wo_l.at[pl.ds(c * wo_rows, wo_rows)]) for c in range(WO_CHUNKS)]
    c_wd = [copy(wd_hbm.at[:, pl.ds(nt * L, L)], wd_l.at[nt]) for nt in range(MT)]

    def swap_heads(src, dst32, rows):
        ch = 64

        def body(i, carry):
            w = src[pl.ds(pl.multiple_of(i * ch, ch), ch)]
            dst32[:, pl.ds(pl.multiple_of(i * (ch // 2), ch // 2), ch // 2), :] = (
                pltpu.bitcast(jnp.swapaxes(w, 0, 1), U32))
            return carry
        jax.lax.fori_loop(0, rows // ch, body, 0)

    def make_wukt():
        def body(i, carry):
            w = wuk_l[pl.ds(pl.multiple_of(i * L, L), L)]
            w = jnp.swapaxes(jnp.swapaxes(w, 0, 1), 1, 2)
            WUKT32[:, pl.ds(pl.multiple_of(i * W2, W2), W2), :] = pltpu.bitcast(w, U32)
            return carry
        jax.lax.fori_loop(0, CT, body, 0)

    def make_ck():
        def body(kt, carry):
            w = ckv_l[pl.ds(pl.multiple_of(kt * L, L), L), :]
            CKT32[kt] = pltpu.bitcast(w.T, U32)
            for ct in range(CT):
                CKV32[ct, pl.ds(pl.multiple_of(kt * W2, W2), W2), :] = pltpu.bitcast(
                    w[:, ct * L:(ct + 1) * L], U32)
            return carry
        jax.lax.fori_loop(0, KT, body, 0)

    def make_wgu(src, dst32):
        def body(ft, carry):
            w = src[pl.ds(pl.multiple_of(ft * L, L), L), :]
            dst32[ft] = pltpu.bitcast(w.T, U32)
            return carry
        jax.lax.fori_loop(0, FT - 1, body, 0)
        w = src[(FT - 1) * L:FF, :]
        w = jnp.concatenate([w, jnp.zeros((L - F_TAIL, M), BF16)], axis=0)
        dst32[FT - 1] = pltpu.bitcast(w.T, U32)

    def make_cols(src, dst32, r0, rows):
        for nt in range(MT):
            dst32[nt, r0 // 2:(r0 + rows) // 2, :] = pltpu.bitcast(
                src[r0:r0 + rows, nt * L:(nt + 1) * L], U32)

    sub = jax.lax.broadcasted_iota(jnp.int32, (R, L), 0)
    zero_v = []

    def link(a, dep):
        if dep is None:
            return a
        z = pltpu.bitcast(dep, U32) & zero_v[0]
        a32 = pltpu.bitcast(a, U32)
        return pltpu.bitcast(a32 | z[:a32.shape[0]], a.dtype)

    def make_xb(xt):
        for t in range(MT):
            w = _col_bcast(xt[t].astype(BF16)[0:1])
            XE[t * W2:(t + 1) * W2, :] = _lo(w)
            XO[t * W2:(t + 1) * W2, :] = _hi(w)

    def tile(ref32, lead, t):
        return _bf(ref32[lead, t * W2:(t + 1) * W2, :])

    def vpu_matvec_step(accs, ref_keys, s, dep):
        xe = link(XE[s * R:(s + 1) * R, :], dep)
        xo = XO[s * R:(s + 1) * R, :]
        for ref32, lead in ref_keys:
            w = ref32[lead, s * R:(s + 1) * R, :]
            _acc(accs, (id(ref32), lead), _lo(w) * xe + _hi(w) * xo)

    def q_partial(oq, x_tile, t):
        lhs = _lhs16([x_tile])[0]

        def op(h):
            def f(dep):
                p = _dot(link(lhs, dep), tile(WQ32, h, t))
                _acc(oq, h, p)
                return p[:R]
            return f
        return [op(h) for h in range(H)]

    def attention(xt, first, oq):
        mu, rstd = _stats(xt)
        qscale = rstd * (D ** -0.5)
        nva = 0 if first else VA_HEADS
        nvo = 0 if first else VO_HEADS
        if first:
            c_wq.wait()
            swap_heads(wq_l, WQ32, M)
            for t in range(MT - 1):
                _run(q_partial(oq, xt[t], t))
            c_wuk.wait()
            make_wukt()

        qh, qa = {}, {}

        def q_last(h, op):
            def f(dep):
                r = op(dep)
                o = oq[h]
                qh[h] = ((o[:R] - mu * o[R:]) * qscale).astype(BF16)
                return r
            return f

        def put_qa(h, ct, t):
            g, i = divmod(h, R)
            qa[g, ct] = t if (g, ct) not in qa else jnp.where(sub == i, t, qa[g, ct])

        def qabs_op(h, ct):
            def f(dep):
                t = _dot(link(qh[h], dep if LINK_P1 else None), tile(WUKT32, h, ct))
                put_qa(h, ct, t)
                return t
            return f

        ms = [q_last(h, op) for h, op in enumerate(q_partial(oq, xt[MT - 1], MT - 1))]
        ms += _by_item(range(nva, H - EDGE), qabs_op, CT)
        ms += _by_column(range(H - EDGE, H), qabs_op, CT)
        qw, aacc = {}, {}

        def qxlu_op(h):
            def f(dep):
                qw[h] = _col_bcast(qh[h][0:1])
                return pltpu.bitcast(qw[h][:R], F32)
            f.ready = lambda: h in qh
            return f

        def qa_vstep(h, k):
            def f(dep):
                w = qw[h][k * R:(k + 1) * R]
                ce, co = link(_lo(w), dep), _hi(w)
                for ct in range(CT):
                    r0 = ct * W2 + k * R
                    w = WUKT32[h, r0:r0 + R, :]
                    _acc(aacc, (h, ct), _lo(w) * ce + _hi(w) * co)
                if k == L // 16 - 1:
                    for ct in range(CT):
                        put_qa(h, ct, _sublane_sum(aacc[h, ct]))
                return aacc[h, 0]
            return f

        vs = [qxlu_op(h) for h in range(min(XLU_AHEAD, nva))]
        for h in range(nva):
            if h + XLU_AHEAD < nva:
                vs.append(qxlu_op(h + XLU_AHEAD))
            vs += [qa_vstep(h, k) for k in range(L // 16)]
        _cosched(ms, vs, P1_CFG)
        qabs = [jnp.concatenate([qa[g, ct] for g in range(H // R)], axis=0).astype(BF16)
                for ct in range(CT)]

        if first:
            c_ckv.wait()
            make_ck()
        nch = KT // KCHUNK
        sc, ps, lats = {}, {}, {}
        mxs, lss = [None] * nch, [None] * nch

        def score_op(kt, ct):
            def f(dep):
                _acc(sc, kt, _dot(qabs[ct], tile(CKT32, kt, ct)))
                j = kt // KCHUNK
                if ct == CT - 1 and kt == (j + 1) * KCHUNK - 1:
                    kts = range(j * KCHUNK, (j + 1) * KCHUNK)
                    mx = sc[kts[0]]
                    for k in kts[1:]:
                        mx = jnp.maximum(mx, sc[k])
                    mx = jnp.max(mx, axis=-1, keepdims=True)
                    lsum = None
                    for k in kts:
                        e = jnp.exp(sc[k] - mx)
                        lsum = e if lsum is None else lsum + e
                        ps[k] = e.astype(BF16)
                    mxs[j], lss[j] = mx, lsum
            return f

        def lat_op(kt, ct):
            def f(dep):
                _acc(lats, (kt // KCHUNK, ct), _dot(ps[kt], tile(CKV32, ct, kt)))
            return f

        def s_produce(j):
            kts = list(range(j * KCHUNK, (j + 1) * KCHUNK))
            if j == 0:
                return (_by_column(kts[:EDGE], score_op, CT)
                        + _by_item(kts[EDGE:], score_op, CT))
            return _by_item(kts, score_op, CT)

        def s_consume(j):
            return _by_column(range(j * KCHUNK, (j + 1) * KCHUNK), lat_op, CT)

        _run(_skewed(nch, SKEW_S, s_produce, s_consume))
        m = mxs[0]
        for t in mxs[1:]:
            m = jnp.maximum(m, t)
        alpha = [jnp.exp(t - m) for t in mxs]
        lsum = alpha[0] * lss[0]
        for a, t in zip(alpha[1:], lss[1:]):
            lsum = lsum + a * t
        inv = 1.0 / jnp.sum(lsum, axis=-1, keepdims=True)
        alpha = [a * inv for a in alpha]
        latg = {}
        for ct in range(CT):
            t = alpha[0] * lats[0, ct]
            for j in range(1, nch):
                t = t + alpha[j] * lats[j, ct]
            for g in range(H // R):
                latg[g, ct] = t[g * R:(g + 1) * R].astype(BF16)

        if first:
            c_wuv.wait()
            swap_heads(wuv_l, WUV32, DC)
        cacc, cbs, o = {}, {}, {}

        def ctx_op(h, ct):
            def f(dep):
                g, i = divmod(h, R)
                p = _dot(link(latg[g, ct], dep), tile(WUV32, h, ct))
                c = _acc(cacc, h, p)
                if ct == CT - 1:
                    cbs[h] = jnp.broadcast_to(c[i:i + 1], (R, D)).astype(BF16)
                return p
            return f

        def out_op(h, nt):
            def f(dep):
                t = _dot(link(cbs[h], dep if LINK_P3 else None), tile(WO32, nt, h))
                _acc(o, nt, t)
                return t
            return f

        if first:
            _run(_by_item(range(H), ctx_op, CT))
            c_wg.wait()
            make_wgu(wg_l, WG32)
            c_wu.wait()
            make_wgu(wu_l, WU32)
            hpc = H // WO_CHUNKS
            for c in range(WO_CHUNKS):
                c_wo[c].wait()
                make_cols(wo_l, WO32, c * wo_rows, wo_rows)
                _run(_by_item(range(c * hpc, (c + 1) * hpc), out_op, MT))
            return [_round_bf16(xt[nt] + o[nt]) for nt in range(MT)]

        ms = _by_column(range(EDGE), ctx_op, CT) + _by_item(range(EDGE, nvo), ctx_op, CT)
        h0 = max(nvo, EDGE)

        def o_produce(i):
            return _by_item([h0 + i], ctx_op, CT)

        def o_consume(h):
            if h >= H - EDGE:
                return _by_column(range(H - EDGE, H), out_op, MT) if h == H - 1 else []
            return _by_item([h], out_op, MT)

        for step in range(H - h0 + SKEW_O):
            if step < H - h0:
                ms += o_produce(step)
            if step >= SKEW_O:
                ms += o_consume(h0 + step - SKEW_O)
        for h in range(nvo, h0):
            ms += o_consume(h)
        cw, ov = {}, {}

        def xlu_op(h):
            def f(dep):
                cw[h] = _col_bcast(cbs[h][0:1])
                return pltpu.bitcast(cw[h][:R], F32)
            f.ready = lambda: h in cbs
            return f

        def o_vstep(h, k):
            def f(dep):
                w = cw[h][k * R:(k + 1) * R]
                ce, co = link(_lo(w), dep), _hi(w)
                r0 = h * W2 + k * R
                for nt in range(MT):
                    w = WO32[nt, r0:r0 + R, :]
                    _acc(ov, nt, _lo(w) * ce + _hi(w) * co)
                return ov[0]
            return f

        vs = [xlu_op(h) for h in range(min(XLU_AHEAD, nvo))]
        for h in range(nvo):
            if h + XLU_AHEAD < nvo:
                vs.append(xlu_op(h + XLU_AHEAD))
            vs += [o_vstep(h, k) for k in range(L // 16)]
        _cosched(ms, vs, P3_CFG)
        if nvo:
            o = {nt: o[nt] + _sublane_sum(ov[nt]) for nt in range(MT)}
        return [_round_bf16(xt[nt] + o[nt]) for nt in range(MT)]

    def ffn(xt, first, oq_next=None):
        mu, rstd = _stats(xt)
        lhs = _lhs16(xt)
        xn = [(x - mu) * rstd for x in xt]
        wr = wr_v[...].reshape(1, M).astype(F32)
        r = jnp.sum(jnp.concatenate(xn, axis=1) * wr, axis=-1, keepdims=True)
        gate = jax.nn.sigmoid(r)
        nvf = 0 if first else VF_TILES
        pre, acts, y = {}, {}, {}

        def finish(ft):
            g, u = pre[ft, 0] * rstd, pre[ft, 1] * rstd
            acts[ft] = (g * jax.nn.sigmoid(g) * u).astype(BF16)

        def gu_op(key, t):
            ft, which = key

            def f(dep):
                p = _dot(link(lhs[t], dep), tile((WG32, WU32)[which], ft, t))
                o = _acc(pre, key, p)
                if t == MT - 1:
                    if first and ft < VF_TILES:
                        (CSG, CSU)[which][ft] = o[R:]
                    pre[key] = o[:R] - mu * o[R:]
                    if which == 1:
                        finish(ft)
                return p[:R]
            return f

        def dn_op(ft, nt):
            def f(dep):
                rows = L if ft < FT - 1 else F_TAIL
                a = acts[ft] if rows == L else acts[ft][:, :rows]
                if first:
                    w = wd_l[nt, ft * L:ft * L + rows, :]
                else:
                    w = _bf(WD32[nt, ft * W2:ft * W2 + rows // 2, :])
                t = _dot(link(a, dep if LINK_P4 else None), w)
                _acc(y, nt, t)
                return t
            f.ready = lambda: ft in acts
            return f

        def gu_keys(fts):
            return [(ft, which) for ft in fts for which in range(2)]

        if first:
            _run(_by_item(gu_keys(range(FT)), gu_op, MT))
            out = []
            for nt in range(MT):
                c_wd[nt].wait()
                _run([dn_op(ft, nt) for ft in range(FT)])
                out.append(_round_bf16(xt[nt] + xn[nt] + y[nt] * gate))
                if nt < MT - 1 and oq_next is not None:
                    _run(q_partial(oq_next, out[nt], nt))
            return out
        else:
            mt = list(range(nvf, FT))
            last = (mt + list(range(nvf)))[-2:] if nvf < 2 else list(range(nvf))[-2:]

            def g_produce(i):
                if i == 0:
                    return _by_column(gu_keys(mt[:2]), gu_op, MT)
                return [] if i == 1 else _by_item(gu_keys([mt[i]]), gu_op, MT)

            def g_consume(ft):
                if ft in last:
                    return _by_column(last, dn_op, MT) if ft == last[-1] else []
                return _by_item([ft], dn_op, MT)

            ms = _skewed(len(mt), SKEW_F, g_produce, lambda i: g_consume(mt[i]))
            for ft in range(nvf):
                ms += g_consume(ft)
            facc = {}

            def f_vstep(fts, s):
                def f(dep):
                    keys = [(w, ft) for ft in fts for w in (WG32, WU32)]
                    vpu_matvec_step(facc, keys, s, dep)
                    if s == M // 16 - 1:
                        for ft in fts:
                            for wh, (w, cs) in enumerate(((WG32, CSG), (WU32, CSU))):
                                pre[ft, wh] = _sublane_sum(facc[id(w), ft]) - mu * cs[ft]
                            finish(ft)
                    return facc[id(WG32), fts[0]]
                return f

            if nvf:
                make_xb(xt)
            vs = [f_vstep(list(range(f0, min(nvf, f0 + VF_GROUP))), s)
                  for f0 in range(0, nvf, VF_GROUP) for s in range(M // 16)]
            _cosched(ms, vs, P4_CFG)
        return [_round_bf16(xt[nt] + xn[nt] + y[nt] * gate) for nt in range(MT)]

    for c in c_small:
        c.wait()
    x = jnp.broadcast_to(x_v[...].astype(F32), (R, M))
    zero_v.append(pltpu.bitcast(x[:, :L], U32) & jnp.uint32(0xFFFF))
    xt = [x[:, t * L:(t + 1) * L] for t in range(MT)]
    xt = attention(xt, True, {})
    oq2 = {}
    xt = ffn(xt, True, oq2 if N_LAYERS > 1 else None)
    if N_LAYERS > 1:
        for nt in range(MT):
            WD32[nt] = pltpu.bitcast(wd_l[nt], U32)
        xt = attention(xt, False, oq2)
        xt = ffn(xt, False)
    o_ref[...] = jnp.concatenate(xt, axis=1)[0:1].astype(o_ref.dtype)


@jax.jit
def pallas_interleave_layers__compressed_kv_cla__moe_arch_mod__decode_kernel(
    A_x: jax.Array,
    A_c_kv: jax.Array,
    A_w_q: jax.Array,
    A_w_uk: jax.Array,
    A_w_uv: jax.Array,
    A_w_o: jax.Array,
    B_x: jax.Array,
    B_w_r: jax.Array,
    B_w_gate: jax.Array,
    B_w_up: jax.Array,
    B_w_down: jax.Array,
):
    del B_x
    args = (
        A_x.reshape(1, M),
        B_w_r,
        A_w_q,
        A_w_uk,
        A_c_kv.reshape(SK, DC),
        A_w_uv,
        B_w_gate.T,
        B_w_up.T,
        A_w_o.reshape(H * D, M),
        B_w_down,
    )
    n_sems = 7 + WO_CHUNKS + MT
    scratch = [
        pltpu.VMEM((1, M), BF16),
        pltpu.VMEM((M,), BF16),
        pltpu.VMEM((M, H, D), BF16),
        pltpu.VMEM((DC, H, D), BF16),
        pltpu.VMEM((SK, DC), BF16),
        pltpu.VMEM((DC, H, D), BF16),
        pltpu.VMEM((FF, M), BF16),
        pltpu.VMEM((FF, M), BF16),
        pltpu.VMEM((H * D, M), BF16),
        pltpu.VMEM((MT, FF, L), BF16),
        pltpu.VMEM((H, M // 2, D), U32),
        pltpu.VMEM((H, DC // 2, L), U32),
        pltpu.VMEM((CT, SK // 2, L), U32),
        pltpu.VMEM((KT, DC // 2, L), U32),
        pltpu.VMEM((H, DC // 2, D), U32),
        pltpu.VMEM((FT, M // 2, L), U32),
        pltpu.VMEM((FT, M // 2, L), U32),
        pltpu.VMEM((MT, H * D // 2, L), U32),
        pltpu.VMEM((MT, FF // 2, L), U32),
        pltpu.VMEM((FT, R, L), F32),
        pltpu.VMEM((FT, R, L), F32),
        pltpu.VMEM((M // 2, L), F32),
        pltpu.VMEM((M // 2, L), F32),
        pltpu.SemaphoreType.DMA((n_sems,)),
    ]
    out = pl.pallas_call(
        _kernel,
        out_shape=jax.ShapeDtypeStruct((1, M), A_x.dtype),
        in_specs=[pl.BlockSpec(memory_space=pl.ANY)] * len(args),
        out_specs=pl.BlockSpec(memory_space=pltpu.VMEM),
        scratch_shapes=scratch,
        compiler_params=pltpu.CompilerParams(
            vmem_limit_bytes=100 * 1024 * 1024,
            disable_semaphore_checks=True),
        name="mla_moe_decode",
    )(*args)
    return out.reshape(1, 1, M)
```

```python
import jax
import jax.numpy as jnp
import jax.experimental.pallas as pl
import jax.experimental.pallas.tpu as pltpu

F32 = jnp.float32
BF16 = jnp.bfloat16
U32 = jnp.uint32

H = 32
D = 128
M = 640
DC = 512
SK = 4096
FF = 1728
EPS = 1e-5
R = 8
L = 128
W2 = L // 2

MT = M // L
CT = DC // L
KT = SK // L
FT = -(-FF // L)
F_TAIL = FF - (FT - 1) * L
KCHUNK = 8
WO_CHUNKS = 4

N_LAYERS = 2
SKEW_S = 1
SKEW_O = 6
SKEW_F = 5
EDGE = 4

VA_HEADS = 8
P1_CFG = (460, 2.5, 16, 140, 2, 560)
VO_HEADS = 16
P3_CFG = (420, 2.8, 40, 170, 2, 760)
XLU_AHEAD = 2
LINK_P1 = False
LINK_P3 = False
LINK_P4 = False
VF_TILES = 4
VF_GROUP = 2
VD_TILES = 3
XLU_EARLY = 10
P4_CFG = (160, 2.2, 8, 150, 1, 0)


def _always():
    return True


def _cosched(ms, vs, cfg):
    vstart, rate, lag_v, lag_m, nlink, lstart = cfg
    mres, vres = [], []
    j, tv = 0, vstart

    def latest(res, t):
        for tt, val in reversed(res):
            if tt <= t:
                return val
        return None

    def emit_v(dep):
        nonlocal j, tv
        val = vs[j](dep)
        tv += getattr(vs[j], "valu", 0) / rate
        vres.append((tv, val))
        j += 1

    for i, m in enumerate(ms):
        t = 8 * i
        while not getattr(m, "ready", _always)():
            emit_v(None)
        dep = None
        if i % nlink == 0 and j < len(vs) and t >= lstart:
            dep = latest(vres, t - lag_v)
        mres.append((t, m(dep)))
        while j < len(vs) and tv <= t + 8 and getattr(vs[j], "ready", _always)():
            emit_v(latest(mres, tv - lag_m) if j % 2 == 0 else None)
    while j < len(vs):
        emit_v(None)


def _valu(n):
    def deco(f):
        f.valu = n
        return f
    return deco


def _skewed(n, skew, produce, consume):
    out = []
    for step in range(n + skew):
        if step < n:
            out += produce(step)
        if step >= skew:
            out += consume(step - skew)
    return out


def _by_column(items, op, ncol):
    return [op(it, c) for c in range(ncol) for it in items]


def _by_item(items, op, ncol):
    return [op(it, c) for it in items for c in range(ncol)]


def _run(ops):
    for f in ops:
        f(None)


def _dot(a, b):
    return jnp.dot(a, b, preferred_element_type=F32)


def _bf(words):
    return pltpu.bitcast(words, BF16)


def _lo(w):
    return pltpu.bitcast(w << 16, F32)


def _hi(w):
    return pltpu.bitcast(w & jnp.uint32(0xFFFF0000), F32)


def _sublane_sum(t):
    t = t + pltpu.roll(t, 4, 0)
    t = t + pltpu.roll(t, 2, 0)
    return t + pltpu.roll(t, 1, 0)


def _col_bcast(row):
    return pltpu.bitcast(jnp.broadcast_to(row, (L, L)).T, U32)


def _round_bf16(x):
    return x.astype(BF16).astype(F32)


def _stats(xt):
    c = jnp.mean(xt[0], axis=-1, keepdims=True)
    s1 = s2 = None
    for x in xt:
        d = x - c
        s1 = d if s1 is None else s1 + d
        s2 = d * d if s2 is None else s2 + d * d
    m1 = jnp.sum(s1, axis=-1, keepdims=True) * (1.0 / M)
    m2 = jnp.sum(s2, axis=-1, keepdims=True) * (1.0 / M)
    var = jnp.maximum(m2 - m1 * m1, 0.0)
    return c + m1, jax.lax.rsqrt(var + EPS)


def _lhs16(xt):
    return [jnp.concatenate([x, jnp.ones_like(x)], axis=0).astype(BF16) for x in xt]


def _acc(d, k, v):
    d[k] = v if d.get(k) is None else d[k] + v
    return d[k]


def _kernel(x_hbm, wr_hbm, wq_hbm, wuk_hbm, ckv_hbm, wuv_hbm, wg_hbm, wu_hbm,
            wo_hbm, wd_hbm,
            o_ref,
            x_v, wr_v, wq_l, wuk_l, ckv_l, wuv_l, wg_l, wu_l, wo_l, wd_l,
            WQ32, WUKT32, CKV32, CKT32, WUV32, WG32, WU32, WO32, WD32,
            CSG, CSU, XE, XO, sems):
    sem_ids = iter(range(64))

    def copy(src, dst, sem=None):
        sem = next(sem_ids) if sem is None else sem
        c = pltpu.make_async_copy(src, dst, sems.at[sem])
        c.start()
        return c

    c_wq = copy(wq_hbm, wq_l)
    s_small = next(sem_ids)
    c_small = [copy(x_hbm, x_v, s_small), copy(wr_hbm, wr_v, s_small)]
    c_wuk = copy(wuk_hbm, wuk_l)
    c_ckv = copy(ckv_hbm, ckv_l)
    c_wuv = copy(wuv_hbm, wuv_l)
    c_wg = copy(wg_hbm, wg_l)
    c_wu = copy(wu_hbm, wu_l)
    wo_rows = H * D // WO_CHUNKS
    c_wo = [copy(wo_hbm.at[pl.ds(c * wo_rows, wo_rows)],
                 wo_l.at[pl.ds(c * wo_rows, wo_rows)]) for c in range(WO_CHUNKS)]
    c_wd = [copy(wd_hbm.at[:, pl.ds(nt * L, L)], wd_l.at[nt]) for nt in range(MT)]

    def swap_heads(src, dst32, rows):
        ch = 64

        def body(i, carry):
            w = src[pl.ds(pl.multiple_of(i * ch, ch), ch)]
            dst32[:, pl.ds(pl.multiple_of(i * (ch // 2), ch // 2), ch // 2), :] = (
                pltpu.bitcast(jnp.swapaxes(w, 0, 1), U32))
            return carry
        jax.lax.fori_loop(0, rows // ch, body, 0)

    def make_wukt():
        def body(i, carry):
            w = wuk_l[pl.ds(pl.multiple_of(i * L, L), L)]
            w = jnp.swapaxes(jnp.swapaxes(w, 0, 1), 1, 2)
            WUKT32[:, pl.ds(pl.multiple_of(i * W2, W2), W2), :] = pltpu.bitcast(w, U32)
            return carry
        jax.lax.fori_loop(0, CT, body, 0)

    def make_ck():
        def body(kt, carry):
            w = ckv_l[pl.ds(pl.multiple_of(kt * L, L), L), :]
            CKT32[kt] = pltpu.bitcast(w.T, U32)
            for ct in range(CT):
                CKV32[ct, pl.ds(pl.multiple_of(kt * W2, W2), W2), :] = pltpu.bitcast(
                    w[:, ct * L:(ct + 1) * L], U32)
            return carry
        jax.lax.fori_loop(0, KT, body, 0)

    def make_wgu(src, dst32):
        def body(ft, carry):
            w = src[pl.ds(pl.multiple_of(ft * L, L), L), :]
            dst32[ft] = pltpu.bitcast(w.T, U32)
            return carry
        jax.lax.fori_loop(0, FT - 1, body, 0)
        w = src[(FT - 1) * L:FF, :]
        w = jnp.concatenate([w, jnp.zeros((L - F_TAIL, M), BF16)], axis=0)
        dst32[FT - 1] = pltpu.bitcast(w.T, U32)

    def make_cols(src, dst32, r0, rows):
        for nt in range(MT):
            dst32[nt, r0 // 2:(r0 + rows) // 2, :] = pltpu.bitcast(
                src[r0:r0 + rows, nt * L:(nt + 1) * L], U32)

    sub = jax.lax.broadcasted_iota(jnp.int32, (R, L), 0)
    zero_v = []

    def link(a, dep):
        if dep is None:
            return a
        z = pltpu.bitcast(dep, U32) & zero_v[0]
        a32 = pltpu.bitcast(a, U32)
        return pltpu.bitcast(a32 | z[:a32.shape[0]], a.dtype)

    def make_xb(xt):
        for t in range(MT):
            w = _col_bcast(xt[t].astype(BF16)[0:1])
            XE[t * W2:(t + 1) * W2, :] = _lo(w)
            XO[t * W2:(t + 1) * W2, :] = _hi(w)

    def tile(ref32, lead, t):
        return _bf(ref32[lead, t * W2:(t + 1) * W2, :])

    def vpu_matvec_step(accs, ref_keys, s, dep):
        xe = link(XE[s * R:(s + 1) * R, :], dep)
        xo = XO[s * R:(s + 1) * R, :]
        for ref32, lead in ref_keys:
            w = ref32[lead, s * R:(s + 1) * R, :]
            _acc(accs, (id(ref32), lead), _lo(w) * xe + _hi(w) * xo)

    def q_partial(oq, x_tile, t):
        lhs = _lhs16([x_tile])[0]

        def op(h):
            def f(dep):
                p = _dot(link(lhs, dep), tile(WQ32, h, t))
                _acc(oq, h, p)
                return p[:R]
            return f
        return [op(h) for h in range(H)]

    def attention(xt, first, oq):
        mu, rstd = _stats(xt)
        qscale = rstd * (D ** -0.5)
        nva = 0 if first else VA_HEADS
        nvo = 0 if first else VO_HEADS
        if first:
            c_wq.wait()
            swap_heads(wq_l, WQ32, M)
            for t in range(MT - 1):
                _run(q_partial(oq, xt[t], t))
            c_wuk.wait()
            make_wukt()

        qh, qa = {}, {}

        def q_last(h, op):
            def f(dep):
                r = op(dep)
                o = oq[h]
                qh[h] = ((o[:R] - mu * o[R:]) * qscale).astype(BF16)
                return r
            return f

        def put_qa(h, ct, t):
            g, i = divmod(h, R)
            qa[g, ct] = t if (g, ct) not in qa else jnp.where(sub == i, t, qa[g, ct])

        def qabs_op(h, ct):
            def f(dep):
                t = _dot(link(qh[h], dep if LINK_P1 else None), tile(WUKT32, h, ct))
                put_qa(h, ct, t)
                return t
            return f

        ms = [q_last(h, op) for h, op in enumerate(q_partial(oq, xt[MT - 1], MT - 1))]
        ms += _by_item(range(nva, H - EDGE), qabs_op, CT)
        ms += _by_column(range(H - EDGE, H), qabs_op, CT)
        qw, aacc = {}, {}

        def qxlu_op(h):
            def f(dep):
                qw[h] = _col_bcast(qh[h][0:1])
                return pltpu.bitcast(qw[h][:R], F32)
            f.ready = lambda: h in qh
            return f

        def qa_vstep(h, k):
            def f(dep):
                w = qw[h][k * R:(k + 1) * R]
                ce, co = link(_lo(w), dep), _hi(w)
                for ct in range(CT):
                    r0 = ct * W2 + k * R
                    w = WUKT32[h, r0:r0 + R, :]
                    _acc(aacc, (h, ct), _lo(w) * ce + _hi(w) * co)
                if k == L // 16 - 1:
                    for ct in range(CT):
                        put_qa(h, ct, _sublane_sum(aacc[h, ct]))
                return aacc[h, 0]
            return _valu(6 * CT + 2)(f)

        vs = [qxlu_op(h) for h in range(min(XLU_AHEAD, nva))]
        for h in range(nva):
            if h + XLU_AHEAD < nva:
                vs.append(qxlu_op(h + XLU_AHEAD))
            vs += [qa_vstep(h, k) for k in range(L // 16)]
        _cosched(ms, vs, P1_CFG)
        qabs = [jnp.concatenate([qa[g, ct] for g in range(H // R)], axis=0).astype(BF16)
                for ct in range(CT)]

        if first:
            c_ckv.wait()
            make_ck()
        nch = KT // KCHUNK
        sc, ps, lats = {}, {}, {}
        mxs, lss = [None] * nch, [None] * nch

        def score_op(kt, ct):
            def f(dep):
                _acc(sc, kt, _dot(qabs[ct], tile(CKT32, kt, ct)))
                j = kt // KCHUNK
                if ct == CT - 1 and kt == (j + 1) * KCHUNK - 1:
                    kts = range(j * KCHUNK, (j + 1) * KCHUNK)
                    mx = sc[kts[0]]
                    for k in kts[1:]:
                        mx = jnp.maximum(mx, sc[k])
                    mx = jnp.max(mx, axis=-1, keepdims=True)
                    lsum = None
                    for k in kts:
                        e = jnp.exp(sc[k] - mx)
                        lsum = e if lsum is None else lsum + e
                        ps[k] = e.astype(BF16)
                    mxs[j], lss[j] = mx, lsum
            return f

        def lat_op(kt, ct):
            def f(dep):
                _acc(lats, (kt // KCHUNK, ct), _dot(ps[kt], tile(CKV32, ct, kt)))
            return f

        def s_produce(j):
            kts = list(range(j * KCHUNK, (j + 1) * KCHUNK))
            if j == 0:
                return (_by_column(kts[:EDGE], score_op, CT)
                        + _by_item(kts[EDGE:], score_op, CT))
            return _by_item(kts, score_op, CT)

        def s_consume(j):
            return _by_column(range(j * KCHUNK, (j + 1) * KCHUNK), lat_op, CT)

        _run(_skewed(nch, SKEW_S, s_produce, s_consume))
        m = mxs[0]
        for t in mxs[1:]:
            m = jnp.maximum(m, t)
        alpha = [jnp.exp(t - m) for t in mxs]
        lsum = alpha[0] * lss[0]
        for a, t in zip(alpha[1:], lss[1:]):
            lsum = lsum + a * t
        inv = 1.0 / jnp.sum(lsum, axis=-1, keepdims=True)
        alpha = [a * inv for a in alpha]
        latg = {}
        for ct in range(CT):
            t = alpha[0] * lats[0, ct]
            for j in range(1, nch):
                t = t + alpha[j] * lats[j, ct]
            for g in range(H // R):
                latg[g, ct] = t[g * R:(g + 1) * R].astype(BF16)

        if first:
            c_wuv.wait()
            swap_heads(wuv_l, WUV32, DC)
        cacc, cbs, o = {}, {}, {}

        def ctx_op(h, ct):
            def f(dep):
                g, i = divmod(h, R)
                p = _dot(link(latg[g, ct], dep), tile(WUV32, h, ct))
                c = _acc(cacc, h, p)
                if ct == CT - 1:
                    cbs[h] = jnp.broadcast_to(c[i:i + 1], (R, D)).astype(BF16)
                return p
            return f

        def out_op(h, nt):
            def f(dep):
                t = _dot(link(cbs[h], dep if LINK_P3 else None), tile(WO32, nt, h))
                _acc(o, nt, t)
                return t
            return f

        if first:
            _run(_by_item(range(H), ctx_op, CT))
            c_wg.wait()
            make_wgu(wg_l, WG32)
            c_wu.wait()
            make_wgu(wu_l, WU32)
            hpc = H // WO_CHUNKS
            for c in range(WO_CHUNKS):
                c_wo[c].wait()
                make_cols(wo_l, WO32, c * wo_rows, wo_rows)
                _run(_by_item(range(c * hpc, (c + 1) * hpc), out_op, MT))
            return [_round_bf16(xt[nt] + o[nt]) for nt in range(MT)]

        ms = _by_column(range(EDGE), ctx_op, CT) + _by_item(range(EDGE, nvo), ctx_op, CT)
        h0 = max(nvo, EDGE)

        def o_produce(i):
            return _by_item([h0 + i], ctx_op, CT)

        def o_consume(h):
            if h >= H - EDGE:
                return _by_column(range(H - EDGE, H), out_op, MT) if h == H - 1 else []
            return _by_item([h], out_op, MT)

        for step in range(H - h0 + SKEW_O):
            if step < H - h0:
                ms += o_produce(step)
            if step >= SKEW_O:
                ms += o_consume(h0 + step - SKEW_O)
        for h in range(nvo, h0):
            ms += o_consume(h)
        cw, ov = {}, {}

        def xlu_op(h):
            def f(dep):
                cw[h] = _col_bcast(cbs[h][0:1])
                return pltpu.bitcast(cw[h][:R], F32)
            f.ready = lambda: h in cbs
            return f

        def o_vstep(h, k):
            def f(dep):
                w = cw[h][k * R:(k + 1) * R]
                ce, co = link(_lo(w), dep), _hi(w)
                r0 = h * W2 + k * R
                for nt in range(MT):
                    w = WO32[nt, r0:r0 + R, :]
                    _acc(ov, nt, _lo(w) * ce + _hi(w) * co)
                return ov[0]
            return _valu(6 * MT + 2)(f)

        vs = [xlu_op(h) for h in range(min(XLU_AHEAD, nvo))]
        for h in range(nvo):
            if h + XLU_AHEAD < nvo:
                vs.append(xlu_op(h + XLU_AHEAD))
            vs += [o_vstep(h, k) for k in range(L // 16)]
        _cosched(ms, vs, P3_CFG)
        if nvo:
            o = {nt: o[nt] + _sublane_sum(ov[nt]) for nt in range(MT)}
        return [_round_bf16(xt[nt] + o[nt]) for nt in range(MT)]

    def ffn(xt, first, oq_next=None):
        mu, rstd = _stats(xt)
        lhs = _lhs16(xt)
        xn = [(x - mu) * rstd for x in xt]
        wr = wr_v[...].reshape(1, M).astype(F32)
        r = jnp.sum(jnp.concatenate(xn, axis=1) * wr, axis=-1, keepdims=True)
        gate = jax.nn.sigmoid(r)
        nvf = 0 if first else VF_TILES
        pre, acts, y = {}, {}, {}

        def finish(ft):
            g, u = pre[ft, 0] * rstd, pre[ft, 1] * rstd
            acts[ft] = (g * jax.nn.sigmoid(g) * u).astype(BF16)

        def gu_op(key, t):
            ft, which = key

            def f(dep):
                p = _dot(link(lhs[t], dep), tile((WG32, WU32)[which], ft, t))
                o = _acc(pre, key, p)
                if t == MT - 1:
                    if first and ft < VF_TILES:
                        (CSG, CSU)[which][ft] = o[R:]
                    pre[key] = o[:R] - mu * o[R:]
                    if which == 1:
                        finish(ft)
                return p[:R]
            return f

        def dn_op(ft, nt):
            def f(dep):
                rows = L if ft < FT - 1 else F_TAIL
                a = acts[ft] if rows == L else acts[ft][:, :rows]
                if first:
                    w = wd_l[nt, ft * L:ft * L + rows, :]
                else:
                    w = _bf(WD32[nt, ft * W2:ft * W2 + rows // 2, :])
                t = _dot(link(a, dep if LINK_P4 else None), w)
                _acc(y, nt, t)
                return t
            f.ready = lambda: ft in acts
            return f

        def gu_keys(fts):
            return [(ft, which) for ft in fts for which in range(2)]

        if first:
            _run(_by_item(gu_keys(range(FT)), gu_op, MT))
            out = []
            for nt in range(MT):
                c_wd[nt].wait()
                _run([dn_op(ft, nt) for ft in range(FT)])
                out.append(_round_bf16(xt[nt] + xn[nt] + y[nt] * gate))
                if nt < MT - 1 and oq_next is not None:
                    _run(q_partial(oq_next, out[nt], nt))
            return out
        else:
            mt = list(range(nvf, FT))
            vd = mt[:VD_TILES]
            md = [ft for ft in mt if ft not in vd] + list(range(nvf))
            last = md[-2:]

            def g_produce(i):
                if i == 0:
                    return _by_column(gu_keys(mt[:2]), gu_op, MT)
                return [] if i == 1 else _by_item(gu_keys([mt[i]]), gu_op, MT)

            def g_consume(ft):
                if ft in vd:
                    return []
                if ft in last:
                    return _by_column(last, dn_op, MT) if ft == last[-1] else []
                return _by_item([ft], dn_op, MT)

            ms = _skewed(len(mt), SKEW_F, g_produce, lambda i: g_consume(mt[i]))
            for ft in range(nvf):
                ms += g_consume(ft)
            facc, aw, yv = {}, {}, {}

            def f_vstep(fts, s):
                def f(dep):
                    keys = [(w, ft) for ft in fts for w in (WG32, WU32)]
                    vpu_matvec_step(facc, keys, s, dep)
                    if s == M // 16 - 1:
                        for ft in fts:
                            for wh, (w, cs) in enumerate(((WG32, CSG), (WU32, CSU))):
                                pre[ft, wh] = _sublane_sum(facc[id(w), ft]) - mu * cs[ft]
                            finish(ft)
                    return facc[id(WG32), fts[0]]
                return _valu(12 * len(fts))(f)

            def dxlu_op(ft):
                def f(dep):
                    aw[ft] = _col_bcast(acts[ft][0:1])
                    return pltpu.bitcast(aw[ft][:R], F32)
                f.ready = lambda: ft in acts
                return f

            def d_vstep(ft, k):
                def f(dep):
                    w = aw[ft][k * R:(k + 1) * R]
                    ce, co = link(_lo(w), dep), _hi(w)
                    r0 = ft * W2 + k * R
                    for nt in range(MT):
                        w = WD32[nt, r0:r0 + R, :]
                        _acc(yv, nt, _lo(w) * ce + _hi(w) * co)
                    return yv[0]
                return _valu(6 * MT + 2)(f)

            if nvf:
                make_xb(xt)
            vs = [f_vstep(list(range(f0, min(nvf, f0 + VF_GROUP))), s)
                  for f0 in range(0, nvf, VF_GROUP) for s in range(M // 16)]
            pos = max(0, len(vs) - XLU_EARLY)
            for i, ft in enumerate(vd[:XLU_AHEAD]):
                vs.insert(pos + i, dxlu_op(ft))
            for i, ft in enumerate(vd):
                if i + XLU_AHEAD < len(vd):
                    vs.append(dxlu_op(vd[i + XLU_AHEAD]))
                vs += [d_vstep(ft, k) for k in range(L // 16)]
            _cosched(ms, vs, P4_CFG)
            if vd:
                y = {nt: y[nt] + _sublane_sum(yv[nt]) for nt in range(MT)}
        return [_round_bf16(xt[nt] + xn[nt] + y[nt] * gate) for nt in range(MT)]

    for c in c_small:
        c.wait()
    x = jnp.broadcast_to(x_v[...].astype(F32), (R, M))
    zero_v.append(pltpu.bitcast(x[:, :L], U32) & jnp.uint32(0xFFFF))
    xt = [x[:, t * L:(t + 1) * L] for t in range(MT)]
    xt = attention(xt, True, {})
    oq2 = {}
    xt = ffn(xt, True, oq2 if N_LAYERS > 1 else None)
    if N_LAYERS > 1:
        for nt in range(MT):
            WD32[nt] = pltpu.bitcast(wd_l[nt], U32)
        xt = attention(xt, False, oq2)
        xt = ffn(xt, False)
    o_ref[...] = jnp.concatenate(xt, axis=1)[0:1].astype(o_ref.dtype)


@jax.jit
def pallas_interleave_layers__compressed_kv_cla__moe_arch_mod__decode_kernel(
    A_x: jax.Array,
    A_c_kv: jax.Array,
    A_w_q: jax.Array,
    A_w_uk: jax.Array,
    A_w_uv: jax.Array,
    A_w_o: jax.Array,
    B_x: jax.Array,
    B_w_r: jax.Array,
    B_w_gate: jax.Array,
    B_w_up: jax.Array,
    B_w_down: jax.Array,
):
    del B_x
    args = (
        A_x.reshape(1, M),
        B_w_r,
        A_w_q,
        A_w_uk,
        A_c_kv.reshape(SK, DC),
        A_w_uv,
        B_w_gate.T,
        B_w_up.T,
        A_w_o.reshape(H * D, M),
        B_w_down,
    )
    n_sems = 7 + WO_CHUNKS + MT
    scratch = [
        pltpu.VMEM((1, M), BF16),
        pltpu.VMEM((M,), BF16),
        pltpu.VMEM((M, H, D), BF16),
        pltpu.VMEM((DC, H, D), BF16),
        pltpu.VMEM((SK, DC), BF16),
        pltpu.VMEM((DC, H, D), BF16),
        pltpu.VMEM((FF, M), BF16),
        pltpu.VMEM((FF, M), BF16),
        pltpu.VMEM((H * D, M), BF16),
        pltpu.VMEM((MT, FF, L), BF16),
        pltpu.VMEM((H, M // 2, D), U32),
        pltpu.VMEM((H, DC // 2, L), U32),
        pltpu.VMEM((CT, SK // 2, L), U32),
        pltpu.VMEM((KT, DC // 2, L), U32),
        pltpu.VMEM((H, DC // 2, D), U32),
        pltpu.VMEM((FT, M // 2, L), U32),
        pltpu.VMEM((FT, M // 2, L), U32),
        pltpu.VMEM((MT, H * D // 2, L), U32),
        pltpu.VMEM((MT, FF // 2, L), U32),
        pltpu.VMEM((FT, R, L), F32),
        pltpu.VMEM((FT, R, L), F32),
        pltpu.VMEM((M // 2, L), F32),
        pltpu.VMEM((M // 2, L), F32),
        pltpu.SemaphoreType.DMA((n_sems,)),
    ]
    out = pl.pallas_call(
        _kernel,
        out_shape=jax.ShapeDtypeStruct((1, M), A_x.dtype),
        in_specs=[pl.BlockSpec(memory_space=pl.ANY)] * len(args),
        out_specs=pl.BlockSpec(memory_space=pltpu.VMEM),
        scratch_shapes=scratch,
        compiler_params=pltpu.CompilerParams(
            vmem_limit_bytes=100 * 1024 * 1024,
            disable_semaphore_checks=True),
        name="mla_moe_decode",
    )(*args)
    return out.reshape(1, 1, M)
```

```python
import jax
import jax.numpy as jnp
import jax.experimental.pallas as pl
import jax.experimental.pallas.tpu as pltpu

F32 = jnp.float32
BF16 = jnp.bfloat16
U32 = jnp.uint32

H = 32
D = 128
M = 640
DC = 512
SK = 4096
FF = 1728
EPS = 1e-5
R = 8
L = 128
W2 = L // 2

MT = M // L
CT = DC // L
KT = SK // L
FT = -(-FF // L)
F_TAIL = FF - (FT - 1) * L
KCHUNK = 8
WO_SPLIT = (0, 10, 20, 28, 32)

N_LAYERS = 2
SKEW_S = 1
SKEW_O = 6
SKEW_F = 5
EDGE = 4

VA_HEADS = 11
P1_CFG = (420, 2.5, 16, 140, 2, 560)
VO_HEADS = 18
P3_CFG = (500, 2.6, 16, 170, 2, 640)
XLU_AHEAD = 2
WD_COPY = False
CK_UNROLL = 4
GU_UNROLL = 3
WD_ROWS = 432
F32_P1 = True
F32_P3 = True
F32_P4 = True
LINK_P1 = False
LINK_P3 = False
LINK_P4 = False
VF_TILES = 4
VF_GROUP = 2
VD_TILES = 3
XLU_EARLY = 10
P4_CFG = (280, 1.9, 16, 150, 1, 200)


SCOPES = False


class _ScopedWait:
    def __init__(self, c, name):
        self.c, self.name = c, name

    def wait(self):
        with jax.named_scope(self.name):
            self.c.wait()


def _always():
    return True


def _cosched(ms, vs, cfg):
    vstart, rate, lag_v, lag_m, nlink, lstart = cfg
    mres, vres = [], []
    j, tv = 0, vstart

    def latest(res, t):
        for tt, val in reversed(res):
            if tt <= t:
                return val
        return None

    def emit_v(dep):
        nonlocal j, tv
        val = vs[j](dep)
        tv += getattr(vs[j], "valu", 0) / rate
        vres.append((tv, val))
        j += 1

    for i, m in enumerate(ms):
        t = 8 * i
        while not getattr(m, "ready", _always)():
            emit_v(None)
        dep = None
        if i % nlink == 0 and j < len(vs) and t >= lstart:
            dep = latest(vres, t - lag_v)
        mres.append((t, m(dep)))
        while j < len(vs) and tv <= t + 8 and getattr(vs[j], "ready", _always)():
            emit_v(latest(mres, tv - lag_m) if j % 2 == 0 else None)
    while j < len(vs):
        emit_v(None)


def _valu(n):
    def deco(f):
        f.valu = n
        return f
    return deco


def _skewed(n, skew, produce, consume):
    out = []
    for step in range(n + skew):
        if step < n:
            out += produce(step)
        if step >= skew:
            out += consume(step - skew)
    return out


def _by_column(items, op, ncol):
    return [op(it, c) for c in range(ncol) for it in items]


def _by_item(items, op, ncol):
    return [op(it, c) for it in items for c in range(ncol)]


def _run(ops):
    for f in ops:
        f(None)


def _dot(a, b):
    return jnp.dot(a, b, preferred_element_type=F32)


def _bf(words):
    return pltpu.bitcast(words, BF16)


def _lo(w):
    return pltpu.bitcast(w << 16, F32)


def _hi(w):
    return pltpu.bitcast(w & jnp.uint32(0xFFFF0000), F32)


def _sublane_sum(t):
    t = t + pltpu.roll(t, 4, 0)
    t = t + pltpu.roll(t, 2, 0)
    return t + pltpu.roll(t, 1, 0)


def _col_bcast(row):
    return pltpu.bitcast(jnp.broadcast_to(row, (L, L)).T, U32)


def _round_bf16(x):
    return x.astype(BF16).astype(F32)


def _stats(xt):
    c = jnp.mean(xt[0], axis=-1, keepdims=True)
    s1 = s2 = None
    for x in xt:
        d = x - c
        s1 = d if s1 is None else s1 + d
        s2 = d * d if s2 is None else s2 + d * d
    m1 = jnp.sum(s1, axis=-1, keepdims=True) * (1.0 / M)
    m2 = jnp.sum(s2, axis=-1, keepdims=True) * (1.0 / M)
    var = jnp.maximum(m2 - m1 * m1, 0.0)
    return c + m1, jax.lax.rsqrt(var + EPS)


def _lhs16(xt):
    return [jnp.concatenate([x, jnp.ones_like(x)], axis=0).astype(BF16) for x in xt]


def _acc(d, k, v):
    d[k] = v if d.get(k) is None else d[k] + v
    return d[k]


def _kernel(x_hbm, wr_hbm, wq_hbm, wuk_hbm, ckv_hbm, wuv_hbm, wg_hbm, wu_hbm,
            wo_hbm, wd_hbm,
            o_ref,
            x_v, wr_v, wq_l, wuk_l, ckv_l, wuv_l, wg_l, wu_l, wo_l, wd_l,
            WQ32, WUKT32, CKV32, CKT32, WUV32, WG32, WU32, WO32, WD32,
            WUKF, WOF, WGF, WUF, CSG, CSU, XE, XO, sems):
    sem_ids = iter(range(64))

    def copy(src, dst, sem=None):
        sem = next(sem_ids) if sem is None else sem
        c = pltpu.make_async_copy(src, dst, sems.at[sem])
        c.start()
        if SCOPES:
            return _ScopedWait(c, "wait%02d" % sem)
        return c

    c_wq = copy(wq_hbm, wq_l)
    s_small = next(sem_ids)
    c_small = [copy(x_hbm, x_v, s_small), copy(wr_hbm, wr_v, s_small)]
    c_wuk = copy(wuk_hbm, wuk_l)
    c_ckv = copy(ckv_hbm, ckv_l)
    c_wuv = copy(wuv_hbm, wuv_l)
    c_wg = copy(wg_hbm, wg_l)
    c_wu = copy(wu_hbm, wu_l)
    wo_chunks = list(zip(WO_SPLIT[:-1], WO_SPLIT[1:]))
    c_wo = [copy(wo_hbm.at[pl.ds(h0 * D, (h1 - h0) * D)],
                 wo_l.at[pl.ds(h0 * D, (h1 - h0) * D)]) for h0, h1 in wo_chunks]
    c_wd = [copy(wd_hbm.at[:, pl.ds(nt * L, L)], wd_l.at[nt]) for nt in range(MT)]

    def swap_heads(src, dst32, rows):
        ch = 64

        def body(i, carry):
            w = src[pl.ds(pl.multiple_of(i * ch, ch), ch)]
            dst32[:, pl.ds(pl.multiple_of(i * (ch // 2), ch // 2), ch // 2), :] = (
                pltpu.bitcast(jnp.swapaxes(w, 0, 1), U32))
            return carry
        jax.lax.fori_loop(0, rows // ch, body, 0)

    def make_wukt():
        def body(i, carry):
            w = wuk_l[pl.ds(pl.multiple_of(i * L, L), L)]
            w = jnp.swapaxes(jnp.swapaxes(w, 0, 1), 1, 2)
            WUKT32[:, pl.ds(pl.multiple_of(i * W2, W2), W2), :] = pltpu.bitcast(w, U32)
            return carry
        jax.lax.fori_loop(0, CT, body, 0)

    def make_ck():
        def body(i, carry):
            for u in range(CK_UNROLL):
                kt = i * CK_UNROLL + u
                w = ckv_l[pl.ds(pl.multiple_of(kt * L, L), L), :]
                CKT32[kt] = pltpu.bitcast(w.T, U32)
                for ct in range(CT):
                    CKV32[ct, pl.ds(pl.multiple_of(kt * W2, W2), W2), :] = pltpu.bitcast(
                        w[:, ct * L:(ct + 1) * L], U32)
            return carry
        jax.lax.fori_loop(0, KT // CK_UNROLL, body, 0)

    def make_wgu(src, dst32):
        def body(i, carry):
            for u in range(GU_UNROLL):
                ft = i * GU_UNROLL + u
                w = src[pl.ds(pl.multiple_of(ft * L, L), L), :]
                dst32[ft] = pltpu.bitcast(w.T, U32)
            return carry
        n = (FT - 1) // GU_UNROLL
        jax.lax.fori_loop(0, n, body, 0)
        for ft in range(n * GU_UNROLL, FT - 1):
            dst32[ft] = pltpu.bitcast(src[ft * L:(ft + 1) * L, :].T, U32)
        w = src[(FT - 1) * L:FF, :]
        w = jnp.concatenate([w, jnp.zeros((L - F_TAIL, M), BF16)], axis=0)
        dst32[FT - 1] = pltpu.bitcast(w.T, U32)

    def widen(src32, dst, n):
        def body(i, carry):
            w = src32[i]
            dst[i, 0] = _lo(w)
            dst[i, 1] = _hi(w)
            return carry
        if n:
            jax.lax.fori_loop(0, n, body, 0)

    def make_wd(nt):
        def body(i, carry):
            r0 = pl.multiple_of(i * WD_ROWS, 16)
            WD32[nt, pl.ds(pl.multiple_of(i * (WD_ROWS // 2), 8), WD_ROWS // 2), :] = (
                pltpu.bitcast(wd_l[nt, pl.ds(r0, WD_ROWS), :], U32))
            return carry
        jax.lax.fori_loop(0, FF // WD_ROWS, body, 0)

    def make_wo(h0, h1, widen):
        def body(h, carry):
            rows = wo_l[pl.ds(pl.multiple_of(h * L, L), L), :]
            for nt in range(MT):
                w = pltpu.bitcast(rows[:, nt * L:(nt + 1) * L], U32)
                WO32[nt, pl.ds(pl.multiple_of(h * W2, W2), W2), :] = w
                if widen:
                    WOF[h, 0, nt] = _lo(w)
                    WOF[h, 1, nt] = _hi(w)
            return carry
        if h1 > h0:
            jax.lax.fori_loop(h0, h1, body, 0)

    sub = jax.lax.broadcasted_iota(jnp.int32, (R, L), 0)
    zero_v = []

    def link(a, dep):
        if dep is None:
            return a
        z = pltpu.bitcast(dep, U32) & zero_v[0]
        a32 = pltpu.bitcast(a, U32)
        return pltpu.bitcast(a32 | z[:a32.shape[0]], a.dtype)

    def make_xb(xt):
        for t in range(MT):
            w = _col_bcast(xt[t].astype(BF16)[0:1])
            XE[t * W2:(t + 1) * W2, :] = _lo(w)
            XO[t * W2:(t + 1) * W2, :] = _hi(w)

    def tile(ref32, lead, t):
        return _bf(ref32[lead, t * W2:(t + 1) * W2, :])

    def vpu_matvec_step(accs, ref_keys, s, dep):
        xe = link(XE[s * R:(s + 1) * R, :], dep)
        xo = XO[s * R:(s + 1) * R, :]
        for ref32, reff, lead in ref_keys:
            if reff is not None:
                we = reff[lead, 0, s * R:(s + 1) * R, :]
                wo_ = reff[lead, 1, s * R:(s + 1) * R, :]
            else:
                w = ref32[lead, s * R:(s + 1) * R, :]
                we, wo_ = _lo(w), _hi(w)
            _acc(accs, (id(ref32), lead), we * xe + wo_ * xo)

    def q_partial(oq, x_tile, t):
        lhs = _lhs16([x_tile])[0]

        def op(h):
            def f(dep):
                p = _dot(link(lhs, dep), tile(WQ32, h, t))
                _acc(oq, h, p)
                return p[:R]
            return f
        return [op(h) for h in range(H)]

    def attention(xt, first, oq):
        mu, rstd = _stats(xt)
        qscale = rstd * (D ** -0.5)
        nva = 0 if first else VA_HEADS
        nvo = 0 if first else VO_HEADS
        if first:
            c_wq.wait()
            swap_heads(wq_l, WQ32, M)
            for t in range(MT - 1):
                _run(q_partial(oq, xt[t], t))
            c_wuk.wait()
            make_wukt()
            if F32_P1:
                widen(WUKT32, WUKF, VA_HEADS)

        qh, qa = {}, {}

        def q_last(h, op):
            def f(dep):
                r = op(dep)
                o = oq[h]
                qh[h] = ((o[:R] - mu * o[R:]) * qscale).astype(BF16)
                return r
            return f

        def put_qa(h, ct, t):
            g, i = divmod(h, R)
            qa[g, ct] = t if (g, ct) not in qa else jnp.where(sub == i, t, qa[g, ct])

        def qabs_op(h, ct):
            def f(dep):
                t = _dot(link(qh[h], dep if LINK_P1 else None), tile(WUKT32, h, ct))
                put_qa(h, ct, t)
                return t
            return f

        ms = [q_last(h, op) for h, op in enumerate(q_partial(oq, xt[MT - 1], MT - 1))]
        ms += _by_item(range(nva, H - EDGE), qabs_op, CT)
        ms += _by_column(range(H - EDGE, H), qabs_op, CT)
        qw, aacc = {}, {}

        def qxlu_op(h):
            def f(dep):
                qw[h] = _col_bcast(qh[h][0:1])
                return pltpu.bitcast(qw[h][:R], F32)
            f.ready = lambda: h in qh
            return f

        def qa_vstep(h, k):
            def f(dep):
                w = qw[h][k * R:(k + 1) * R]
                ce, co = link(_lo(w), dep), _hi(w)
                for ct in range(CT):
                    r0 = ct * W2 + k * R
                    if F32_P1:
                        we, wo_ = WUKF[h, 0, r0:r0 + R, :], WUKF[h, 1, r0:r0 + R, :]
                    else:
                        w = WUKT32[h, r0:r0 + R, :]
                        we, wo_ = _lo(w), _hi(w)
                    _acc(aacc, (h, ct), we * ce + wo_ * co)
                if k == L // 16 - 1:
                    for ct in range(CT):
                        put_qa(h, ct, _sublane_sum(aacc[h, ct]))
                return aacc[h, 0]
            return _valu((4 if F32_P1 else 6) * CT + 2)(f)

        vs = [qxlu_op(h) for h in range(min(XLU_AHEAD, nva))]
        for h in range(nva):
            if h + XLU_AHEAD < nva:
                vs.append(qxlu_op(h + XLU_AHEAD))
            vs += [qa_vstep(h, k) for k in range(L // 16)]
        _cosched(ms, vs, P1_CFG)
        qabs = [jnp.concatenate([qa[g, ct] for g in range(H // R)], axis=0).astype(BF16)
                for ct in range(CT)]

        if first:
            c_ckv.wait()
            make_ck()
        nch = KT // KCHUNK
        sc, ps, lats = {}, {}, {}
        mxs, lss = [None] * nch, [None] * nch

        def score_op(kt, ct):
            def f(dep):
                _acc(sc, kt, _dot(qabs[ct], tile(CKT32, kt, ct)))
                j = kt // KCHUNK
                if ct == CT - 1 and kt == (j + 1) * KCHUNK - 1:
                    kts = range(j * KCHUNK, (j + 1) * KCHUNK)
                    mx = sc[kts[0]]
                    for k in kts[1:]:
                        mx = jnp.maximum(mx, sc[k])
                    mx = jnp.max(mx, axis=-1, keepdims=True)
                    lsum = None
                    for k in kts:
                        e = jnp.exp(sc[k] - mx)
                        lsum = e if lsum is None else lsum + e
                        ps[k] = e.astype(BF16)
                    mxs[j], lss[j] = mx, lsum
            return f

        def lat_op(kt, ct):
            def f(dep):
                _acc(lats, (kt // KCHUNK, ct), _dot(ps[kt], tile(CKV32, ct, kt)))
            return f

        def s_produce(j):
            kts = list(range(j * KCHUNK, (j + 1) * KCHUNK))
            if j == 0:
                return (_by_column(kts[:EDGE], score_op, CT)
                        + _by_item(kts[EDGE:], score_op, CT))
            return _by_item(kts, score_op, CT)

        def s_consume(j):
            return _by_column(range(j * KCHUNK, (j + 1) * KCHUNK), lat_op, CT)

        _run(_skewed(nch, SKEW_S, s_produce, s_consume))
        m = mxs[0]
        for t in mxs[1:]:
            m = jnp.maximum(m, t)
        alpha = [jnp.exp(t - m) for t in mxs]
        lsum = alpha[0] * lss[0]
        for a, t in zip(alpha[1:], lss[1:]):
            lsum = lsum + a * t
        inv = 1.0 / jnp.sum(lsum, axis=-1, keepdims=True)
        alpha = [a * inv for a in alpha]
        latg = {}
        for ct in range(CT):
            t = alpha[0] * lats[0, ct]
            for j in range(1, nch):
                t = t + alpha[j] * lats[j, ct]
            for g in range(H // R):
                latg[g, ct] = t[g * R:(g + 1) * R].astype(BF16)

        if first:
            c_wuv.wait()
            swap_heads(wuv_l, WUV32, DC)
        cacc, cbs, o = {}, {}, {}

        def ctx_op(h, ct):
            def f(dep):
                g, i = divmod(h, R)
                p = _dot(link(latg[g, ct], dep), tile(WUV32, h, ct))
                c = _acc(cacc, h, p)
                if ct == CT - 1:
                    cbs[h] = jnp.broadcast_to(c[i:i + 1], (R, D)).astype(BF16)
                return p
            return f

        def out_op(h, nt):
            def f(dep):
                t = _dot(link(cbs[h], dep if LINK_P3 else None), tile(WO32, nt, h))
                _acc(o, nt, t)
                return t
            return f

        if first:
            _run(_by_item(range(H), ctx_op, CT))
            c_wg.wait()
            make_wgu(wg_l, WG32)
            c_wu.wait()
            make_wgu(wu_l, WU32)
            if F32_P4:
                widen(WG32, WGF, VF_TILES)
                widen(WU32, WUF, VF_TILES)
            for c, (h0, h1) in enumerate(wo_chunks):
                c_wo[c].wait()
                hm = min(max(VO_HEADS if F32_P3 else 0, h0), h1)
                make_wo(h0, hm, True)
                make_wo(hm, h1, False)
                if c == len(wo_chunks) - 1:
                    _run(_by_column(range(h0, h1), out_op, MT))
                else:
                    _run(_by_item(range(h0, h1), out_op, MT))
            return [_round_bf16(xt[nt] + o[nt]) for nt in range(MT)]

        ms = _by_column(range(EDGE), ctx_op, CT) + _by_item(range(EDGE, nvo), ctx_op, CT)
        h0 = max(nvo, EDGE)

        def o_produce(i):
            return _by_item([h0 + i], ctx_op, CT)

        def o_consume(h):
            if h >= H - EDGE:
                return _by_column(range(H - EDGE, H), out_op, MT) if h == H - 1 else []
            return _by_item([h], out_op, MT)

        for step in range(H - h0 + SKEW_O):
            if step < H - h0:
                ms += o_produce(step)
            if step >= SKEW_O:
                ms += o_consume(h0 + step - SKEW_O)
        for h in range(nvo, h0):
            ms += o_consume(h)
        cw, ov = {}, {}

        def xlu_op(h):
            def f(dep):
                cw[h] = _col_bcast(cbs[h][0:1])
                return pltpu.bitcast(cw[h][:R], F32)
            f.ready = lambda: h in cbs
            return f

        def o_vstep(h, k):
            def f(dep):
                w = cw[h][k * R:(k + 1) * R]
                ce, co = link(_lo(w), dep), _hi(w)
                r0 = h * W2 + k * R
                for nt in range(MT):
                    if F32_P3:
                        we = WOF[h, 0, nt, k * R:(k + 1) * R, :]
                        wo_ = WOF[h, 1, nt, k * R:(k + 1) * R, :]
                    else:
                        w = WO32[nt, r0:r0 + R, :]
                        we, wo_ = _lo(w), _hi(w)
                    _acc(ov, nt, we * ce + wo_ * co)
                return ov[0]
            return _valu((4 if F32_P3 else 6) * MT + 2)(f)

        vs = [xlu_op(h) for h in range(min(XLU_AHEAD, nvo))]
        for h in range(nvo):
            if h + XLU_AHEAD < nvo:
                vs.append(xlu_op(h + XLU_AHEAD))
            vs += [o_vstep(h, k) for k in range(L // 16)]
        _cosched(ms, vs, P3_CFG)
        if nvo:
            o = {nt: o[nt] + _sublane_sum(ov[nt]) for nt in range(MT)}
        return [_round_bf16(xt[nt] + o[nt]) for nt in range(MT)]

    def ffn(xt, first, oq_next=None):
        mu, rstd = _stats(xt)
        lhs = _lhs16(xt)
        xn = [(x - mu) * rstd for x in xt]
        wr = wr_v[...].reshape(1, M).astype(F32)
        r = jnp.sum(jnp.concatenate(xn, axis=1) * wr, axis=-1, keepdims=True)
        gate = jax.nn.sigmoid(r)
        nvf = 0 if first else VF_TILES
        pre, acts, y = {}, {}, {}

        def finish(ft):
            g, u = pre[ft, 0] * rstd, pre[ft, 1] * rstd
            acts[ft] = (g * jax.nn.sigmoid(g) * u).astype(BF16)

        def gu_op(key, t):
            ft, which = key

            def f(dep):
                p = _dot(link(lhs[t], dep), tile((WG32, WU32)[which], ft, t))
                o = _acc(pre, key, p)
                if t == MT - 1:
                    if first and ft < VF_TILES:
                        (CSG, CSU)[which][ft] = o[R:]
                    pre[key] = o[:R] - mu * o[R:]
                    if which == 1:
                        finish(ft)
                return p[:R]
            return f

        def dn_op(ft, nt):
            def f(dep):
                rows = L if ft < FT - 1 else F_TAIL
                a = acts[ft] if rows == L else acts[ft][:, :rows]
                if first:
                    w = wd_l[nt, ft * L:ft * L + rows, :]
                else:
                    w = _bf(WD32[nt, ft * W2:ft * W2 + rows // 2, :])
                t = _dot(link(a, dep if LINK_P4 else None), w)
                _acc(y, nt, t)
                return t
            f.ready = lambda: ft in acts
            return f

        def gu_keys(fts):
            return [(ft, which) for ft in fts for which in range(2)]

        if first:
            _run(_by_column(gu_keys(range(2)), gu_op, MT))
            _run(_by_item(gu_keys(range(2, FT)), gu_op, MT))
            out = []
            for nt in range(MT):
                c_wd[nt].wait()
                _run([dn_op(ft, nt) for ft in range(FT)])
                out.append(_round_bf16(xt[nt] + xn[nt] + y[nt] * gate))
                if oq_next is not None:
                    if 0 < nt < MT - 1:
                        _run(q_partial(oq_next, out[nt - 1], nt - 1))
                    if nt == MT - 2:
                        _run(q_partial(oq_next, out[nt], nt))
                    if WD_COPY and nt < MT - 1:
                        make_wd(nt)
            return out
        else:
            mt = list(range(nvf, FT))
            vd = mt[:VD_TILES]
            md = [ft for ft in mt if ft not in vd] + list(range(nvf))
            last = md[-2:]

            def g_produce(i):
                if i == 0:
                    return _by_column(gu_keys(mt[:2]), gu_op, MT)
                return [] if i == 1 else _by_item(gu_keys([mt[i]]), gu_op, MT)

            def g_consume(ft):
                if ft in vd:
                    return []
                if ft in last:
                    return _by_column(last, dn_op, MT) if ft == last[-1] else []
                return _by_item([ft], dn_op, MT)

            ms = _skewed(len(mt), SKEW_F, g_produce, lambda i: g_consume(mt[i]))
            for ft in range(nvf):
                ms += g_consume(ft)
            facc, aw, yv = {}, {}, {}

            def f_vstep(fts, s):
                def f(dep):
                    keys = [(w, wf if F32_P4 else None, ft) for ft in fts
                            for w, wf in ((WG32, WGF), (WU32, WUF))]
                    vpu_matvec_step(facc, keys, s, dep)
                    if s == M // 16 - 1:
                        for ft in fts:
                            for wh, (w, cs) in enumerate(((WG32, CSG), (WU32, CSU))):
                                pre[ft, wh] = _sublane_sum(facc[id(w), ft]) - mu * cs[ft]
                            finish(ft)
                    return facc[id(WG32), fts[0]]
                return _valu((8 if F32_P4 else 12) * len(fts))(f)

            def dxlu_op(ft):
                def f(dep):
                    aw[ft] = _col_bcast(acts[ft][0:1])
                    return pltpu.bitcast(aw[ft][:R], F32)
                f.ready = lambda: ft in acts
                return f

            def d_vstep(ft, k):
                def f(dep):
                    w = aw[ft][k * R:(k + 1) * R]
                    ce, co = link(_lo(w), dep), _hi(w)
                    r0 = ft * W2 + k * R
                    for nt in range(MT):
                        w = WD32[nt, r0:r0 + R, :]
                        _acc(yv, nt, _lo(w) * ce + _hi(w) * co)
                    return yv[0]
                return _valu(6 * MT + 2)(f)

            if nvf:
                make_xb(xt)
            vs = [f_vstep(list(range(f0, min(nvf, f0 + VF_GROUP))), s)
                  for f0 in range(0, nvf, VF_GROUP) for s in range(M // 16)]
            pos = max(0, len(vs) - XLU_EARLY)
            for i, ft in enumerate(vd[:XLU_AHEAD]):
                vs.insert(pos + i, dxlu_op(ft))
            for i, ft in enumerate(vd):
                if i + XLU_AHEAD < len(vd):
                    vs.append(dxlu_op(vd[i + XLU_AHEAD]))
                vs += [d_vstep(ft, k) for k in range(L // 16)]
            _cosched(ms, vs, P4_CFG)
            if vd:
                y = {nt: y[nt] + _sublane_sum(yv[nt]) for nt in range(MT)}
        return [_round_bf16(xt[nt] + xn[nt] + y[nt] * gate) for nt in range(MT)]

    for c in c_small:
        c.wait()
    x = jnp.broadcast_to(x_v[...].astype(F32), (R, M))
    zero_v.append(pltpu.bitcast(x[:, :L], U32) & jnp.uint32(0xFFFF))
    xt = [x[:, t * L:(t + 1) * L] for t in range(MT)]
    xt = attention(xt, True, {})
    oq2 = {}
    xt = ffn(xt, True, oq2 if N_LAYERS > 1 else None)
    if N_LAYERS > 1:
        for nt in range(MT - 1 if WD_COPY else 0, MT):
            WD32[nt] = pltpu.bitcast(wd_l[nt], U32)
        xt = attention(xt, False, oq2)
        xt = ffn(xt, False)
    o_ref[...] = jnp.concatenate(xt, axis=1)[0:1].astype(o_ref.dtype)


@jax.jit
def pallas_interleave_layers__compressed_kv_cla__moe_arch_mod__decode_kernel(
    A_x: jax.Array,
    A_c_kv: jax.Array,
    A_w_q: jax.Array,
    A_w_uk: jax.Array,
    A_w_uv: jax.Array,
    A_w_o: jax.Array,
    B_x: jax.Array,
    B_w_r: jax.Array,
    B_w_gate: jax.Array,
    B_w_up: jax.Array,
    B_w_down: jax.Array,
):
    del B_x
    args = (
        A_x.reshape(1, M),
        B_w_r,
        A_w_q,
        A_w_uk,
        A_c_kv.reshape(SK, DC),
        A_w_uv,
        B_w_gate.T,
        B_w_up.T,
        A_w_o.reshape(H * D, M),
        B_w_down,
    )
    n_sems = 6 + len(WO_SPLIT) + MT
    scratch = [
        pltpu.VMEM((1, M), BF16),
        pltpu.VMEM((M,), BF16),
        pltpu.VMEM((M, H, D), BF16),
        pltpu.VMEM((DC, H, D), BF16),
        pltpu.VMEM((SK, DC), BF16),
        pltpu.VMEM((DC, H, D), BF16),
        pltpu.VMEM((FF, M), BF16),
        pltpu.VMEM((FF, M), BF16),
        pltpu.VMEM((H * D, M), BF16),
        pltpu.VMEM((MT, FF, L), BF16),
        pltpu.VMEM((H, M // 2, D), U32),
        pltpu.VMEM((H, DC // 2, L), U32),
        pltpu.VMEM((CT, SK // 2, L), U32),
        pltpu.VMEM((KT, DC // 2, L), U32),
        pltpu.VMEM((H, DC // 2, D), U32),
        pltpu.VMEM((FT, M // 2, L), U32),
        pltpu.VMEM((FT, M // 2, L), U32),
        pltpu.VMEM((MT, H * D // 2, L), U32),
        pltpu.VMEM((MT, FF // 2, L), U32),
        pltpu.VMEM((max(VA_HEADS, 1), 2, DC // 2, L), F32),
        pltpu.VMEM((max(VO_HEADS, 1), 2, MT, W2, L), F32),
        pltpu.VMEM((max(VF_TILES, 1), 2, M // 2, L), F32),
        pltpu.VMEM((max(VF_TILES, 1), 2, M // 2, L), F32),
        pltpu.VMEM((FT, R, L), F32),
        pltpu.VMEM((FT, R, L), F32),
        pltpu.VMEM((M // 2, L), F32),
        pltpu.VMEM((M // 2, L), F32),
        pltpu.SemaphoreType.DMA((n_sems,)),
    ]
    out = pl.pallas_call(
        _kernel,
        out_shape=jax.ShapeDtypeStruct((1, M), A_x.dtype),
        in_specs=[pl.BlockSpec(memory_space=pl.ANY)] * len(args),
        out_specs=pl.BlockSpec(memory_space=pltpu.VMEM),
        scratch_shapes=scratch,
        compiler_params=pltpu.CompilerParams(
            vmem_limit_bytes=100 * 1024 * 1024,
            disable_semaphore_checks=True),
        name="mla_moe_decode",
    )(*args)
    return out.reshape(1, 1, M)
```

```python
import jax
import jax.numpy as jnp
import jax.experimental.pallas as pl
import jax.experimental.pallas.tpu as pltpu

F32 = jnp.float32
BF16 = jnp.bfloat16
U32 = jnp.uint32

H = 32
D = 128
M = 640
DC = 512
SK = 4096
FF = 1728
EPS = 1e-5
R = 8
L = 128
W2 = L // 2

MT = M // L
CT = DC // L
KT = SK // L
FT = -(-FF // L)
F_TAIL = FF - (FT - 1) * L
KCHUNK = 8
WO_SPLIT = (0, 10, 20, 28, 32)

N_LAYERS = 2
SKEW_S = 1
SKEW_O = 6
SKEW_F = 5
EDGE = 4

VA_HEADS = 11
P1_CFG = (420, 2.5, 16, 140, 2, 560)
VO_HEADS = 18
P3_CFG = (460, 2.6, 24, 150, 1, 800)
XLU_AHEAD = 2
WD_COPY = False
WD_P2 = True
WD_STEP = 128
P2_CFG = (100, 0.4, 16, 150, 4, 200)
CK_UNROLL = 4
GU_UNROLL = 3
WD_ROWS = 432
F32_P1 = True
F32_P3 = True
F32_P4 = True
LINK_P1 = False
LINK_P3 = False
LINK_P4 = False
VF_TILES = 6
VF_GROUP = 2
VD_TILES = 1
XLU_EARLY = 10
P4_CFG = (260, 2.4, 24, 150, 1, 520)


SCOPES = False


class _ScopedWait:
    def __init__(self, c, name):
        self.c, self.name = c, name

    def wait(self):
        with jax.named_scope(self.name):
            self.c.wait()


def _always():
    return True


def _cosched(ms, vs, cfg):
    vstart, rate, lag_v, lag_m, nlink, lstart = cfg
    mres, vres = [], []
    j, tv = 0, vstart

    def latest(res, t):
        for tt, val in reversed(res):
            if tt <= t:
                return val
        return None

    def emit_v(dep):
        nonlocal j, tv
        val = vs[j](dep)
        tv += getattr(vs[j], "valu", 0) / rate
        vres.append((tv, val))
        j += 1

    for i, m in enumerate(ms):
        t = 8 * i
        while not getattr(m, "ready", _always)():
            emit_v(None)
        dep = None
        if i % nlink == 0 and j < len(vs) and t >= lstart:
            dep = latest(vres, t - lag_v)
        mres.append((t, m(dep)))
        while j < len(vs) and tv <= t + 8 and getattr(vs[j], "ready", _always)():
            emit_v(latest(mres, tv - lag_m) if j % 2 == 0 else None)
    while j < len(vs):
        emit_v(None)


def _valu(n):
    def deco(f):
        f.valu = n
        return f
    return deco


def _skewed(n, skew, produce, consume):
    out = []
    for step in range(n + skew):
        if step < n:
            out += produce(step)
        if step >= skew:
            out += consume(step - skew)
    return out


def _by_column(items, op, ncol):
    return [op(it, c) for c in range(ncol) for it in items]


def _by_item(items, op, ncol):
    return [op(it, c) for it in items for c in range(ncol)]


def _run(ops):
    for f in ops:
        f(None)


def _dot(a, b):
    return jnp.dot(a, b, preferred_element_type=F32)


def _bf(words):
    return pltpu.bitcast(words, BF16)


def _lo(w):
    return pltpu.bitcast(w << 16, F32)


def _hi(w):
    return pltpu.bitcast(w & jnp.uint32(0xFFFF0000), F32)


def _sublane_sum(t):
    t = t + pltpu.roll(t, 4, 0)
    t = t + pltpu.roll(t, 2, 0)
    return t + pltpu.roll(t, 1, 0)


def _col_bcast(row):
    return pltpu.bitcast(jnp.broadcast_to(row, (L, L)).T, U32)


def _round_bf16(x):
    return x.astype(BF16).astype(F32)


def _stats(xt):
    c = jnp.mean(xt[0], axis=-1, keepdims=True)
    s1 = s2 = None
    for x in xt:
        d = x - c
        s1 = d if s1 is None else s1 + d
        s2 = d * d if s2 is None else s2 + d * d
    m1 = jnp.sum(s1, axis=-1, keepdims=True) * (1.0 / M)
    m2 = jnp.sum(s2, axis=-1, keepdims=True) * (1.0 / M)
    var = jnp.maximum(m2 - m1 * m1, 0.0)
    return c + m1, jax.lax.rsqrt(var + EPS)


def _lhs16(xt):
    return [jnp.concatenate([x, jnp.ones_like(x)], axis=0).astype(BF16) for x in xt]


def _acc(d, k, v):
    d[k] = v if d.get(k) is None else d[k] + v
    return d[k]


def _kernel(x_hbm, wr_hbm, wq_hbm, wuk_hbm, ckv_hbm, wuv_hbm, wg_hbm, wu_hbm,
            wo_hbm, wd_hbm,
            o_ref,
            x_v, wr_v, wq_l, wuk_l, ckv_l, wuv_l, wg_l, wu_l, wo_l, wd_l,
            WQ32, WUKT32, CKV32, CKT32, WUV32, WG32, WU32, WO32, WD32,
            WUKF, WOF, WGF, WUF, CSG, CSU, XE, XO, sems):
    sem_ids = iter(range(64))

    def copy(src, dst, sem=None):
        sem = next(sem_ids) if sem is None else sem
        c = pltpu.make_async_copy(src, dst, sems.at[sem])
        c.start()
        if SCOPES:
            return _ScopedWait(c, "wait%02d" % sem)
        return c

    c_wq = copy(wq_hbm, wq_l)
    s_small = next(sem_ids)
    c_small = [copy(x_hbm, x_v, s_small), copy(wr_hbm, wr_v, s_small)]
    c_wuk = copy(wuk_hbm, wuk_l)
    c_ckv = copy(ckv_hbm, ckv_l)
    c_wuv = copy(wuv_hbm, wuv_l)
    c_wg = copy(wg_hbm, wg_l)
    c_wu = copy(wu_hbm, wu_l)
    wo_chunks = list(zip(WO_SPLIT[:-1], WO_SPLIT[1:]))
    c_wo = [copy(wo_hbm.at[pl.ds(h0 * D, (h1 - h0) * D)],
                 wo_l.at[pl.ds(h0 * D, (h1 - h0) * D)]) for h0, h1 in wo_chunks]
    c_wd = [copy(wd_hbm.at[:, pl.ds(nt * L, L)], wd_l.at[nt]) for nt in range(MT)]

    def swap_heads(src, dst32, rows):
        ch = 64

        def body(i, carry):
            w = src[pl.ds(pl.multiple_of(i * ch, ch), ch)]
            dst32[:, pl.ds(pl.multiple_of(i * (ch // 2), ch // 2), ch // 2), :] = (
                pltpu.bitcast(jnp.swapaxes(w, 0, 1), U32))
            return carry
        jax.lax.fori_loop(0, rows // ch, body, 0)

    def make_wukt():
        def body(i, carry):
            w = wuk_l[pl.ds(pl.multiple_of(i * L, L), L)]
            w = jnp.swapaxes(jnp.swapaxes(w, 0, 1), 1, 2)
            WUKT32[:, pl.ds(pl.multiple_of(i * W2, W2), W2), :] = pltpu.bitcast(w, U32)
            return carry
        jax.lax.fori_loop(0, CT, body, 0)

    def make_ck():
        def body(i, carry):
            for u in range(CK_UNROLL):
                kt = i * CK_UNROLL + u
                w = ckv_l[pl.ds(pl.multiple_of(kt * L, L), L), :]
                CKT32[kt] = pltpu.bitcast(w.T, U32)
                for ct in range(CT):
                    CKV32[ct, pl.ds(pl.multiple_of(kt * W2, W2), W2), :] = pltpu.bitcast(
                        w[:, ct * L:(ct + 1) * L], U32)
            return carry
        jax.lax.fori_loop(0, KT // CK_UNROLL, body, 0)

    def make_wgu(src, dst32):
        def body(i, carry):
            for u in range(GU_UNROLL):
                ft = i * GU_UNROLL + u
                w = src[pl.ds(pl.multiple_of(ft * L, L), L), :]
                dst32[ft] = pltpu.bitcast(w.T, U32)
            return carry
        n = (FT - 1) // GU_UNROLL
        jax.lax.fori_loop(0, n, body, 0)
        for ft in range(n * GU_UNROLL, FT - 1):
            dst32[ft] = pltpu.bitcast(src[ft * L:(ft + 1) * L, :].T, U32)
        w = src[(FT - 1) * L:FF, :]
        w = jnp.concatenate([w, jnp.zeros((L - F_TAIL, M), BF16)], axis=0)
        dst32[FT - 1] = pltpu.bitcast(w.T, U32)

    def widen(src32, dst, n):
        def body(i, carry):
            w = src32[i]
            dst[i, 0] = _lo(w)
            dst[i, 1] = _hi(w)
            return carry
        if n:
            jax.lax.fori_loop(0, n, body, 0)

    def make_wd(nt):
        def body(i, carry):
            r0 = pl.multiple_of(i * WD_ROWS, 16)
            WD32[nt, pl.ds(pl.multiple_of(i * (WD_ROWS // 2), 8), WD_ROWS // 2), :] = (
                pltpu.bitcast(wd_l[nt, pl.ds(r0, WD_ROWS), :], U32))
            return carry
        jax.lax.fori_loop(0, FF // WD_ROWS, body, 0)

    def make_wo(h0, h1, widen):
        def body(h, carry):
            rows = wo_l[pl.ds(pl.multiple_of(h * L, L), L), :]
            for nt in range(MT):
                w = pltpu.bitcast(rows[:, nt * L:(nt + 1) * L], U32)
                WO32[nt, pl.ds(pl.multiple_of(h * W2, W2), W2), :] = w
                if widen:
                    WOF[h, 0, nt] = _lo(w)
                    WOF[h, 1, nt] = _hi(w)
            return carry
        if h1 > h0:
            jax.lax.fori_loop(h0, h1, body, 0)

    sub = jax.lax.broadcasted_iota(jnp.int32, (R, L), 0)
    zero_v, zero_s = [], []

    def link(a, dep):
        if dep is None:
            return a
        z = pltpu.bitcast(dep, U32) & zero_v[0]
        a32 = pltpu.bitcast(a, U32)
        n = a32.shape[0]
        if n > R:
            a32 = jnp.concatenate([a32[:R] | z, a32[R:]], axis=0)
        else:
            a32 = a32 | z[:n]
        return pltpu.bitcast(a32, a.dtype)

    def make_xb(xt):
        for t in range(MT):
            w = _col_bcast(xt[t].astype(BF16)[0:1])
            XE[t * W2:(t + 1) * W2, :] = _lo(w)
            XO[t * W2:(t + 1) * W2, :] = _hi(w)

    def tile(ref32, lead, t):
        return _bf(ref32[lead, t * W2:(t + 1) * W2, :])

    def vpu_matvec_step(accs, ref_keys, s, dep):
        xe = link(XE[s * R:(s + 1) * R, :], dep)
        xo = XO[s * R:(s + 1) * R, :]
        for ref32, reff, lead in ref_keys:
            if reff is not None:
                we = reff[lead, 0, s * R:(s + 1) * R, :]
                wo_ = reff[lead, 1, s * R:(s + 1) * R, :]
            else:
                w = ref32[lead, s * R:(s + 1) * R, :]
                we, wo_ = _lo(w), _hi(w)
            _acc(accs, (id(ref32), lead), we * xe + wo_ * xo)

    def q_partial(oq, x_tile, t):
        lhs = _lhs16([x_tile])[0]

        def op(h):
            def f(dep):
                p = _dot(link(lhs, dep), tile(WQ32, h, t))
                _acc(oq, h, p)
                return p[:R]
            return f
        return [op(h) for h in range(H)]

    def attention(xt, first, oq):
        mu, rstd = _stats(xt)
        qscale = rstd * (D ** -0.5)
        nva = 0 if first else VA_HEADS
        nvo = 0 if first else VO_HEADS
        if first:
            c_wq.wait()
            swap_heads(wq_l, WQ32, M)
            for t in range(MT - 1):
                _run(q_partial(oq, xt[t], t))
            c_wuk.wait()
            make_wukt()
            if F32_P1:
                widen(WUKT32, WUKF, VA_HEADS)

        qh, qa = {}, {}

        def q_last(h, op):
            def f(dep):
                r = op(dep)
                o = oq[h]
                qh[h] = ((o[:R] - mu * o[R:]) * qscale).astype(BF16)
                return r
            return f

        def put_qa(h, ct, t):
            g, i = divmod(h, R)
            qa[g, ct] = t if (g, ct) not in qa else jnp.where(sub == i, t, qa[g, ct])

        def qabs_op(h, ct):
            def f(dep):
                t = _dot(link(qh[h], dep if LINK_P1 else None), tile(WUKT32, h, ct))
                put_qa(h, ct, t)
                return t
            return f

        ms = [q_last(h, op) for h, op in enumerate(q_partial(oq, xt[MT - 1], MT - 1))]
        ms += _by_item(range(nva, H - EDGE), qabs_op, CT)
        ms += _by_column(range(H - EDGE, H), qabs_op, CT)
        qw, aacc = {}, {}

        def qxlu_op(h):
            def f(dep):
                qw[h] = _col_bcast(qh[h][0:1])
                return pltpu.bitcast(qw[h][:R], F32)
            f.ready = lambda: h in qh
            return f

        def qa_vstep(h, k):
            def f(dep):
                w = qw[h][k * R:(k + 1) * R]
                ce, co = link(_lo(w), dep), _hi(w)
                for ct in range(CT):
                    r0 = ct * W2 + k * R
                    if F32_P1:
                        we, wo_ = WUKF[h, 0, r0:r0 + R, :], WUKF[h, 1, r0:r0 + R, :]
                    else:
                        w = WUKT32[h, r0:r0 + R, :]
                        we, wo_ = _lo(w), _hi(w)
                    _acc(aacc, (h, ct), we * ce + wo_ * co)
                if k == L // 16 - 1:
                    for ct in range(CT):
                        put_qa(h, ct, _sublane_sum(aacc[h, ct]))
                return aacc[h, 0]
            return _valu((4 if F32_P1 else 6) * CT + 2)(f)

        vs = [qxlu_op(h) for h in range(min(XLU_AHEAD, nva))]
        for h in range(nva):
            if h + XLU_AHEAD < nva:
                vs.append(qxlu_op(h + XLU_AHEAD))
            vs += [qa_vstep(h, k) for k in range(L // 16)]
        _cosched(ms, vs, P1_CFG)
        qabs = [jnp.concatenate([qa[g, ct] for g in range(H // R)], axis=0).astype(BF16)
                for ct in range(CT)]

        if first:
            c_ckv.wait()
            make_ck()
        nch = KT // KCHUNK
        sc, ps, lats = {}, {}, {}
        mxs, lss = [None] * nch, [None] * nch

        def score_op(kt, ct):
            def f(dep):
                p = _dot(link(qabs[ct], dep), tile(CKT32, kt, ct))
                _acc(sc, kt, p)
                j = kt // KCHUNK
                if ct == CT - 1 and kt == (j + 1) * KCHUNK - 1:
                    kts = range(j * KCHUNK, (j + 1) * KCHUNK)
                    mx = sc[kts[0]]
                    for k in kts[1:]:
                        mx = jnp.maximum(mx, sc[k])
                    mx = jnp.max(mx, axis=-1, keepdims=True)
                    lsum = None
                    for k in kts:
                        e = jnp.exp(sc[k] - mx)
                        lsum = e if lsum is None else lsum + e
                        ps[k] = e.astype(BF16)
                    mxs[j], lss[j] = mx, lsum
                return p[:R]
            return f

        def lat_op(kt, ct):
            def f(dep):
                p = _dot(link(ps[kt], dep), tile(CKV32, ct, kt))
                _acc(lats, (kt // KCHUNK, ct), p)
                return p[:R]
            return f

        def s_produce(j):
            kts = list(range(j * KCHUNK, (j + 1) * KCHUNK))
            if j == 0:
                return (_by_column(kts[:EDGE], score_op, CT)
                        + _by_item(kts[EDGE:], score_op, CT))
            return _by_item(kts, score_op, CT)

        def s_consume(j):
            return _by_column(range(j * KCHUNK, (j + 1) * KCHUNK), lat_op, CT)

        def wd_copy_op(nt, r0, rows):
            def f(dep):
                w = pltpu.bitcast(wd_l[nt, r0:r0 + rows, :], U32)
                w = link(w, dep)
                d0 = jnp.clip(zero_s[0] + r0 // 2, 0, (FF - rows) // 2)
                WD32[nt, pl.ds(pl.multiple_of(d0, R), rows // 2), :] = w
                return pltpu.bitcast(w[:R], F32)
            return _valu(rows // 16)(f)

        cs = []
        if not first and WD_P2:
            cs = [wd_copy_op(nt, r0, min(WD_STEP, FF - r0))
                  for nt in range(MT) for r0 in range(0, FF, WD_STEP)]
        _cosched(_skewed(nch, SKEW_S, s_produce, s_consume), cs, P2_CFG)
        m = mxs[0]
        for t in mxs[1:]:
            m = jnp.maximum(m, t)
        alpha = [jnp.exp(t - m) for t in mxs]
        lsum = alpha[0] * lss[0]
        for a, t in zip(alpha[1:], lss[1:]):
            lsum = lsum + a * t
        inv = 1.0 / jnp.sum(lsum, axis=-1, keepdims=True)
        alpha = [a * inv for a in alpha]
        latg = {}
        for ct in range(CT):
            t = alpha[0] * lats[0, ct]
            for j in range(1, nch):
                t = t + alpha[j] * lats[j, ct]
            for g in range(H // R):
                latg[g, ct] = t[g * R:(g + 1) * R].astype(BF16)

        if first:
            c_wuv.wait()
            swap_heads(wuv_l, WUV32, DC)
        cacc, cbs, o = {}, {}, {}

        def ctx_op(h, ct):
            def f(dep):
                g, i = divmod(h, R)
                p = _dot(link(latg[g, ct], dep), tile(WUV32, h, ct))
                c = _acc(cacc, h, p)
                if ct == CT - 1:
                    cbs[h] = jnp.broadcast_to(c[i:i + 1], (R, D)).astype(BF16)
                return p
            return f

        def out_op(h, nt):
            def f(dep):
                t = _dot(link(cbs[h], dep if LINK_P3 else None), tile(WO32, nt, h))
                _acc(o, nt, t)
                return t
            return f

        if first:
            _run(_by_item(range(H), ctx_op, CT))
            c_wg.wait()
            make_wgu(wg_l, WG32)
            c_wu.wait()
            make_wgu(wu_l, WU32)
            if F32_P4:
                widen(WG32, WGF, VF_TILES)
                widen(WU32, WUF, VF_TILES)
            for c, (h0, h1) in enumerate(wo_chunks):
                c_wo[c].wait()
                hm = min(max(VO_HEADS if F32_P3 else 0, h0), h1)
                make_wo(h0, hm, True)
                make_wo(hm, h1, False)
                if c == len(wo_chunks) - 1:
                    _run(_by_column(range(h0, h1), out_op, MT))
                else:
                    _run(_by_item(range(h0, h1), out_op, MT))
            return [_round_bf16(xt[nt] + o[nt]) for nt in range(MT)]

        ms = _by_column(range(EDGE), ctx_op, CT) + _by_item(range(EDGE, nvo), ctx_op, CT)
        h0 = max(nvo, EDGE)

        def o_produce(i):
            return _by_item([h0 + i], ctx_op, CT)

        def o_consume(h):
            if h >= H - EDGE:
                return _by_column(range(H - EDGE, H), out_op, MT) if h == H - 1 else []
            return _by_item([h], out_op, MT)

        for step in range(H - h0 + SKEW_O):
            if step < H - h0:
                ms += o_produce(step)
            if step >= SKEW_O:
                ms += o_consume(h0 + step - SKEW_O)
        for h in range(nvo, h0):
            ms += o_consume(h)
        cw, ov = {}, {}

        def xlu_op(h):
            def f(dep):
                cw[h] = _col_bcast(cbs[h][0:1])
                return pltpu.bitcast(cw[h][:R], F32)
            f.ready = lambda: h in cbs
            return f

        def o_vstep(h, k):
            def f(dep):
                w = cw[h][k * R:(k + 1) * R]
                ce, co = link(_lo(w), dep), _hi(w)
                r0 = h * W2 + k * R
                for nt in range(MT):
                    if F32_P3:
                        we = WOF[h, 0, nt, k * R:(k + 1) * R, :]
                        wo_ = WOF[h, 1, nt, k * R:(k + 1) * R, :]
                    else:
                        w = WO32[nt, r0:r0 + R, :]
                        we, wo_ = _lo(w), _hi(w)
                    _acc(ov, nt, we * ce + wo_ * co)
                return ov[0]
            return _valu((4 if F32_P3 else 6) * MT + 2)(f)

        vs = [xlu_op(h) for h in range(min(XLU_AHEAD, nvo))]
        for h in range(nvo):
            if h + XLU_AHEAD < nvo:
                vs.append(xlu_op(h + XLU_AHEAD))
            vs += [o_vstep(h, k) for k in range(L // 16)]
        _cosched(ms, vs, P3_CFG)
        if nvo:
            o = {nt: o[nt] + _sublane_sum(ov[nt]) for nt in range(MT)}
        return [_round_bf16(xt[nt] + o[nt]) for nt in range(MT)]

    def ffn(xt, first, oq_next=None):
        mu, rstd = _stats(xt)
        lhs = _lhs16(xt)
        xn = [(x - mu) * rstd for x in xt]
        wr = wr_v[...].reshape(1, M).astype(F32)
        r = jnp.sum(jnp.concatenate(xn, axis=1) * wr, axis=-1, keepdims=True)
        gate = jax.nn.sigmoid(r)
        nvf = 0 if first else VF_TILES
        pre, acts, y = {}, {}, {}

        def finish(ft):
            g, u = pre[ft, 0] * rstd, pre[ft, 1] * rstd
            acts[ft] = (g * jax.nn.sigmoid(g) * u).astype(BF16)

        def gu_op(key, t):
            ft, which = key

            def f(dep):
                p = _dot(link(lhs[t], dep), tile((WG32, WU32)[which], ft, t))
                o = _acc(pre, key, p)
                if t == MT - 1:
                    if first and ft < VF_TILES:
                        (CSG, CSU)[which][ft] = o[R:]
                    pre[key] = o[:R] - mu * o[R:]
                    if which == 1:
                        finish(ft)
                return p[:R]
            return f

        def dn_op(ft, nt):
            def f(dep):
                rows = L if ft < FT - 1 else F_TAIL
                a = acts[ft] if rows == L else acts[ft][:, :rows]
                if first:
                    w = wd_l[nt, ft * L:ft * L + rows, :]
                else:
                    w = _bf(WD32[nt, ft * W2:ft * W2 + rows // 2, :])
                t = _dot(link(a, dep if LINK_P4 else None), w)
                _acc(y, nt, t)
                return t
            f.ready = lambda: ft in acts
            return f

        def gu_keys(fts):
            return [(ft, which) for ft in fts for which in range(2)]

        if first:
            _run(_by_column(gu_keys(range(2)), gu_op, MT))
            _run(_by_item(gu_keys(range(2, FT)), gu_op, MT))
            out = []
            for nt in range(MT):
                c_wd[nt].wait()
                _run([dn_op(ft, nt) for ft in range(FT)])
                out.append(_round_bf16(xt[nt] + xn[nt] + y[nt] * gate))
                if oq_next is not None:
                    if 0 < nt < MT - 1:
                        _run(q_partial(oq_next, out[nt - 1], nt - 1))
                    if nt == MT - 2:
                        _run(q_partial(oq_next, out[nt], nt))
                    if WD_COPY and nt < MT - 1:
                        make_wd(nt)
            return out
        else:
            mt = list(range(nvf, FT))
            vd = mt[:VD_TILES]
            md = [ft for ft in mt if ft not in vd] + list(range(nvf))
            last = md[-2:]

            def g_produce(i):
                if i == 0:
                    return _by_column(gu_keys(mt[:2]), gu_op, MT)
                return [] if i == 1 else _by_item(gu_keys([mt[i]]), gu_op, MT)

            def g_consume(ft):
                if ft in vd:
                    return []
                if ft in last:
                    return _by_column(last, dn_op, MT) if ft == last[-1] else []
                return _by_item([ft], dn_op, MT)

            ms = _skewed(len(mt), SKEW_F, g_produce, lambda i: g_consume(mt[i]))
            for ft in range(nvf):
                ms += g_consume(ft)
            facc, aw, yv = {}, {}, {}

            def f_vstep(fts, s):
                def f(dep):
                    keys = [(w, wf if F32_P4 else None, ft) for ft in fts
                            for w, wf in ((WG32, WGF), (WU32, WUF))]
                    vpu_matvec_step(facc, keys, s, dep)
                    if s == M // 16 - 1:
                        for ft in fts:
                            for wh, (w, cs) in enumerate(((WG32, CSG), (WU32, CSU))):
                                pre[ft, wh] = _sublane_sum(facc[id(w), ft]) - mu * cs[ft]
                            finish(ft)
                    return facc[id(WG32), fts[0]]
                return _valu((8 if F32_P4 else 12) * len(fts))(f)

            def dxlu_op(ft):
                def f(dep):
                    aw[ft] = _col_bcast(acts[ft][0:1])
                    return pltpu.bitcast(aw[ft][:R], F32)
                f.ready = lambda: ft in acts
                return f

            def d_vstep(ft, k):
                def f(dep):
                    w = aw[ft][k * R:(k + 1) * R]
                    ce, co = link(_lo(w), dep), _hi(w)
                    r0 = ft * W2 + k * R
                    for nt in range(MT):
                        w = WD32[nt, r0:r0 + R, :]
                        _acc(yv, nt, _lo(w) * ce + _hi(w) * co)
                    return yv[0]
                return _valu(6 * MT + 2)(f)

            if nvf:
                make_xb(xt)
            vs = [f_vstep(list(range(f0, min(nvf, f0 + VF_GROUP))), s)
                  for f0 in range(0, nvf, VF_GROUP) for s in range(M // 16)]
            pos = max(0, len(vs) - XLU_EARLY)
            for i, ft in enumerate(vd[:XLU_AHEAD]):
                vs.insert(pos + i, dxlu_op(ft))
            for i, ft in enumerate(vd):
                if i + XLU_AHEAD < len(vd):
                    vs.append(dxlu_op(vd[i + XLU_AHEAD]))
                vs += [d_vstep(ft, k) for k in range(L // 16)]
            _cosched(ms, vs, P4_CFG)
            if vd:
                y = {nt: y[nt] + _sublane_sum(yv[nt]) for nt in range(MT)}
        return [_round_bf16(xt[nt] + xn[nt] + y[nt] * gate) for nt in range(MT)]

    for c in c_small:
        c.wait()
    x = jnp.broadcast_to(x_v[...].astype(F32), (R, M))
    zero_v.append(pltpu.bitcast(x[:, :L], U32) & jnp.uint32(0xFFFF))
    zero_s.append(jnp.max(zero_v[0].astype(jnp.int32)))
    xt = [x[:, t * L:(t + 1) * L] for t in range(MT)]
    xt = attention(xt, True, {})
    oq2 = {}
    xt = ffn(xt, True, oq2 if N_LAYERS > 1 else None)
    if N_LAYERS > 1:
        if not WD_P2:
            for nt in range(MT - 1 if WD_COPY else 0, MT):
                WD32[nt] = pltpu.bitcast(wd_l[nt], U32)
        xt = attention(xt, False, oq2)
        xt = ffn(xt, False)
    o_ref[...] = jnp.concatenate(xt, axis=1)[0:1].astype(o_ref.dtype)


@jax.jit
def pallas_interleave_layers__compressed_kv_cla__moe_arch_mod__decode_kernel(
    A_x: jax.Array,
    A_c_kv: jax.Array,
    A_w_q: jax.Array,
    A_w_uk: jax.Array,
    A_w_uv: jax.Array,
    A_w_o: jax.Array,
    B_x: jax.Array,
    B_w_r: jax.Array,
    B_w_gate: jax.Array,
    B_w_up: jax.Array,
    B_w_down: jax.Array,
):
    del B_x
    args = (
        A_x.reshape(1, M),
        B_w_r,
        A_w_q,
        A_w_uk,
        A_c_kv.reshape(SK, DC),
        A_w_uv,
        B_w_gate.T,
        B_w_up.T,
        A_w_o.reshape(H * D, M),
        B_w_down,
    )
    n_sems = 6 + len(WO_SPLIT) + MT
    scratch = [
        pltpu.VMEM((1, M), BF16),
        pltpu.VMEM((M,), BF16),
        pltpu.VMEM((M, H, D), BF16),
        pltpu.VMEM((DC, H, D), BF16),
        pltpu.VMEM((SK, DC), BF16),
        pltpu.VMEM((DC, H, D), BF16),
        pltpu.VMEM((FF, M), BF16),
        pltpu.VMEM((FF, M), BF16),
        pltpu.VMEM((H * D, M), BF16),
        pltpu.VMEM((MT, FF, L), BF16),
        pltpu.VMEM((H, M // 2, D), U32),
        pltpu.VMEM((H, DC // 2, L), U32),
        pltpu.VMEM((CT, SK // 2, L), U32),
        pltpu.VMEM((KT, DC // 2, L), U32),
        pltpu.VMEM((H, DC // 2, D), U32),
        pltpu.VMEM((FT, M // 2, L), U32),
        pltpu.VMEM((FT, M // 2, L), U32),
        pltpu.VMEM((MT, H * D // 2, L), U32),
        pltpu.VMEM((MT, FF // 2, L), U32),
        pltpu.VMEM((max(VA_HEADS, 1), 2, DC // 2, L), F32),
        pltpu.VMEM((max(VO_HEADS, 1), 2, MT, W2, L), F32),
        pltpu.VMEM((max(VF_TILES, 1), 2, M // 2, L), F32),
        pltpu.VMEM((max(VF_TILES, 1), 2, M // 2, L), F32),
        pltpu.VMEM((FT, R, L), F32),
        pltpu.VMEM((FT, R, L), F32),
        pltpu.VMEM((M // 2, L), F32),
        pltpu.VMEM((M // 2, L), F32),
        pltpu.SemaphoreType.DMA((n_sems,)),
    ]
    out = pl.pallas_call(
        _kernel,
        out_shape=jax.ShapeDtypeStruct((1, M), A_x.dtype),
        in_specs=[pl.BlockSpec(memory_space=pl.ANY)] * len(args),
        out_specs=pl.BlockSpec(memory_space=pltpu.VMEM),
        scratch_shapes=scratch,
        compiler_params=pltpu.CompilerParams(
            vmem_limit_bytes=100 * 1024 * 1024,
            disable_semaphore_checks=True),
        name="mla_moe_decode",
    )(*args)
    return out.reshape(1, 1, M)
```

```python
import jax
import jax.numpy as jnp
import jax.experimental.pallas as pl
import jax.experimental.pallas.tpu as pltpu

F32 = jnp.float32
BF16 = jnp.bfloat16
U32 = jnp.uint32

H = 32
D = 128
M = 640
DC = 512
SK = 4096
FF = 1728
EPS = 1e-5
R = 8
L = 128
W2 = L // 2

MT = M // L
CT = DC // L
KT = SK // L
FT = -(-FF // L)
F_TAIL = FF - (FT - 1) * L
KCHUNK = 8
WO_SPLIT = (0, 10, 20, 28, 32)

N_LAYERS = 2
SKEW_S = 1
SKEW_O = 6
SKEW_F = 5
EDGE = 4

VA_HEADS = 11
P1_CFG = (420, 2.5, 16, 140, 2, 560)
VO_HEADS = 18
P3_CFG = (460, 2.6, 24, 150, 1, 800)
XLU_AHEAD = 2
WD_COPY = False
WD_P2 = True
WD_STEP = 128
P2_CFG = (100, 0.4, 16, 150, 4, 200)
CK_UNROLL = 4
GU_UNROLL = 3
WD_ROWS = 432
F32_P1 = True
F32_P3 = True
F32_P4 = True
LINK_P1 = False
LINK_P3 = False
LINK_P4 = False
VF_TILES = 5
VF_GROUP = 2
VD_TILES = 2
XLU_EARLY = 10
P4_CFG = (290, 2.2, 24, 150, 1, 460)


SCOPES = False


class _ScopedWait:
    def __init__(self, c, name):
        self.c, self.name = c, name

    def wait(self):
        with jax.named_scope(self.name):
            self.c.wait()


def _always():
    return True


def _cosched(ms, vs, cfg):
    vstart, rate, lag_v, lag_m, nlink, lstart = cfg
    mres, vres = [], []
    j, tv = 0, vstart

    def latest(res, t):
        for tt, val in reversed(res):
            if tt <= t:
                return val
        return None

    def emit_v(dep):
        nonlocal j, tv
        val = vs[j](dep)
        tv += getattr(vs[j], "valu", 0) / rate
        vres.append((tv, val))
        j += 1

    for i, m in enumerate(ms):
        t = 8 * i
        while not getattr(m, "ready", _always)():
            emit_v(None)
        dep = None
        if i % nlink == 0 and j < len(vs) and t >= lstart:
            dep = latest(vres, t - lag_v)
        mres.append((t, m(dep)))
        while j < len(vs) and tv <= t + 8 and getattr(vs[j], "ready", _always)():
            emit_v(latest(mres, tv - lag_m) if j % 2 == 0 else None)
    while j < len(vs):
        emit_v(None)


def _valu(n):
    def deco(f):
        f.valu = n
        return f
    return deco


def _skewed(n, skew, produce, consume):
    out = []
    for step in range(n + skew):
        if step < n:
            out += produce(step)
        if step >= skew:
            out += consume(step - skew)
    return out


def _by_column(items, op, ncol):
    return [op(it, c) for c in range(ncol) for it in items]


def _by_item(items, op, ncol):
    return [op(it, c) for it in items for c in range(ncol)]


def _run(ops):
    for f in ops:
        f(None)


def _dot(a, b):
    return jnp.dot(a, b, preferred_element_type=F32)


def _bf(words):
    return pltpu.bitcast(words, BF16)


def _lo(w):
    return pltpu.bitcast(w << 16, F32)


def _hi(w):
    return pltpu.bitcast(w & jnp.uint32(0xFFFF0000), F32)


def _sublane_sum(t):
    t = t + pltpu.roll(t, 4, 0)
    t = t + pltpu.roll(t, 2, 0)
    return t + pltpu.roll(t, 1, 0)


def _col_bcast(row):
    return pltpu.bitcast(jnp.broadcast_to(row, (L, L)).T, U32)


def _round_bf16(x):
    return x.astype(BF16).astype(F32)


def _stats(xt):
    c = jnp.mean(xt[0], axis=-1, keepdims=True)
    s1 = s2 = None
    for x in xt:
        d = x - c
        s1 = d if s1 is None else s1 + d
        s2 = d * d if s2 is None else s2 + d * d
    m1 = jnp.sum(s1, axis=-1, keepdims=True) * (1.0 / M)
    m2 = jnp.sum(s2, axis=-1, keepdims=True) * (1.0 / M)
    var = jnp.maximum(m2 - m1 * m1, 0.0)
    return c + m1, jax.lax.rsqrt(var + EPS)


def _lhs16(xt):
    return [jnp.concatenate([x, jnp.ones_like(x)], axis=0).astype(BF16) for x in xt]


def _acc(d, k, v):
    d[k] = v if d.get(k) is None else d[k] + v
    return d[k]


def _kernel(x_hbm, wr_hbm, wq_hbm, wuk_hbm, ckv_hbm, wuv_hbm, wg_hbm, wu_hbm,
            wo_hbm, wd_hbm,
            o_ref,
            x_v, wr_v, wq_l, wuk_l, ckv_l, wuv_l, wg_l, wu_l, wo_l, wd_l,
            WQ32, WUKT32, CKV32, CKT32, WUV32, WG32, WU32, WO32, WD32,
            WUKF, WOF, WGF, WUF, CSG, CSU, XE, XO, sems):
    sem_ids = iter(range(64))

    def copy(src, dst, sem=None):
        sem = next(sem_ids) if sem is None else sem
        c = pltpu.make_async_copy(src, dst, sems.at[sem])
        c.start()
        if SCOPES:
            return _ScopedWait(c, "wait%02d" % sem)
        return c

    c_wq = copy(wq_hbm, wq_l)
    s_small = next(sem_ids)
    c_small = [copy(x_hbm, x_v, s_small), copy(wr_hbm, wr_v, s_small)]
    c_wuk = copy(wuk_hbm, wuk_l)
    c_ckv = copy(ckv_hbm, ckv_l)
    c_wuv = copy(wuv_hbm, wuv_l)
    c_wg = copy(wg_hbm, wg_l)
    c_wu = copy(wu_hbm, wu_l)
    wo_chunks = list(zip(WO_SPLIT[:-1], WO_SPLIT[1:]))
    c_wo = [copy(wo_hbm.at[pl.ds(h0 * D, (h1 - h0) * D)],
                 wo_l.at[pl.ds(h0 * D, (h1 - h0) * D)]) for h0, h1 in wo_chunks]
    c_wd = [copy(wd_hbm.at[:, pl.ds(nt * L, L)], wd_l.at[nt]) for nt in range(MT)]

    def swap_heads(src, dst32, rows):
        ch = 64

        def body(i, carry):
            w = src[pl.ds(pl.multiple_of(i * ch, ch), ch)]
            dst32[:, pl.ds(pl.multiple_of(i * (ch // 2), ch // 2), ch // 2), :] = (
                pltpu.bitcast(jnp.swapaxes(w, 0, 1), U32))
            return carry
        jax.lax.fori_loop(0, rows // ch, body, 0)

    def make_wukt():
        def body(i, carry):
            w = wuk_l[pl.ds(pl.multiple_of(i * L, L), L)]
            w = jnp.swapaxes(jnp.swapaxes(w, 0, 1), 1, 2)
            WUKT32[:, pl.ds(pl.multiple_of(i * W2, W2), W2), :] = pltpu.bitcast(w, U32)
            return carry
        jax.lax.fori_loop(0, CT, body, 0)

    def make_ck():
        def body(i, carry):
            for u in range(CK_UNROLL):
                kt = i * CK_UNROLL + u
                w = ckv_l[pl.ds(pl.multiple_of(kt * L, L), L), :]
                CKT32[kt] = pltpu.bitcast(w.T, U32)
                for ct in range(CT):
                    CKV32[ct, pl.ds(pl.multiple_of(kt * W2, W2), W2), :] = pltpu.bitcast(
                        w[:, ct * L:(ct + 1) * L], U32)
            return carry
        jax.lax.fori_loop(0, KT // CK_UNROLL, body, 0)

    def make_wgu(src, dst32):
        def body(i, carry):
            for u in range(GU_UNROLL):
                ft = i * GU_UNROLL + u
                w = src[pl.ds(pl.multiple_of(ft * L, L), L), :]
                dst32[ft] = pltpu.bitcast(w.T, U32)
            return carry
        n = (FT - 1) // GU_UNROLL
        jax.lax.fori_loop(0, n, body, 0)
        for ft in range(n * GU_UNROLL, FT - 1):
            dst32[ft] = pltpu.bitcast(src[ft * L:(ft + 1) * L, :].T, U32)

    def make_gu_tail():
        w = jnp.concatenate([wg_l[(FT - 1) * L:FF, :], wu_l[(FT - 1) * L:FF, :]], axis=0)
        WG32[FT - 1] = pltpu.bitcast(w.T, U32)

    def widen(src32, dst, n):
        def body(i, carry):
            w = src32[i]
            dst[i, 0] = _lo(w)
            dst[i, 1] = _hi(w)
            return carry
        if n:
            jax.lax.fori_loop(0, n, body, 0)

    def make_wd(nt):
        def body(i, carry):
            r0 = pl.multiple_of(i * WD_ROWS, 16)
            WD32[nt, pl.ds(pl.multiple_of(i * (WD_ROWS // 2), 8), WD_ROWS // 2), :] = (
                pltpu.bitcast(wd_l[nt, pl.ds(r0, WD_ROWS), :], U32))
            return carry
        jax.lax.fori_loop(0, FF // WD_ROWS, body, 0)

    def make_wo(h0, h1, widen):
        def body(h, carry):
            rows = wo_l[pl.ds(pl.multiple_of(h * L, L), L), :]
            for nt in range(MT):
                w = pltpu.bitcast(rows[:, nt * L:(nt + 1) * L], U32)
                WO32[nt, pl.ds(pl.multiple_of(h * W2, W2), W2), :] = w
                if widen:
                    WOF[h, 0, nt] = _lo(w)
                    WOF[h, 1, nt] = _hi(w)
            return carry
        if h1 > h0:
            jax.lax.fori_loop(h0, h1, body, 0)

    sub = jax.lax.broadcasted_iota(jnp.int32, (R, L), 0)
    zero_v, zero_s = [], []

    def link(a, dep):
        if dep is None:
            return a
        z = pltpu.bitcast(dep, U32) & zero_v[0]
        a32 = pltpu.bitcast(a, U32)
        n = a32.shape[0]
        if n > R:
            a32 = jnp.concatenate([a32[:R] | z, a32[R:]], axis=0)
        else:
            a32 = a32 | z[:n]
        return pltpu.bitcast(a32, a.dtype)

    def make_xb(xt):
        for t in range(MT):
            w = _col_bcast(xt[t].astype(BF16)[0:1])
            XE[t * W2:(t + 1) * W2, :] = _lo(w)
            XO[t * W2:(t + 1) * W2, :] = _hi(w)

    def tile(ref32, lead, t):
        return _bf(ref32[lead, t * W2:(t + 1) * W2, :])

    def vpu_matvec_step(accs, ref_keys, s, dep):
        xe = link(XE[s * R:(s + 1) * R, :], dep)
        xo = XO[s * R:(s + 1) * R, :]
        for ref32, reff, lead in ref_keys:
            if reff is not None:
                we = reff[lead, 0, s * R:(s + 1) * R, :]
                wo_ = reff[lead, 1, s * R:(s + 1) * R, :]
            else:
                w = ref32[lead, s * R:(s + 1) * R, :]
                we, wo_ = _lo(w), _hi(w)
            _acc(accs, (id(ref32), lead), we * xe + wo_ * xo)

    def q_partial(oq, x_tile, t):
        lhs = _lhs16([x_tile])[0]

        def op(h):
            def f(dep):
                p = _dot(link(lhs, dep), tile(WQ32, h, t))
                _acc(oq, h, p)
                return p[:R]
            return f
        return [op(h) for h in range(H)]

    def attention(xt, first, oq):
        mu, rstd = _stats(xt)
        qscale = rstd * (D ** -0.5)
        nva = 0 if first else VA_HEADS
        nvo = 0 if first else VO_HEADS
        if first:
            c_wq.wait()
            swap_heads(wq_l, WQ32, M)
            for t in range(MT - 1):
                _run(q_partial(oq, xt[t], t))
            c_wuk.wait()
            make_wukt()
            if F32_P1:
                widen(WUKT32, WUKF, VA_HEADS)

        qh, qa = {}, {}

        def q_last(h, op):
            def f(dep):
                r = op(dep)
                o = oq[h]
                qh[h] = ((o[:R] - mu * o[R:]) * qscale).astype(BF16)
                return r
            return f

        def put_qa(h, ct, t):
            g, i = divmod(h, R)
            qa[g, ct] = t if (g, ct) not in qa else jnp.where(sub == i, t, qa[g, ct])

        def qabs_op(h, ct):
            def f(dep):
                t = _dot(link(qh[h], dep if LINK_P1 else None), tile(WUKT32, h, ct))
                put_qa(h, ct, t)
                return t
            return f

        ms = [q_last(h, op) for h, op in enumerate(q_partial(oq, xt[MT - 1], MT - 1))]
        ms += _by_item(range(nva, H - EDGE), qabs_op, CT)
        ms += _by_column(range(H - EDGE, H), qabs_op, CT)
        qw, aacc = {}, {}

        def qxlu_op(h):
            def f(dep):
                qw[h] = _col_bcast(qh[h][0:1])
                return pltpu.bitcast(qw[h][:R], F32)
            f.ready = lambda: h in qh
            return f

        def qa_vstep(h, k):
            def f(dep):
                w = qw[h][k * R:(k + 1) * R]
                ce, co = link(_lo(w), dep), _hi(w)
                for ct in range(CT):
                    r0 = ct * W2 + k * R
                    if F32_P1:
                        we, wo_ = WUKF[h, 0, r0:r0 + R, :], WUKF[h, 1, r0:r0 + R, :]
                    else:
                        w = WUKT32[h, r0:r0 + R, :]
                        we, wo_ = _lo(w), _hi(w)
                    _acc(aacc, (h, ct), we * ce + wo_ * co)
                if k == L // 16 - 1:
                    for ct in range(CT):
                        put_qa(h, ct, _sublane_sum(aacc[h, ct]))
                return aacc[h, 0]
            return _valu((4 if F32_P1 else 6) * CT + 2)(f)

        vs = [qxlu_op(h) for h in range(min(XLU_AHEAD, nva))]
        for h in range(nva):
            if h + XLU_AHEAD < nva:
                vs.append(qxlu_op(h + XLU_AHEAD))
            vs += [qa_vstep(h, k) for k in range(L // 16)]
        _cosched(ms, vs, P1_CFG)
        qabs = [jnp.concatenate([qa[g, ct] for g in range(H // R)], axis=0).astype(BF16)
                for ct in range(CT)]

        if first:
            c_ckv.wait()
            make_ck()
        nch = KT // KCHUNK
        sc, ps, lats = {}, {}, {}
        mxs, lss = [None] * nch, [None] * nch

        def score_op(kt, ct):
            def f(dep):
                p = _dot(link(qabs[ct], dep), tile(CKT32, kt, ct))
                _acc(sc, kt, p)
                j = kt // KCHUNK
                if ct == CT - 1 and kt == (j + 1) * KCHUNK - 1:
                    kts = range(j * KCHUNK, (j + 1) * KCHUNK)
                    mx = sc[kts[0]]
                    for k in kts[1:]:
                        mx = jnp.maximum(mx, sc[k])
                    mx = jnp.max(mx, axis=-1, keepdims=True)
                    lsum = None
                    for k in kts:
                        e = jnp.exp(sc[k] - mx)
                        lsum = e if lsum is None else lsum + e
                        ps[k] = e.astype(BF16)
                    mxs[j], lss[j] = mx, lsum
                return p[:R]
            return f

        def lat_op(kt, ct):
            def f(dep):
                p = _dot(link(ps[kt], dep), tile(CKV32, ct, kt))
                _acc(lats, (kt // KCHUNK, ct), p)
                return p[:R]
            return f

        def s_produce(j):
            kts = list(range(j * KCHUNK, (j + 1) * KCHUNK))
            if j == 0:
                return (_by_column(kts[:EDGE], score_op, CT)
                        + _by_item(kts[EDGE:], score_op, CT))
            return _by_item(kts, score_op, CT)

        def s_consume(j):
            return _by_column(range(j * KCHUNK, (j + 1) * KCHUNK), lat_op, CT)

        def wd_copy_op(nt, r0, rows):
            def f(dep):
                w = pltpu.bitcast(wd_l[nt, r0:r0 + rows, :], U32)
                w = link(w, dep)
                d0 = jnp.clip(zero_s[0] + r0 // 2, 0, (FF - rows) // 2)
                WD32[nt, pl.ds(pl.multiple_of(d0, R), rows // 2), :] = w
                return pltpu.bitcast(w[:R], F32)
            return _valu(rows // 16)(f)

        cs = []
        if not first and WD_P2:
            cs = [wd_copy_op(nt, r0, min(WD_STEP, FF - r0))
                  for nt in range(MT) for r0 in range(0, FF, WD_STEP)]
        _cosched(_skewed(nch, SKEW_S, s_produce, s_consume), cs, P2_CFG)
        m = mxs[0]
        for t in mxs[1:]:
            m = jnp.maximum(m, t)
        alpha = [jnp.exp(t - m) for t in mxs]
        lsum = alpha[0] * lss[0]
        for a, t in zip(alpha[1:], lss[1:]):
            lsum = lsum + a * t
        inv = 1.0 / jnp.sum(lsum, axis=-1, keepdims=True)
        alpha = [a * inv for a in alpha]
        latg = {}
        for ct in range(CT):
            t = alpha[0] * lats[0, ct]
            for j in range(1, nch):
                t = t + alpha[j] * lats[j, ct]
            for g in range(H // R):
                latg[g, ct] = t[g * R:(g + 1) * R].astype(BF16)

        if first:
            c_wuv.wait()
            swap_heads(wuv_l, WUV32, DC)
        cacc, cbs, o = {}, {}, {}

        def ctx_op(h, ct):
            def f(dep):
                g, i = divmod(h, R)
                p = _dot(link(latg[g, ct], dep), tile(WUV32, h, ct))
                c = _acc(cacc, h, p)
                if ct == CT - 1:
                    cbs[h] = jnp.broadcast_to(c[i:i + 1], (R, D)).astype(BF16)
                return p
            return f

        def out_op(h, nt):
            def f(dep):
                t = _dot(link(cbs[h], dep if LINK_P3 else None), tile(WO32, nt, h))
                _acc(o, nt, t)
                return t
            return f

        if first:
            _run(_by_item(range(H), ctx_op, CT))
            c_wg.wait()
            make_wgu(wg_l, WG32)
            c_wu.wait()
            make_wgu(wu_l, WU32)
            make_gu_tail()
            if F32_P4:
                widen(WG32, WGF, VF_TILES)
                widen(WU32, WUF, VF_TILES)
            for c, (h0, h1) in enumerate(wo_chunks):
                c_wo[c].wait()
                hm = min(max(VO_HEADS if F32_P3 else 0, h0), h1)
                make_wo(h0, hm, True)
                make_wo(hm, h1, False)
                if c == len(wo_chunks) - 1:
                    _run(_by_column(range(h0, h1), out_op, MT))
                else:
                    _run(_by_item(range(h0, h1), out_op, MT))
            return [_round_bf16(xt[nt] + o[nt]) for nt in range(MT)]

        ms = _by_column(range(EDGE), ctx_op, CT) + _by_item(range(EDGE, nvo), ctx_op, CT)
        h0 = max(nvo, EDGE)

        def o_produce(i):
            return _by_item([h0 + i], ctx_op, CT)

        def o_consume(h):
            if h >= H - EDGE:
                return _by_column(range(H - EDGE, H), out_op, MT) if h == H - 1 else []
            return _by_item([h], out_op, MT)

        for step in range(H - h0 + SKEW_O):
            if step < H - h0:
                ms += o_produce(step)
            if step >= SKEW_O:
                ms += o_consume(h0 + step - SKEW_O)
        for h in range(nvo, h0):
            ms += o_consume(h)
        cw, ov = {}, {}

        def xlu_op(h):
            def f(dep):
                cw[h] = _col_bcast(cbs[h][0:1])
                return pltpu.bitcast(cw[h][:R], F32)
            f.ready = lambda: h in cbs
            return f

        def o_vstep(h, k):
            def f(dep):
                w = cw[h][k * R:(k + 1) * R]
                ce, co = link(_lo(w), dep), _hi(w)
                r0 = h * W2 + k * R
                for nt in range(MT):
                    if F32_P3:
                        we = WOF[h, 0, nt, k * R:(k + 1) * R, :]
                        wo_ = WOF[h, 1, nt, k * R:(k + 1) * R, :]
                    else:
                        w = WO32[nt, r0:r0 + R, :]
                        we, wo_ = _lo(w), _hi(w)
                    _acc(ov, nt, we * ce + wo_ * co)
                return ov[0]
            return _valu((4 if F32_P3 else 6) * MT + 2)(f)

        vs = [xlu_op(h) for h in range(min(XLU_AHEAD, nvo))]
        for h in range(nvo):
            if h + XLU_AHEAD < nvo:
                vs.append(xlu_op(h + XLU_AHEAD))
            vs += [o_vstep(h, k) for k in range(L // 16)]
        _cosched(ms, vs, P3_CFG)
        if nvo:
            o = {nt: o[nt] + _sublane_sum(ov[nt]) for nt in range(MT)}
        return [_round_bf16(xt[nt] + o[nt]) for nt in range(MT)]

    def ffn(xt, first, oq_next=None):
        mu, rstd = _stats(xt)
        lhs = _lhs16(xt)
        xn = [(x - mu) * rstd for x in xt]
        wr = wr_v[...].reshape(1, M).astype(F32)
        r = jnp.sum(jnp.concatenate(xn, axis=1) * wr, axis=-1, keepdims=True)
        gate = jax.nn.sigmoid(r)
        nvf = 0 if first else VF_TILES
        pre, acts, y = {}, {}, {}

        def finish(ft):
            g, u = pre[ft, 0] * rstd, pre[ft, 1] * rstd
            acts[ft] = (g * jax.nn.sigmoid(g) * u).astype(BF16)

        def gu_op(key, t):
            ft, which = key

            def f(dep):
                p = _dot(link(lhs[t], dep), tile((WG32, WU32)[which], ft, t))
                o = _acc(pre, key, p)
                if t == MT - 1:
                    if first and ft < VF_TILES:
                        (CSG, CSU)[which][ft] = o[R:]
                    pre[key] = o[:R] - mu * o[R:]
                    if ft == FT - 1:
                        pre[ft, 1] = pltpu.roll(pre[key], L - F_TAIL, 1)
                    if which == 1 or ft == FT - 1:
                        finish(ft)
                return p[:R]
            return f

        def dn_op(ft, nt):
            def f(dep):
                rows = L if ft < FT - 1 else F_TAIL
                a = acts[ft] if rows == L else acts[ft][:, :rows]
                if first:
                    w = wd_l[nt, ft * L:ft * L + rows, :]
                else:
                    w = _bf(WD32[nt, ft * W2:ft * W2 + rows // 2, :])
                t = _dot(link(a, dep if LINK_P4 else None), w)
                _acc(y, nt, t)
                return t
            f.ready = lambda: ft in acts
            return f

        def gu_keys(fts):
            return [(ft, which) for ft in fts
                    for which in range(1 if ft == FT - 1 else 2)]

        if first:
            _run(_by_column(gu_keys(range(2)), gu_op, MT))
            _run(_by_item(gu_keys(range(2, FT)), gu_op, MT))
            out = []
            for nt in range(MT):
                c_wd[nt].wait()
                _run([dn_op(ft, nt) for ft in range(FT)])
                out.append(_round_bf16(xt[nt] + xn[nt] + y[nt] * gate))
                if oq_next is not None:
                    if 0 < nt < MT - 1:
                        _run(q_partial(oq_next, out[nt - 1], nt - 1))
                    if nt == MT - 2:
                        _run(q_partial(oq_next, out[nt], nt))
                    if WD_COPY and nt < MT - 1:
                        make_wd(nt)
            return out
        else:
            mt = list(range(nvf, FT))
            vd = mt[:VD_TILES]
            md = [ft for ft in mt if ft not in vd] + list(range(nvf))
            last = md[-2:]

            def g_produce(i):
                if i == 0:
                    return _by_column(gu_keys(mt[:2]), gu_op, MT)
                return [] if i == 1 else _by_item(gu_keys([mt[i]]), gu_op, MT)

            def g_consume(ft):
                if ft in vd:
                    return []
                if ft in last:
                    return _by_column(last, dn_op, MT) if ft == last[-1] else []
                return _by_item([ft], dn_op, MT)

            ms = _skewed(len(mt), SKEW_F, g_produce, lambda i: g_consume(mt[i]))
            for ft in range(nvf):
                ms += g_consume(ft)
            facc, aw, yv = {}, {}, {}

            def f_vstep(fts, s):
                def f(dep):
                    keys = [(w, wf if F32_P4 else None, ft) for ft in fts
                            for w, wf in ((WG32, WGF), (WU32, WUF))]
                    vpu_matvec_step(facc, keys, s, dep)
                    if s == M // 16 - 1:
                        for ft in fts:
                            for wh, (w, cs) in enumerate(((WG32, CSG), (WU32, CSU))):
                                pre[ft, wh] = _sublane_sum(facc[id(w), ft]) - mu * cs[ft]
                            finish(ft)
                    return facc[id(WG32), fts[0]]
                return _valu((8 if F32_P4 else 12) * len(fts))(f)

            def dxlu_op(ft):
                def f(dep):
                    aw[ft] = _col_bcast(acts[ft][0:1])
                    return pltpu.bitcast(aw[ft][:R], F32)
                f.ready = lambda: ft in acts
                return f

            def d_vstep(ft, k):
                def f(dep):
                    w = aw[ft][k * R:(k + 1) * R]
                    ce, co = link(_lo(w), dep), _hi(w)
                    r0 = ft * W2 + k * R
                    for nt in range(MT):
                        w = WD32[nt, r0:r0 + R, :]
                        _acc(yv, nt, _lo(w) * ce + _hi(w) * co)
                    return yv[0]
                return _valu(6 * MT + 2)(f)

            if nvf:
                make_xb(xt)
            vs = [f_vstep(list(range(f0, min(nvf, f0 + VF_GROUP))), s)
                  for f0 in range(0, nvf, VF_GROUP) for s in range(M // 16)]
            pos = max(0, len(vs) - XLU_EARLY)
            for i, ft in enumerate(vd[:XLU_AHEAD]):
                vs.insert(pos + i, dxlu_op(ft))
            for i, ft in enumerate(vd):
                if i + XLU_AHEAD < len(vd):
                    vs.append(dxlu_op(vd[i + XLU_AHEAD]))
                vs += [d_vstep(ft, k) for k in range(L // 16)]
            _cosched(ms, vs, P4_CFG)
            if vd:
                y = {nt: y[nt] + _sublane_sum(yv[nt]) for nt in range(MT)}
        return [_round_bf16(xt[nt] + xn[nt] + y[nt] * gate) for nt in range(MT)]

    for c in c_small:
        c.wait()
    x = jnp.broadcast_to(x_v[...].astype(F32), (R, M))
    zero_v.append(pltpu.bitcast(x[:, :L], U32) & jnp.uint32(0xFFFF))
    zero_s.append(jnp.max(zero_v[0].astype(jnp.int32)))
    xt = [x[:, t * L:(t + 1) * L] for t in range(MT)]
    xt = attention(xt, True, {})
    oq2 = {}
    xt = ffn(xt, True, oq2 if N_LAYERS > 1 else None)
    if N_LAYERS > 1:
        if not WD_P2:
            for nt in range(MT - 1 if WD_COPY else 0, MT):
                WD32[nt] = pltpu.bitcast(wd_l[nt], U32)
        xt = attention(xt, False, oq2)
        xt = ffn(xt, False)
    o_ref[...] = jnp.concatenate(xt, axis=1)[0:1].astype(o_ref.dtype)


@jax.jit
def pallas_interleave_layers__compressed_kv_cla__moe_arch_mod__decode_kernel(
    A_x: jax.Array,
    A_c_kv: jax.Array,
    A_w_q: jax.Array,
    A_w_uk: jax.Array,
    A_w_uv: jax.Array,
    A_w_o: jax.Array,
    B_x: jax.Array,
    B_w_r: jax.Array,
    B_w_gate: jax.Array,
    B_w_up: jax.Array,
    B_w_down: jax.Array,
):
    del B_x
    args = (
        A_x.reshape(1, M),
        B_w_r,
        A_w_q,
        A_w_uk,
        A_c_kv.reshape(SK, DC),
        A_w_uv,
        B_w_gate.T,
        B_w_up.T,
        A_w_o.reshape(H * D, M),
        B_w_down,
    )
    n_sems = 6 + len(WO_SPLIT) + MT
    scratch = [
        pltpu.VMEM((1, M), BF16),
        pltpu.VMEM((M,), BF16),
        pltpu.VMEM((M, H, D), BF16),
        pltpu.VMEM((DC, H, D), BF16),
        pltpu.VMEM((SK, DC), BF16),
        pltpu.VMEM((DC, H, D), BF16),
        pltpu.VMEM((FF, M), BF16),
        pltpu.VMEM((FF, M), BF16),
        pltpu.VMEM((H * D, M), BF16),
        pltpu.VMEM((MT, FF, L), BF16),
        pltpu.VMEM((H, M // 2, D), U32),
        pltpu.VMEM((H, DC // 2, L), U32),
        pltpu.VMEM((CT, SK // 2, L), U32),
        pltpu.VMEM((KT, DC // 2, L), U32),
        pltpu.VMEM((H, DC // 2, D), U32),
        pltpu.VMEM((FT, M // 2, L), U32),
        pltpu.VMEM((FT - 1, M // 2, L), U32),
        pltpu.VMEM((MT, H * D // 2, L), U32),
        pltpu.VMEM((MT, FF // 2, L), U32),
        pltpu.VMEM((max(VA_HEADS, 1), 2, DC // 2, L), F32),
        pltpu.VMEM((max(VO_HEADS, 1), 2, MT, W2, L), F32),
        pltpu.VMEM((max(VF_TILES, 1), 2, M // 2, L), F32),
        pltpu.VMEM((max(VF_TILES, 1), 2, M // 2, L), F32),
        pltpu.VMEM((FT, R, L), F32),
        pltpu.VMEM((FT, R, L), F32),
        pltpu.VMEM((M // 2, L), F32),
        pltpu.VMEM((M // 2, L), F32),
        pltpu.SemaphoreType.DMA((n_sems,)),
    ]
    out = pl.pallas_call(
        _kernel,
        out_shape=jax.ShapeDtypeStruct((1, M), A_x.dtype),
        in_specs=[pl.BlockSpec(memory_space=pl.ANY)] * len(args),
        out_specs=pl.BlockSpec(memory_space=pltpu.VMEM),
        scratch_shapes=scratch,
        compiler_params=pltpu.CompilerParams(
            vmem_limit_bytes=100 * 1024 * 1024,
            disable_semaphore_checks=True),
        name="mla_moe_decode",
    )(*args)
    return out.reshape(1, 1, M)
```

```python
import jax
import jax.numpy as jnp
import jax.experimental.pallas as pl
import jax.experimental.pallas.tpu as pltpu

F32 = jnp.float32
BF16 = jnp.bfloat16
U32 = jnp.uint32

H = 32
D = 128
M = 640
DC = 512
SK = 4096
FF = 1728
EPS = 1e-5
R = 8
L = 128
W2 = L // 2

MT = M // L
CT = DC // L
KT = SK // L
FT = -(-FF // L)
F_TAIL = FF - (FT - 1) * L
KCHUNK = 8
WO_SPLIT = (0, 10, 20, 28, 32)

N_LAYERS = 2
SKEW_S = 1
SKEW_O = 6
SKEW_F = 5
EDGE = 4

VA_HEADS = 11
P1_CFG = (420, 2.5, 16, 140, 2, 560)
VO_HEADS = 18
P3_CFG = (460, 2.6, 24, 150, 1, 800)
XLU_AHEAD = 2
WD_STEP = 128
P2_CFG = (100, 0.4, 16, 150, 4, 200)
CK_UNROLL = 4
GU_UNROLL = 3
F32_P1 = True
F32_P3 = True
F32_P4 = True
VF_TILES = 5
VF_GROUP = 2
VD_TILES = 2
XLU_EARLY = 10
P4_CFG = (290, 2.2, 24, 150, 1, 460)


def _always():
    return True


def _cosched(ms, vs, cfg):
    vstart, rate, lag_v, lag_m, nlink, lstart = cfg
    mres, vres = [], []
    j, tv = 0, vstart

    def latest(res, t):
        for tt, val in reversed(res):
            if tt <= t:
                return val
        return None

    def emit_v(dep):
        nonlocal j, tv
        val = vs[j](dep)
        tv += getattr(vs[j], "valu", 0) / rate
        vres.append((tv, val))
        j += 1

    for i, m in enumerate(ms):
        t = 8 * i
        while not getattr(m, "ready", _always)():
            emit_v(None)
        dep = None
        if i % nlink == 0 and j < len(vs) and t >= lstart:
            dep = latest(vres, t - lag_v)
        mres.append((t, m(dep)))
        while j < len(vs) and tv <= t + 8 and getattr(vs[j], "ready", _always)():
            emit_v(latest(mres, tv - lag_m) if j % 2 == 0 else None)
    while j < len(vs):
        emit_v(None)


def _valu(n):
    def deco(f):
        f.valu = n
        return f
    return deco


def _skewed(n, skew, produce, consume):
    out = []
    for step in range(n + skew):
        if step < n:
            out += produce(step)
        if step >= skew:
            out += consume(step - skew)
    return out


def _by_column(items, op, ncol):
    return [op(it, c) for c in range(ncol) for it in items]


def _by_item(items, op, ncol):
    return [op(it, c) for it in items for c in range(ncol)]


def _run(ops):
    for f in ops:
        f(None)


def _dot(a, b):
    return jnp.dot(a, b, preferred_element_type=F32)


def _bf(words):
    return pltpu.bitcast(words, BF16)


def _lo(w):
    return pltpu.bitcast(w << 16, F32)


def _hi(w):
    return pltpu.bitcast(w & jnp.uint32(0xFFFF0000), F32)


def _sublane_sum(t):
    t = t + pltpu.roll(t, 4, 0)
    t = t + pltpu.roll(t, 2, 0)
    return t + pltpu.roll(t, 1, 0)


def _col_bcast(row):
    return pltpu.bitcast(jnp.broadcast_to(row, (L, L)).T, U32)


def _round_bf16(x):
    return x.astype(BF16).astype(F32)


def _stats(xt):
    c = jnp.mean(xt[0], axis=-1, keepdims=True)
    s1 = s2 = None
    for x in xt:
        d = x - c
        s1 = d if s1 is None else s1 + d
        s2 = d * d if s2 is None else s2 + d * d
    m1 = jnp.sum(s1, axis=-1, keepdims=True) * (1.0 / M)
    m2 = jnp.sum(s2, axis=-1, keepdims=True) * (1.0 / M)
    var = jnp.maximum(m2 - m1 * m1, 0.0)
    return c + m1, jax.lax.rsqrt(var + EPS)


def _lhs16(xt):
    return [jnp.concatenate([x, jnp.ones_like(x)], axis=0).astype(BF16) for x in xt]


def _acc(d, k, v):
    d[k] = v if d.get(k) is None else d[k] + v
    return d[k]


def _kernel(x_hbm, wr_hbm, wq_hbm, wuk_hbm, ckv_hbm, wuv_hbm, wg_hbm, wu_hbm,
            wo_hbm, wd_hbm,
            o_ref,
            x_v, wr_v, wq_l, wuk_l, ckv_l, wuv_l, wg_l, wu_l, wo_l, wd_l,
            WQ32, WUKT32, CKV32, CKT32, WUV32, WG32, WU32, WO32, WD32,
            WUKF, WOF, WGF, WUF, CSG, CSU, XE, XO, sems):
    sem_ids = iter(range(64))

    def copy(src, dst, sem=None):
        sem = next(sem_ids) if sem is None else sem
        c = pltpu.make_async_copy(src, dst, sems.at[sem])
        c.start()
        return c

    c_wq = copy(wq_hbm, wq_l)
    s_small = next(sem_ids)
    c_small = [copy(x_hbm, x_v, s_small), copy(wr_hbm, wr_v, s_small)]
    c_wuk = copy(wuk_hbm, wuk_l)
    c_ckv = copy(ckv_hbm, ckv_l)
    c_wuv = copy(wuv_hbm, wuv_l)
    c_wg = copy(wg_hbm, wg_l)
    c_wu = copy(wu_hbm, wu_l)
    wo_chunks = list(zip(WO_SPLIT[:-1], WO_SPLIT[1:]))
    c_wo = [copy(wo_hbm.at[pl.ds(h0 * D, (h1 - h0) * D)],
                 wo_l.at[pl.ds(h0 * D, (h1 - h0) * D)]) for h0, h1 in wo_chunks]
    c_wd = [copy(wd_hbm.at[:, pl.ds(nt * L, L)], wd_l.at[nt]) for nt in range(MT)]

    def swap_heads(src, dst32, rows):
        ch = 64

        def body(i, carry):
            w = src[pl.ds(pl.multiple_of(i * ch, ch), ch)]
            dst32[:, pl.ds(pl.multiple_of(i * (ch // 2), ch // 2), ch // 2), :] = (
                pltpu.bitcast(jnp.swapaxes(w, 0, 1), U32))
            return carry
        jax.lax.fori_loop(0, rows // ch, body, 0)

    def make_wukt():
        def body(i, carry):
            w = wuk_l[pl.ds(pl.multiple_of(i * L, L), L)]
            w = jnp.swapaxes(jnp.swapaxes(w, 0, 1), 1, 2)
            WUKT32[:, pl.ds(pl.multiple_of(i * W2, W2), W2), :] = pltpu.bitcast(w, U32)
            return carry
        jax.lax.fori_loop(0, CT, body, 0)

    def make_ck():
        def body(i, carry):
            for u in range(CK_UNROLL):
                kt = i * CK_UNROLL + u
                w = ckv_l[pl.ds(pl.multiple_of(kt * L, L), L), :]
                CKT32[kt] = pltpu.bitcast(w.T, U32)
                for ct in range(CT):
                    CKV32[ct, pl.ds(pl.multiple_of(kt * W2, W2), W2), :] = pltpu.bitcast(
                        w[:, ct * L:(ct + 1) * L], U32)
            return carry
        jax.lax.fori_loop(0, KT // CK_UNROLL, body, 0)

    def make_wgu(src, dst32):
        def body(i, carry):
            for u in range(GU_UNROLL):
                ft = i * GU_UNROLL + u
                w = src[pl.ds(pl.multiple_of(ft * L, L), L), :]
                dst32[ft] = pltpu.bitcast(w.T, U32)
            return carry
        n = (FT - 1) // GU_UNROLL
        jax.lax.fori_loop(0, n, body, 0)
        for ft in range(n * GU_UNROLL, FT - 1):
            dst32[ft] = pltpu.bitcast(src[ft * L:(ft + 1) * L, :].T, U32)

    def make_gu_tail():
        w = jnp.concatenate([wg_l[(FT - 1) * L:FF, :], wu_l[(FT - 1) * L:FF, :]], axis=0)
        WG32[FT - 1] = pltpu.bitcast(w.T, U32)

    def widen(src32, dst, n):
        def body(i, carry):
            w = src32[i]
            dst[i, 0] = _lo(w)
            dst[i, 1] = _hi(w)
            return carry
        if n:
            jax.lax.fori_loop(0, n, body, 0)

    def make_wo(h0, h1, widen):
        def body(h, carry):
            rows = wo_l[pl.ds(pl.multiple_of(h * L, L), L), :]
            for nt in range(MT):
                w = pltpu.bitcast(rows[:, nt * L:(nt + 1) * L], U32)
                WO32[nt, pl.ds(pl.multiple_of(h * W2, W2), W2), :] = w
                if widen:
                    WOF[h, 0, nt] = _lo(w)
                    WOF[h, 1, nt] = _hi(w)
            return carry
        if h1 > h0:
            jax.lax.fori_loop(h0, h1, body, 0)

    sub = jax.lax.broadcasted_iota(jnp.int32, (R, L), 0)
    zero_v, zero_s = [], []

    def link(a, dep):
        if dep is None:
            return a
        z = pltpu.bitcast(dep, U32) & zero_v[0]
        a32 = pltpu.bitcast(a, U32)
        n = a32.shape[0]
        if n > R:
            a32 = jnp.concatenate([a32[:R] | z, a32[R:]], axis=0)
        else:
            a32 = a32 | z[:n]
        return pltpu.bitcast(a32, a.dtype)

    def make_xb(xt):
        for t in range(MT):
            w = _col_bcast(xt[t].astype(BF16)[0:1])
            XE[t * W2:(t + 1) * W2, :] = _lo(w)
            XO[t * W2:(t + 1) * W2, :] = _hi(w)

    def tile(ref32, lead, t):
        return _bf(ref32[lead, t * W2:(t + 1) * W2, :])

    def vpu_matvec_step(accs, ref_keys, s, dep):
        xe = link(XE[s * R:(s + 1) * R, :], dep)
        xo = XO[s * R:(s + 1) * R, :]
        for ref32, reff, lead in ref_keys:
            if reff is not None:
                we = reff[lead, 0, s * R:(s + 1) * R, :]
                wo_ = reff[lead, 1, s * R:(s + 1) * R, :]
            else:
                w = ref32[lead, s * R:(s + 1) * R, :]
                we, wo_ = _lo(w), _hi(w)
            _acc(accs, (id(ref32), lead), we * xe + wo_ * xo)

    def q_partial(oq, x_tile, t):
        lhs = _lhs16([x_tile])[0]

        def op(h):
            def f(dep):
                p = _dot(link(lhs, dep), tile(WQ32, h, t))
                _acc(oq, h, p)
                return p[:R]
            return f
        return [op(h) for h in range(H)]

    def attention(xt, first, oq):
        mu, rstd = _stats(xt)
        qscale = rstd * (D ** -0.5)
        nva = 0 if first else VA_HEADS
        nvo = 0 if first else VO_HEADS
        if first:
            c_wq.wait()
            swap_heads(wq_l, WQ32, M)
            for t in range(MT - 1):
                _run(q_partial(oq, xt[t], t))
            c_wuk.wait()
            make_wukt()
            if F32_P1:
                widen(WUKT32, WUKF, VA_HEADS)

        qh, qa = {}, {}

        def q_last(h, op):
            def f(dep):
                r = op(dep)
                o = oq[h]
                qh[h] = ((o[:R] - mu * o[R:]) * qscale).astype(BF16)
                return r
            return f

        def put_qa(h, ct, t):
            g, i = divmod(h, R)
            qa[g, ct] = t if (g, ct) not in qa else jnp.where(sub == i, t, qa[g, ct])

        def qabs_op(h, ct):
            def f(dep):
                t = _dot(qh[h], tile(WUKT32, h, ct))
                put_qa(h, ct, t)
                return t
            return f

        ms = [q_last(h, op) for h, op in enumerate(q_partial(oq, xt[MT - 1], MT - 1))]
        ms += _by_item(range(nva, H - EDGE), qabs_op, CT)
        ms += _by_column(range(H - EDGE, H), qabs_op, CT)
        qw, aacc = {}, {}

        def qxlu_op(h):
            def f(dep):
                qw[h] = _col_bcast(qh[h][0:1])
                return pltpu.bitcast(qw[h][:R], F32)
            f.ready = lambda: h in qh
            return f

        def qa_vstep(h, k):
            def f(dep):
                w = qw[h][k * R:(k + 1) * R]
                ce, co = link(_lo(w), dep), _hi(w)
                for ct in range(CT):
                    r0 = ct * W2 + k * R
                    if F32_P1:
                        we, wo_ = WUKF[h, 0, r0:r0 + R, :], WUKF[h, 1, r0:r0 + R, :]
                    else:
                        w = WUKT32[h, r0:r0 + R, :]
                        we, wo_ = _lo(w), _hi(w)
                    _acc(aacc, (h, ct), we * ce + wo_ * co)
                if k == L // 16 - 1:
                    for ct in range(CT):
                        put_qa(h, ct, _sublane_sum(aacc[h, ct]))
                return aacc[h, 0]
            return _valu((4 if F32_P1 else 6) * CT + 2)(f)

        vs = [qxlu_op(h) for h in range(min(XLU_AHEAD, nva))]
        for h in range(nva):
            if h + XLU_AHEAD < nva:
                vs.append(qxlu_op(h + XLU_AHEAD))
            vs += [qa_vstep(h, k) for k in range(L // 16)]
        _cosched(ms, vs, P1_CFG)
        qabs = [jnp.concatenate([qa[g, ct] for g in range(H // R)], axis=0).astype(BF16)
                for ct in range(CT)]

        if first:
            c_ckv.wait()
            make_ck()
        nch = KT // KCHUNK
        sc, ps, lats = {}, {}, {}
        mxs, lss = [None] * nch, [None] * nch

        def score_op(kt, ct):
            def f(dep):
                p = _dot(link(qabs[ct], dep), tile(CKT32, kt, ct))
                _acc(sc, kt, p)
                j = kt // KCHUNK
                if ct == CT - 1 and kt == (j + 1) * KCHUNK - 1:
                    kts = range(j * KCHUNK, (j + 1) * KCHUNK)
                    mx = sc[kts[0]]
                    for k in kts[1:]:
                        mx = jnp.maximum(mx, sc[k])
                    mx = jnp.max(mx, axis=-1, keepdims=True)
                    lsum = None
                    for k in kts:
                        e = jnp.exp(sc[k] - mx)
                        lsum = e if lsum is None else lsum + e
                        ps[k] = e.astype(BF16)
                    mxs[j], lss[j] = mx, lsum
                return p[:R]
            return f

        def lat_op(kt, ct):
            def f(dep):
                p = _dot(link(ps[kt], dep), tile(CKV32, ct, kt))
                _acc(lats, (kt // KCHUNK, ct), p)
                return p[:R]
            return f

        def s_produce(j):
            kts = list(range(j * KCHUNK, (j + 1) * KCHUNK))
            if j == 0:
                return (_by_column(kts[:EDGE], score_op, CT)
                        + _by_item(kts[EDGE:], score_op, CT))
            return _by_item(kts, score_op, CT)

        def s_consume(j):
            return _by_column(range(j * KCHUNK, (j + 1) * KCHUNK), lat_op, CT)

        def wd_copy_op(nt, r0, rows):
            def f(dep):
                w = pltpu.bitcast(wd_l[nt, r0:r0 + rows, :], U32)
                w = link(w, dep)
                d0 = jnp.clip(zero_s[0] + r0 // 2, 0, (FF - rows) // 2)
                WD32[nt, pl.ds(pl.multiple_of(d0, R), rows // 2), :] = w
                return pltpu.bitcast(w[:R], F32)
            return _valu(rows // 16)(f)

        cs = []
        if not first:
            cs = [wd_copy_op(nt, r0, min(WD_STEP, FF - r0))
                  for nt in range(MT) for r0 in range(0, FF, WD_STEP)]
        _cosched(_skewed(nch, SKEW_S, s_produce, s_consume), cs, P2_CFG)
        m = mxs[0]
        for t in mxs[1:]:
            m = jnp.maximum(m, t)
        alpha = [jnp.exp(t - m) for t in mxs]
        lsum = alpha[0] * lss[0]
        for a, t in zip(alpha[1:], lss[1:]):
            lsum = lsum + a * t
        inv = 1.0 / jnp.sum(lsum, axis=-1, keepdims=True)
        alpha = [a * inv for a in alpha]
        latg = {}
        for ct in range(CT):
            t = alpha[0] * lats[0, ct]
            for j in range(1, nch):
                t = t + alpha[j] * lats[j, ct]
            for g in range(H // R):
                latg[g, ct] = t[g * R:(g + 1) * R].astype(BF16)

        if first:
            c_wuv.wait()
            swap_heads(wuv_l, WUV32, DC)
        cacc, cbs, o = {}, {}, {}

        def ctx_op(h, ct):
            def f(dep):
                g, i = divmod(h, R)
                p = _dot(link(latg[g, ct], dep), tile(WUV32, h, ct))
                c = _acc(cacc, h, p)
                if ct == CT - 1:
                    cbs[h] = jnp.broadcast_to(c[i:i + 1], (R, D)).astype(BF16)
                return p
            return f

        def out_op(h, nt):
            def f(dep):
                t = _dot(cbs[h], tile(WO32, nt, h))
                _acc(o, nt, t)
                return t
            return f

        if first:
            _run(_by_item(range(H), ctx_op, CT))
            c_wg.wait()
            make_wgu(wg_l, WG32)
            c_wu.wait()
            make_wgu(wu_l, WU32)
            make_gu_tail()
            if F32_P4:
                widen(WG32, WGF, VF_TILES)
                widen(WU32, WUF, VF_TILES)
            for c, (h0, h1) in enumerate(wo_chunks):
                c_wo[c].wait()
                hm = min(max(VO_HEADS if F32_P3 else 0, h0), h1)
                make_wo(h0, hm, True)
                make_wo(hm, h1, False)
                if c == len(wo_chunks) - 1:
                    _run(_by_column(range(h0, h1), out_op, MT))
                else:
                    _run(_by_item(range(h0, h1), out_op, MT))
            return [_round_bf16(xt[nt] + o[nt]) for nt in range(MT)]

        ms = _by_column(range(EDGE), ctx_op, CT) + _by_item(range(EDGE, nvo), ctx_op, CT)
        h0 = max(nvo, EDGE)

        def o_produce(i):
            return _by_item([h0 + i], ctx_op, CT)

        def o_consume(h):
            if h >= H - EDGE:
                return _by_column(range(H - EDGE, H), out_op, MT) if h == H - 1 else []
            return _by_item([h], out_op, MT)

        for step in range(H - h0 + SKEW_O):
            if step < H - h0:
                ms += o_produce(step)
            if step >= SKEW_O:
                ms += o_consume(h0 + step - SKEW_O)
        for h in range(nvo, h0):
            ms += o_consume(h)
        cw, ov = {}, {}

        def xlu_op(h):
            def f(dep):
                cw[h] = _col_bcast(cbs[h][0:1])
                return pltpu.bitcast(cw[h][:R], F32)
            f.ready = lambda: h in cbs
            return f

        def o_vstep(h, k):
            def f(dep):
                w = cw[h][k * R:(k + 1) * R]
                ce, co = link(_lo(w), dep), _hi(w)
                r0 = h * W2 + k * R
                for nt in range(MT):
                    if F32_P3:
                        we = WOF[h, 0, nt, k * R:(k + 1) * R, :]
                        wo_ = WOF[h, 1, nt, k * R:(k + 1) * R, :]
                    else:
                        w = WO32[nt, r0:r0 + R, :]
                        we, wo_ = _lo(w), _hi(w)
                    _acc(ov, nt, we * ce + wo_ * co)
                return ov[0]
            return _valu((4 if F32_P3 else 6) * MT + 2)(f)

        vs = [xlu_op(h) for h in range(min(XLU_AHEAD, nvo))]
        for h in range(nvo):
            if h + XLU_AHEAD < nvo:
                vs.append(xlu_op(h + XLU_AHEAD))
            vs += [o_vstep(h, k) for k in range(L // 16)]
        _cosched(ms, vs, P3_CFG)
        if nvo:
            o = {nt: o[nt] + _sublane_sum(ov[nt]) for nt in range(MT)}
        return [_round_bf16(xt[nt] + o[nt]) for nt in range(MT)]

    def ffn(xt, first, oq_next=None):
        mu, rstd = _stats(xt)
        lhs = _lhs16(xt)
        xn = [(x - mu) * rstd for x in xt]
        wr = wr_v[...].reshape(1, M).astype(F32)
        r = jnp.sum(jnp.concatenate(xn, axis=1) * wr, axis=-1, keepdims=True)
        gate = jax.nn.sigmoid(r)
        nvf = 0 if first else VF_TILES
        pre, acts, y = {}, {}, {}

        def finish(ft):
            g, u = pre[ft, 0] * rstd, pre[ft, 1] * rstd
            acts[ft] = (g * jax.nn.sigmoid(g) * u).astype(BF16)

        def gu_op(key, t):
            ft, which = key

            def f(dep):
                p = _dot(link(lhs[t], dep), tile((WG32, WU32)[which], ft, t))
                o = _acc(pre, key, p)
                if t == MT - 1:
                    if first and ft < VF_TILES:
                        (CSG, CSU)[which][ft] = o[R:]
                    pre[key] = o[:R] - mu * o[R:]
                    if ft == FT - 1:
                        pre[ft, 1] = pltpu.roll(pre[key], L - F_TAIL, 1)
                    if which == 1 or ft == FT - 1:
                        finish(ft)
                return p[:R]
            return f

        def dn_op(ft, nt):
            def f(dep):
                rows = L if ft < FT - 1 else F_TAIL
                a = acts[ft] if rows == L else acts[ft][:, :rows]
                if first:
                    w = wd_l[nt, ft * L:ft * L + rows, :]
                else:
                    w = _bf(WD32[nt, ft * W2:ft * W2 + rows // 2, :])
                t = _dot(a, w)
                _acc(y, nt, t)
                return t
            f.ready = lambda: ft in acts
            return f

        def gu_keys(fts):
            return [(ft, which) for ft in fts
                    for which in range(1 if ft == FT - 1 else 2)]

        if first:
            _run(_by_column(gu_keys(range(2)), gu_op, MT))
            _run(_by_item(gu_keys(range(2, FT)), gu_op, MT))
            out = []
            for nt in range(MT):
                c_wd[nt].wait()
                _run([dn_op(ft, nt) for ft in range(FT)])
                out.append(_round_bf16(xt[nt] + xn[nt] + y[nt] * gate))
                if oq_next is not None:
                    if 0 < nt < MT - 1:
                        _run(q_partial(oq_next, out[nt - 1], nt - 1))
                    if nt == MT - 2:
                        _run(q_partial(oq_next, out[nt], nt))
            return out
        else:
            mt = list(range(nvf, FT))
            vd = mt[:VD_TILES]
            md = [ft for ft in mt if ft not in vd] + list(range(nvf))
            last = md[-2:]

            def g_produce(i):
                if i == 0:
                    return _by_column(gu_keys(mt[:2]), gu_op, MT)
                return [] if i == 1 else _by_item(gu_keys([mt[i]]), gu_op, MT)

            def g_consume(ft):
                if ft in vd:
                    return []
                if ft in last:
                    return _by_column(last, dn_op, MT) if ft == last[-1] else []
                return _by_item([ft], dn_op, MT)

            ms = _skewed(len(mt), SKEW_F, g_produce, lambda i: g_consume(mt[i]))
            for ft in range(nvf):
                ms += g_consume(ft)
            facc, aw, yv = {}, {}, {}

            def f_vstep(fts, s):
                def f(dep):
                    keys = [(w, wf if F32_P4 else None, ft) for ft in fts
                            for w, wf in ((WG32, WGF), (WU32, WUF))]
                    vpu_matvec_step(facc, keys, s, dep)
                    if s == M // 16 - 1:
                        for ft in fts:
                            for wh, (w, cs) in enumerate(((WG32, CSG), (WU32, CSU))):
                                pre[ft, wh] = _sublane_sum(facc[id(w), ft]) - mu * cs[ft]
                            finish(ft)
                    return facc[id(WG32), fts[0]]
                return _valu((8 if F32_P4 else 12) * len(fts))(f)

            def dxlu_op(ft):
                def f(dep):
                    aw[ft] = _col_bcast(acts[ft][0:1])
                    return pltpu.bitcast(aw[ft][:R], F32)
                f.ready = lambda: ft in acts
                return f

            def d_vstep(ft, k):
                def f(dep):
                    w = aw[ft][k * R:(k + 1) * R]
                    ce, co = link(_lo(w), dep), _hi(w)
                    r0 = ft * W2 + k * R
                    for nt in range(MT):
                        w = WD32[nt, r0:r0 + R, :]
                        _acc(yv, nt, _lo(w) * ce + _hi(w) * co)
                    return yv[0]
                return _valu(6 * MT + 2)(f)

            if nvf:
                make_xb(xt)
            vs = [f_vstep(list(range(f0, min(nvf, f0 + VF_GROUP))), s)
                  for f0 in range(0, nvf, VF_GROUP) for s in range(M // 16)]
            pos = max(0, len(vs) - XLU_EARLY)
            for i, ft in enumerate(vd[:XLU_AHEAD]):
                vs.insert(pos + i, dxlu_op(ft))
            for i, ft in enumerate(vd):
                if i + XLU_AHEAD < len(vd):
                    vs.append(dxlu_op(vd[i + XLU_AHEAD]))
                vs += [d_vstep(ft, k) for k in range(L // 16)]
            _cosched(ms, vs, P4_CFG)
            if vd:
                y = {nt: y[nt] + _sublane_sum(yv[nt]) for nt in range(MT)}
        return [_round_bf16(xt[nt] + xn[nt] + y[nt] * gate) for nt in range(MT)]

    for c in c_small:
        c.wait()
    x = jnp.broadcast_to(x_v[...].astype(F32), (R, M))
    zero_v.append(pltpu.bitcast(x[:, :L], U32) & jnp.uint32(0xFFFF))
    zero_s.append(jnp.max(zero_v[0].astype(jnp.int32)))
    xt = [x[:, t * L:(t + 1) * L] for t in range(MT)]
    xt = attention(xt, True, {})
    oq2 = {}
    xt = ffn(xt, True, oq2 if N_LAYERS > 1 else None)
    if N_LAYERS > 1:
        xt = attention(xt, False, oq2)
        xt = ffn(xt, False)
    for nt in range(MT):
        o_ref[:, nt * L:(nt + 1) * L] = xt[nt][0:1].astype(o_ref.dtype)


@jax.jit
def pallas_interleave_layers__compressed_kv_cla__moe_arch_mod__decode_kernel(
    A_x: jax.Array,
    A_c_kv: jax.Array,
    A_w_q: jax.Array,
    A_w_uk: jax.Array,
    A_w_uv: jax.Array,
    A_w_o: jax.Array,
    B_x: jax.Array,
    B_w_r: jax.Array,
    B_w_gate: jax.Array,
    B_w_up: jax.Array,
    B_w_down: jax.Array,
):
    del B_x
    args = (
        A_x.reshape(1, M),
        B_w_r,
        A_w_q,
        A_w_uk,
        A_c_kv.reshape(SK, DC),
        A_w_uv,
        B_w_gate.T,
        B_w_up.T,
        A_w_o.reshape(H * D, M),
        B_w_down,
    )
    n_sems = 6 + len(WO_SPLIT) + MT
    scratch = [
        pltpu.VMEM((1, M), BF16),
        pltpu.VMEM((M,), BF16),
        pltpu.VMEM((M, H, D), BF16),
        pltpu.VMEM((DC, H, D), BF16),
        pltpu.VMEM((SK, DC), BF16),
        pltpu.VMEM((DC, H, D), BF16),
        pltpu.VMEM((FF, M), BF16),
        pltpu.VMEM((FF, M), BF16),
        pltpu.VMEM((H * D, M), BF16),
        pltpu.VMEM((MT, FF, L), BF16),
        pltpu.VMEM((H, M // 2, D), U32),
        pltpu.VMEM((H, DC // 2, L), U32),
        pltpu.VMEM((CT, SK // 2, L), U32),
        pltpu.VMEM((KT, DC // 2, L), U32),
        pltpu.VMEM((H, DC // 2, D), U32),
        pltpu.VMEM((FT, M // 2, L), U32),
        pltpu.VMEM((FT - 1, M // 2, L), U32),
        pltpu.VMEM((MT, H * D // 2, L), U32),
        pltpu.VMEM((MT, FF // 2, L), U32),
        pltpu.VMEM((max(VA_HEADS, 1), 2, DC // 2, L), F32),
        pltpu.VMEM((max(VO_HEADS, 1), 2, MT, W2, L), F32),
        pltpu.VMEM((max(VF_TILES, 1), 2, M // 2, L), F32),
        pltpu.VMEM((max(VF_TILES, 1), 2, M // 2, L), F32),
        pltpu.VMEM((FT, R, L), F32),
        pltpu.VMEM((FT, R, L), F32),
        pltpu.VMEM((M // 2, L), F32),
        pltpu.VMEM((M // 2, L), F32),
        pltpu.SemaphoreType.DMA((n_sems,)),
    ]
    out = pl.pallas_call(
        _kernel,
        out_shape=jax.ShapeDtypeStruct((1, M), A_x.dtype),
        in_specs=[pl.BlockSpec(memory_space=pl.ANY)] * len(args),
        out_specs=pl.BlockSpec(memory_space=pltpu.VMEM),
        scratch_shapes=scratch,
        compiler_params=pltpu.CompilerParams(
            vmem_limit_bytes=100 * 1024 * 1024,
            disable_semaphore_checks=True),
        name="mla_moe_decode",
    )(*args)
    return out.reshape(1, 1, M)
```
